```python
import jax
import jax.numpy as jnp

def _softmax(x, axis=-1):
    return jax.nn.softmax(x, axis=axis)

def _gelu(x):
    return jax.nn.gelu(x, approximate=True)

def _silu(x):
    return jax.nn.silu(x)

def _sigmoid(x):
    return jax.nn.sigmoid(x)

def _layernorm(x, axis=-1, eps=1e-05):
    m = jnp.mean(x, axis=axis, keepdims=True)
    v = jnp.var(x, axis=axis, keepdims=True)
    return (x - m) / jnp.sqrt(v + eps)

def _scatter_add(tgt, idx, src, axis=0):
    return tgt.at[idx].add(src)

def _segment_sum(src, seg, n):
    return jax.ops.segment_sum(src, seg, n)

class _Rng:

    def __init__(self, key):
        self._k = key

    def _next(self):
        self._k, sub = jax.random.split(self._k)
        return sub

    def normal(self, shape):
        return jax.random.normal(self._next(), shape, dtype=jnp.bfloat16)

    def randint(self, lo, hi, shape):
        return jax.random.randint(self._next(), shape, lo, hi, dtype=jnp.int32)

    def uniform(self, shape, lo=0.0, hi=1.0):
        return jax.random.uniform(self._next(), shape, jnp.bfloat16, lo, hi)

    def permutation(self, n):
        return jax.random.permutation(self._next(), n)
kernel_name = 'interleave_layers__memory_aug_recurrent_mem_tr__moe_arch_mod__prompt'

def setup_inputs():
    _rng = _Rng(jax.random.key(int.from_bytes(__import__("os").urandom(4), "little")))
    _w = lambda a: (lambda t: t.astype(jnp.bfloat16) if jnp.issubdtype(t.dtype, jnp.floating) else t)(jnp.asarray(a))

    def _A_setup():
        B, S, Dm = (1, 2048, 512)
        H, Dh = (32, 128)
        M, seg = (8, 32)
        seg = min(seg, S)
        S = S // seg * seg
        return {'x': _w((lambda *s: _rng.normal(s) * 0.05)(B, S, Dm)), 'mem0': _w((lambda *s: _rng.normal(s) * 0.05)(B, M, Dm)), 'Wq': _w((lambda *s: _rng.normal(s) * 0.05)(Dm, H, Dh) * Dm ** (-0.5)), 'Wk': _w((lambda *s: _rng.normal(s) * 0.05)(Dm, H, Dh) * Dm ** (-0.5)), 'Wv': _w((lambda *s: _rng.normal(s) * 0.05)(Dm, H, Dh) * Dm ** (-0.5)), 'Wo': _w((lambda *s: _rng.normal(s) * 0.05)(H, Dh, Dm) * (H * Dh) ** (-0.5)), 'seg_len': seg}
    _A_in = _A_setup()

    def _B_setup():
        B, S, D, F, C = (1, 2048, 512, 1792, 1)
        return {'x': _w((lambda *s: _rng.normal(s) * 0.05)(B, S, D)), 'w_r': _w((lambda *s: _rng.normal(s) * 0.05)(D)), 'w_gate': _w((lambda *s: _rng.normal(s) * 0.05)(D, F)), 'w_up': _w((lambda *s: _rng.normal(s) * 0.05)(D, F)), 'w_down': _w((lambda *s: _rng.normal(s) * 0.05)(F, D))}
    _B_in = _B_setup()
    return {'A_x': _A_in['x'], 'A_mem0': _A_in['mem0'], 'A_Wq': _A_in['Wq'], 'A_Wk': _A_in['Wk'], 'A_Wv': _A_in['Wv'], 'A_Wo': _A_in['Wo'], 'A_seg_len': _A_in['seg_len'], 'B_x': _B_in['x'], 'B_w_r': _B_in['w_r'], 'B_w_gate': _B_in['w_gate'], 'B_w_up': _B_in['w_up'], 'B_w_down': _B_in['w_down']}

def reference(A_x, A_mem0, A_Wq, A_Wk, A_Wv, A_Wo, A_seg_len, B_x, B_w_r, B_w_gate, B_w_up, B_w_down):

    def _A_ref(x, mem0, Wq, Wk, Wv, Wo, seg_len):
        B, S, Dm = x.shape
        H, Dh = (Wq.shape[1], Wq.shape[2])
        M = mem0.shape[1]
        scale = Dh ** (-0.5)
        n_seg = S // seg_len
        L = M + seg_len
        idx = jnp.arange(L)
        mask = (idx[:, None] < M) | (idx[:, None] >= idx[None, :])
        mem = mem0
        outs = []
        for s in range(n_seg):
            xs = x[:, s * seg_len:(s + 1) * seg_len, :].copy()
            h = jnp.concatenate([mem, xs], axis=1)
            q = jnp.einsum('btd,dhe->bhte', h, Wq)
            k = jnp.einsum('btd,dhe->bhte', h, Wk)
            v = jnp.einsum('btd,dhe->bhte', h, Wv)
            scores = jnp.einsum('bhqe,bhke->bhqk', q, k) * scale
            scores = jnp.where(mask[None, None], scores, -1000000000.0)
            p = _softmax(scores, axis=-1)
            o = jnp.einsum('bhqk,bhke->bhqe', p, v)
            o = jnp.einsum('bhte,hed->btd', o, Wo)
            mem = o[:, :M, :].copy()
            outs.append(o[:, M:, :])
        return jnp.concatenate(outs, axis=1)

    def _B_ref(x, w_r, w_gate, w_up, w_down):
        B, S, D = x.shape
        C = 1
        r = x @ w_r
        idx = jnp.argsort(-r, axis=-1)[:, :C]
        idx_e = jnp.repeat(idx.reshape(B, C, 1), D, axis=2)
        x_sel = jnp.take_along_axis(x, idx_e, axis=1)
        g = _silu(x_sel @ w_gate)
        u = x_sel @ w_up
        y = g * u @ w_down
        r_sel = _sigmoid(jnp.take_along_axis(r, idx, axis=1))
        y = y * r_sel.reshape(B, C, 1)
        b_off = (jnp.arange(B) * S).reshape(B, 1)
        flat_idx = (idx + b_off).reshape(B * C)
        zero = (x * 0.0).reshape(B * S, D)
        upd = _scatter_add(zero, flat_idx, y.reshape(B * C, D), axis=0)
        return x + upd.reshape(B, S, D)
    x = A_x
    x = x + _A_ref(_layernorm(x, axis=-1), A_mem0, A_Wq, A_Wk, A_Wv, A_Wo, A_seg_len)
    x = x + _B_ref(_layernorm(x, axis=-1), B_w_r, B_w_gate, B_w_up, B_w_down)
    x = x + _A_ref(_layernorm(x, axis=-1), A_mem0, A_Wq, A_Wk, A_Wv, A_Wo, A_seg_len)
    x = x + _B_ref(_layernorm(x, axis=-1), B_w_r, B_w_gate, B_w_up, B_w_down)
    return x
```

```python
import functools
import math

import jax
import jax.numpy as jnp
from jax import lax
import jax.experimental.pallas as pl
import jax.experimental.pallas.tpu as pltpu

F32 = jnp.float32
BF16 = jnp.bfloat16
U32 = jnp.uint32

S, D, H, DH, M, SEG = 2048, 512, 32, 128, 8, 32
FF = 1792
HD = H * DH
PAIR = 2 * SEG
NPAIR = S // PAIR
PAD = PAIR
LN_EPS = 1e-05
NEG = -1000000000.0
EXP2_SCALE = (DH ** -0.5) * math.log2(math.e)


def _rnd(x):
    return x.astype(BF16).astype(F32)


def _layernorm(x):
    mean = jnp.sum(x, axis=-1, keepdims=True) * (1.0 / D)
    c = x - mean
    var = jnp.sum(c * c, axis=-1, keepdims=True) * (1.0 / D)
    den = _rnd(jnp.sqrt(_rnd(_rnd(var) + _rnd(jnp.float32(LN_EPS)))))
    inv = 1.0 / den
    return _rnd(_rnd(x - _rnd(mean)) * inv)


def _dot(a, b):
    return jnp.dot(a, b, preferred_element_type=F32)


def _dot_nt(a, b):
    return lax.dot_general(a, b, (((1,), (1,)), ((), ())), preferred_element_type=F32)


def _softmax_bf16(s, mask):
    s = jnp.where(mask, s, NEG)
    m = jnp.max(s, axis=-1, keepdims=True)
    e = jnp.exp2((s - m) * EXP2_SCALE)
    l = jnp.sum(e, axis=-1, keepdims=True)
    r = pl.reciprocal(l, approx=True)
    r = r * (2.0 - l * r)
    return (e * r).astype(BF16)


def _kernel(x_hbm, mem0_hbm, wq_hbm, wk_hbm, wv_hbm, wo_hbm, wr_hbm, wg_hbm, wu_hbm, wd_hbm,
            out_ref,
            x_raw, mem0_v, wr_v, stage, wo_raw, wg_v, wu_v, wd_v,
            wqkv, wo, tmp, xres, x1buf, lbuf, hbuf, rbuf, obuf, sems, *, G):
    NG = H // G
    GW = G * DH

    cp_x = pltpu.make_async_copy(x_hbm, x_raw, sems.at[0])
    cp_m = pltpu.make_async_copy(mem0_hbm, mem0_v, sems.at[1])
    cp_r = pltpu.make_async_copy(wr_hbm, wr_v, sems.at[2])
    cp_w = [pltpu.make_async_copy(w, stage.at[i], sems.at[3 + i])
            for i, w in enumerate((wq_hbm, wk_hbm, wv_hbm))]
    cp_o = pltpu.make_async_copy(wo_hbm, wo_raw, sems.at[6])
    cp_mlp = [pltpu.make_async_copy(s_, d_, sems.at[7 + i])
              for i, (s_, d_) in enumerate(((wg_hbm, wg_v), (wu_hbm, wu_v), (wd_hbm, wd_v)))]
    cp_x.start()
    cp_m.start()
    cp_r.start()
    for c in cp_w:
        c.start()
    cp_o.start()
    for c in cp_mlp:
        c.start()

    xres[0:PAD, :] = jnp.zeros((PAD, D), F32)
    cp_x.wait()

    def ln0(i, carry):
        r0 = pl.multiple_of(i * 32, 32)
        xv = x_raw[pl.ds(r0, 32), :].astype(F32)
        xres[pl.ds(PAD + r0, 32), :] = xv
        hbuf[pl.ds(PAD + r0, 32), :] = _layernorm(xv)
        return carry

    lax.fori_loop(0, S // 32, ln0, 0)

    for mi in range(3):
        cp_w[mi].wait()

        def relay(c, carry, mi=mi):
            r0 = pl.multiple_of(c * (16 * H), 16 * H)
            tmp[...] = stage[mi, pl.ds(r0, 16 * H), :].astype(F32)
            o0 = pl.multiple_of(c * 8, 8)
            for h in range(H):
                t = tmp[pl.ds(h, 16, stride=H), :].astype(BF16)
                col = mi * HD + h * DH
                wqkv[pl.ds(o0, 8), col:col + DH] = pltpu.bitcast(t, U32)
            return carry

        lax.fori_loop(0, D // 16, relay, 0)

    cp_o.wait()

    def relay_o(c, carry):
        r0 = pl.multiple_of(c * 128, 128)
        o0 = pl.multiple_of(c * 64, 64)
        wo[pl.ds(o0, 64), :] = pltpu.bitcast(wo_raw[pl.ds(r0, 128), :], U32)
        return carry

    lax.fori_loop(0, HD // 128, relay_o, 0)

    cp_m.wait()
    cp_r.wait()
    wr = wr_v[...].astype(F32)

    L = 48
    qi = lax.broadcasted_iota(jnp.int32, (L, L), 0)
    kj = lax.broadcasted_iota(jnp.int32, (L, L), 1)
    mask_a = (kj < 40) & ((qi < M) | (kj <= qi))
    qpos = jnp.where(qi >= 40, qi - 40, qi)
    kpos = jnp.where(kj >= 40, kj - 40, kj)
    kvalid = (kj < 32) | (kj >= 40)
    mask_b = (kj < M) | (kvalid & ((qi < M) | (kpos <= qpos)))

    def w_cols(mi, g):
        c0 = mi * HD + g * GW
        return pltpu.bitcast(wqkv[:, c0:c0 + GW], BF16)

    def wo_rows(g):
        r0 = g * GW // 2
        return pltpu.bitcast(wo[r0:r0 + GW // 2, :], BF16)

    def seg_step(lhs, mask, carry_in):
        first = carry_in is None
        q, k, v, p, o = {}, {}, {}, {}, {}
        keep = dict(q={}, k={}, v={}, o={})
        acc = [None]

        def proj(mi, g, name):
            y = _dot(lhs, w_cols(mi, g)).astype(BF16)
            if first:
                keep[name][g] = y[32:48]
                return y
            return jnp.concatenate([y, carry_in[name][g]], axis=0)

        def qk(g):
            q[g] = proj(0, g, 'q')
            k[g] = proj(1, g, 'k')

        def sc(g):
            for j in range(G):
                sl = slice(j * DH, (j + 1) * DH)
                p[g, j] = _softmax_bf16(_dot_nt(q[g][:, sl], k[g][:, sl]), mask)

        def vv(g):
            v[g] = proj(2, g, 'v')

        def pv(g):
            og = jnp.concatenate(
                [_dot(p[g, j], v[g][:, j * DH:(j + 1) * DH]) for j in range(G)], axis=1)
            if first:
                keep['o'][g] = og[32:40]
                o[g] = og[0:32].astype(BF16)
            else:
                o[g] = jnp.concatenate(
                    [og[0:32], carry_in['o'][g], og[40:48]], axis=0).astype(BF16)

        def op(g):
            y = _dot(o[g], wo_rows(g))
            acc[0] = y if acc[0] is None else acc[0] + y

        qk(0)
        for g in range(1, NG):
            qk(g)
            sc(g - 1)
        vv(0)
        sc(NG - 1)
        for g in range(1, NG + 2):
            if g < NG:
                vv(g)
            if g - 1 < NG:
                pv(g - 1)
            if g >= 2:
                op(g - 2)
        return acc[0], keep

    def post(base):
        for c in range(PAIR // 16):
            rows = pl.ds(base + c * 16, 16)
            x1 = _rnd(xres[rows, :] + _rnd(obuf[c * 16:(c + 1) * 16, :]))
            ln = _layernorm(x1)
            r = _rnd(jnp.sum(ln * wr, axis=-1, keepdims=True))
            x2 = _rnd(x1 + ln)
            x1buf[rows, :] = x1
            lbuf[rows, :] = ln
            rbuf[rows, :] = jnp.broadcast_to(r, (16, 128))
            xres[rows, :] = x2
            hbuf[rows, :] = _layernorm(x2)

    def pair_body(pi, mem):
        base = pl.multiple_of(pi * PAIR, PAIR)
        ha = hbuf[pl.ds(base + PAD, 40), :]
        hb = hbuf[pl.ds(base + PAD + 40, 24), :]
        lhs_a = jnp.concatenate([mem, ha], axis=0).astype(BF16)
        post(base)
        acc_a, keep = seg_step(lhs_a, mask_a, None)
        lhs_b = jnp.concatenate([acc_a[0:8], hb], axis=0).astype(BF16)
        acc_b, _ = seg_step(lhs_b, mask_b, keep)
        obuf[0:24, :] = acc_a[8:32]
        obuf[24:40, :] = acc_b[32:48]
        obuf[40:64, :] = acc_b[8:32]
        return acc_b[0:8]

    def layer(li, carry):
        obuf[...] = jnp.zeros((PAIR, D), F32)
        mem0 = mem0_v[...].astype(F32)
        lax.fori_loop(0, NPAIR, pair_body, mem0)
        post(S)

        @pl.when(li == 0)
        def _():
            for c in cp_mlp:
                c.wait()

        rall = rbuf[PAD:PAD + S, :]
        rmax = jnp.max(rall)
        rows = lax.broadcasted_iota(jnp.int32, (S, 128), 0)
        idx = jnp.min(jnp.where(rall == rmax, rows, S - 1))
        row = pl.ds(PAD + idx, 1)
        lsel = lbuf[row, :]
        xs = jnp.broadcast_to(lsel, (16, D)).astype(BF16)
        gpre = _rnd(_dot(xs, wg_v[...]))
        gate = _rnd(gpre * _rnd(jax.nn.sigmoid(gpre)))
        up = _rnd(_dot(xs, wu_v[...]))
        y = _rnd(_dot((gate * up).astype(BF16), wd_v[...]))[0:1]
        rsel = _rnd(jax.nn.sigmoid(rbuf[row, :][:, 0:1]))
        y = _rnd(y * rsel)
        x2 = _rnd(x1buf[row, :] + _rnd(lsel + y))
        xres[row, :] = x2
        hbuf[row, :] = _layernorm(x2)
        return carry

    lax.fori_loop(0, 2, layer, 0)

    def wout(i, carry):
        r0 = pl.multiple_of(i * 64, 64)
        out_ref[pl.ds(r0, 64), :] = xres[pl.ds(PAD + r0, 64), :].astype(BF16)
        return carry

    lax.fori_loop(0, S // 64, wout, 0)


def _build(G=4):
    any_spec = pl.BlockSpec(memory_space=pl.ANY)
    return pl.pallas_call(
        functools.partial(_kernel, G=G),
        out_shape=jax.ShapeDtypeStruct((S, D), BF16),
        in_specs=[any_spec] * 10,
        out_specs=pl.BlockSpec(memory_space=pltpu.VMEM),
        scratch_shapes=[
            pltpu.VMEM((S, D), BF16),
            pltpu.VMEM((M, D), BF16),
            pltpu.VMEM((1, D), BF16),
            pltpu.VMEM((3, D * H, DH), BF16),
            pltpu.VMEM((HD, D), BF16),
            pltpu.VMEM((D, FF), BF16),
            pltpu.VMEM((D, FF), BF16),
            pltpu.VMEM((FF, D), BF16),
            pltpu.VMEM((D // 2, 3 * HD), U32),
            pltpu.VMEM((HD // 2, D), U32),
            pltpu.VMEM((16 * H, DH), F32),
            pltpu.VMEM((PAD + S, D), F32),
            pltpu.VMEM((PAD + S, D), F32),
            pltpu.VMEM((PAD + S, D), F32),
            pltpu.VMEM((PAD + S, D), F32),
            pltpu.VMEM((PAD + S, 128), F32),
            pltpu.VMEM((PAIR, D), F32),
            pltpu.SemaphoreType.DMA((10,)),
        ],
        compiler_params=pltpu.CompilerParams(vmem_limit_bytes=110 * 1024 * 1024),
    )


@functools.partial(jax.jit, static_argnames=("A_seg_len",))
def pallas_interleave_layers__memory_aug_recurrent_mem_tr__moe_arch_mod__prompt_kernel(
    A_x: jax.Array,
    A_mem0: jax.Array,
    A_Wq: jax.Array,
    A_Wk: jax.Array,
    A_Wv: jax.Array,
    A_Wo: jax.Array,
    A_seg_len,
    B_x: jax.Array,
    B_w_r: jax.Array,
    B_w_gate: jax.Array,
    B_w_up: jax.Array,
    B_w_down: jax.Array,
):
    assert A_seg_len == SEG and A_x.shape == (1, S, D)
    del B_x
    out = _build()(
        A_x.reshape(S, D),
        A_mem0.reshape(M, D),
        A_Wq.reshape(D * H, DH),
        A_Wk.reshape(D * H, DH),
        A_Wv.reshape(D * H, DH),
        A_Wo.reshape(HD, D),
        B_w_r.reshape(1, D),
        B_w_gate,
        B_w_up,
        B_w_down,
    )
    return out.reshape(1, S, D)
```

```python
import functools
import math

import jax
import jax.numpy as jnp
from jax import lax
import jax.experimental.pallas as pl
import jax.experimental.pallas.tpu as pltpu

F32 = jnp.float32
BF16 = jnp.bfloat16
U32 = jnp.uint32

S, D, H, DH, M, SEG = 2048, 512, 32, 128, 8, 32
FF = 1792
HD = H * DH
PAIR = 2 * SEG
NPAIR = S // PAIR
PAD = PAIR
LN_EPS = 1e-05
NEG = -1000000000.0
EXP2_SCALE = (DH ** -0.5) * math.log2(math.e)


def _rnd(x):
    return x.astype(BF16).astype(F32)


def _layernorm(x):
    mean = jnp.sum(x, axis=-1, keepdims=True) * (1.0 / D)
    c = x - mean
    var = jnp.sum(c * c, axis=-1, keepdims=True) * (1.0 / D)
    den = _rnd(jnp.sqrt(_rnd(_rnd(var) + _rnd(jnp.float32(LN_EPS)))))
    inv = 1.0 / den
    return _rnd(_rnd(x - _rnd(mean)) * inv)


def _dot(a, b):
    return jnp.dot(a, b, preferred_element_type=F32)


def _dot_nt(a, b):
    return lax.dot_general(a, b, (((1,), (1,)), ((), ())), preferred_element_type=F32)


def _softmax_bf16(s, mask):
    s = jnp.where(mask, s, NEG)
    m = jnp.max(s, axis=-1, keepdims=True)
    e = jnp.exp2((s - m) * EXP2_SCALE)
    l = jnp.sum(e, axis=-1, keepdims=True)
    r = pl.reciprocal(l, approx=True)
    r = r * (2.0 - l * r)
    return (e * r).astype(BF16)


def _kernel(x_hbm, mem0_hbm, wq_hbm, wk_hbm, wv_hbm, wo_hbm, wr_hbm, wg_hbm, wu_hbm, wd_hbm,
            out_ref,
            x_raw, mem0_v, wr_v, stage, wo_raw, wg_v, wu_v, wd_v,
            wqkv, wo, tmp, xres, x1buf, lbuf, hbuf, rbuf, obuf, sems, *, G):
    NG = H // G
    GW = G * DH

    cp_x = pltpu.make_async_copy(x_hbm, x_raw, sems.at[0])
    cp_m = pltpu.make_async_copy(mem0_hbm, mem0_v, sems.at[1])
    cp_r = pltpu.make_async_copy(wr_hbm, wr_v, sems.at[2])
    cp_w = [pltpu.make_async_copy(w, stage.at[i], sems.at[3 + i])
            for i, w in enumerate((wq_hbm, wk_hbm, wv_hbm))]
    cp_o = pltpu.make_async_copy(wo_hbm, wo_raw, sems.at[6])
    cp_mlp = [pltpu.make_async_copy(s_, d_, sems.at[7 + i])
              for i, (s_, d_) in enumerate(((wg_hbm, wg_v), (wu_hbm, wu_v), (wd_hbm, wd_v)))]
    cp_x.start()
    cp_m.start()
    cp_r.start()
    for c in cp_w:
        c.start()
    cp_o.start()
    for c in cp_mlp:
        c.start()

    xres[0:PAD, :] = jnp.zeros((PAD, D), F32)
    cp_x.wait()

    def ln0(i, carry):
        r0 = pl.multiple_of(i * 32, 32)
        xv = x_raw[pl.ds(r0, 32), :].astype(F32)
        xres[pl.ds(PAD + r0, 32), :] = xv
        hbuf[pl.ds(PAD + r0, 32), :] = _layernorm(xv)
        return carry

    lax.fori_loop(0, S // 32, ln0, 0)

    for mi in range(3):
        cp_w[mi].wait()

        def relay(c, carry, mi=mi):
            r0 = pl.multiple_of(c * (16 * H), 16 * H)
            tmp[...] = stage[mi, pl.ds(r0, 16 * H), :].astype(F32)
            o0 = pl.multiple_of(c * 8, 8)
            for h in range(H):
                t = tmp[pl.ds(h, 16, stride=H), :].astype(BF16)
                col = mi * HD + h * DH
                wqkv[pl.ds(o0, 8), col:col + DH] = pltpu.bitcast(t, U32)
            return carry

        lax.fori_loop(0, D // 16, relay, 0)

    cp_o.wait()

    def relay_o(c, carry):
        r0 = pl.multiple_of(c * 128, 128)
        o0 = pl.multiple_of(c * 64, 64)
        wo[pl.ds(o0, 64), :] = pltpu.bitcast(wo_raw[pl.ds(r0, 128), :], U32)
        return carry

    lax.fori_loop(0, HD // 128, relay_o, 0)

    cp_m.wait()
    cp_r.wait()
    wr = wr_v[...].astype(F32)

    qi = lax.broadcasted_iota(jnp.int32, (32, 48), 0)
    kj = lax.broadcasted_iota(jnp.int32, (32, 48), 1)
    mask_a = (kj < 40) & ((qi < M) | (kj <= qi))
    qi = lax.broadcasted_iota(jnp.int32, (48, 80), 0)
    kj = lax.broadcasted_iota(jnp.int32, (48, 80), 1)
    kb0 = (kj >= 40) & (kj < 48)
    m_mem = (qi < M) & ((kj < 32) | kb0)
    m_xb = (qi >= M) & (qi < 32) & ((kj <= qi) | kb0)
    m_xa = (qi >= 32) & (qi < 40) & ((kj >= 48) | ((kj >= 32) & (kj <= qi)))
    m_b0 = (qi >= 40) & ((kj < M) | (kb0 & (kj <= qi)))
    mask_b = m_mem | m_xb | m_xa | m_b0

    def w_cols(mi, g):
        c0 = mi * HD + g * GW
        return pltpu.bitcast(wqkv[:, c0:c0 + GW], BF16)

    def wo_rows(g):
        r0 = g * GW // 2
        return pltpu.bitcast(wo[r0:r0 + GW // 2, :], BF16)

    def seg_step(lhs_q, lhs_kv, mask, prev):
        q, k, v, p, o = {}, {}, {}, {}, {}
        acc = [None]

        def kv(mi, g):
            y = _dot(lhs_kv, w_cols(mi, g)).astype(BF16)
            if prev is None:
                return y
            z = prev[mi - 1][g]
            return jnp.concatenate([y, z[32:48], z[0:32]], axis=0)

        def qk(g):
            q[g] = _dot(lhs_q, w_cols(0, g)).astype(BF16)
            k[g] = kv(1, g)

        def sc(g):
            for j in range(G):
                sl = slice(j * DH, (j + 1) * DH)
                p[g, j] = _softmax_bf16(_dot_nt(q[g][:, sl], k[g][:, sl]), mask)

        def vv(g):
            v[g] = kv(2, g)

        def pv(g):
            o[g] = jnp.concatenate(
                [_dot(p[g, j], v[g][:, j * DH:(j + 1) * DH]) for j in range(G)],
                axis=1).astype(BF16)

        def op(g):
            y = _dot(o[g], wo_rows(g))
            acc[0] = y if acc[0] is None else acc[0] + y

        qk(0)
        for g in range(1, NG):
            qk(g)
            sc(g - 1)
        vv(0)
        sc(NG - 1)
        for g in range(1, NG + 2):
            if g < NG:
                vv(g)
            if g - 1 < NG:
                pv(g - 1)
            if g >= 2:
                op(g - 2)
        return acc[0], (k, v)

    def post(base):
        for c in range(PAIR // 16):
            rows = pl.ds(base + c * 16, 16)
            x1 = _rnd(xres[rows, :] + _rnd(obuf[c * 16:(c + 1) * 16, :]))
            ln = _layernorm(x1)
            r = _rnd(jnp.sum(ln * wr, axis=-1, keepdims=True))
            x2 = _rnd(x1 + ln)
            x1buf[rows, :] = x1
            lbuf[rows, :] = ln
            rbuf[rows, :] = jnp.broadcast_to(r, (16, 128))
            xres[rows, :] = x2
            hbuf[rows, :] = _layernorm(x2)

    def pair_body(pi, mem):
        base = pl.multiple_of(pi * PAIR, PAIR)
        ha = hbuf[pl.ds(base + PAD, 40), :]
        hb = hbuf[pl.ds(base + PAD + 40, 24), :]
        lhs_a = jnp.concatenate([mem, ha], axis=0).astype(BF16)
        post(base)
        acc_a, kv_a = seg_step(lhs_a[0:32], lhs_a, mask_a, None)
        lhs_b = jnp.concatenate([acc_a[0:8], hb], axis=0).astype(BF16)
        lhs_bq = jnp.concatenate([lhs_b, lhs_a[32:48]], axis=0)
        acc_b, _ = seg_step(lhs_bq, lhs_b, mask_b, kv_a)
        obuf[0:24, :] = acc_a[8:32]
        obuf[24:40, :] = acc_b[32:48]
        obuf[40:64, :] = acc_b[8:32]
        return acc_b[0:8]

    def layer(li, carry):
        obuf[...] = jnp.zeros((PAIR, D), F32)
        mem0 = mem0_v[...].astype(F32)
        lax.fori_loop(0, NPAIR, pair_body, mem0)
        post(S)

        @pl.when(li == 0)
        def _():
            for c in cp_mlp:
                c.wait()

        rall = rbuf[PAD:PAD + S, :]
        rmax = jnp.max(rall)
        rows = lax.broadcasted_iota(jnp.int32, (S, 128), 0)
        idx = jnp.min(jnp.where(rall == rmax, rows, S - 1))
        row = pl.ds(PAD + idx, 1)
        lsel = lbuf[row, :]
        xs = jnp.broadcast_to(lsel, (16, D)).astype(BF16)
        gpre = _rnd(_dot(xs, wg_v[...]))
        gate = _rnd(gpre * _rnd(jax.nn.sigmoid(gpre)))
        up = _rnd(_dot(xs, wu_v[...]))
        y = _rnd(_dot((gate * up).astype(BF16), wd_v[...]))[0:1]
        rsel = _rnd(jax.nn.sigmoid(rbuf[row, :][:, 0:1]))
        y = _rnd(y * rsel)
        x2 = _rnd(x1buf[row, :] + _rnd(lsel + y))
        xres[row, :] = x2
        hbuf[row, :] = _layernorm(x2)
        return carry

    lax.fori_loop(0, 2, layer, 0)

    def wout(i, carry):
        r0 = pl.multiple_of(i * 64, 64)
        out_ref[pl.ds(r0, 64), :] = xres[pl.ds(PAD + r0, 64), :].astype(BF16)
        return carry

    lax.fori_loop(0, S // 64, wout, 0)


CFG = dict(G=4)


def _build():
    any_spec = pl.BlockSpec(memory_space=pl.ANY)
    return pl.pallas_call(
        functools.partial(_kernel, **CFG),
        out_shape=jax.ShapeDtypeStruct((S, D), BF16),
        in_specs=[any_spec] * 10,
        out_specs=pl.BlockSpec(memory_space=pltpu.VMEM),
        scratch_shapes=[
            pltpu.VMEM((S, D), BF16),
            pltpu.VMEM((M, D), BF16),
            pltpu.VMEM((1, D), BF16),
            pltpu.VMEM((3, D * H, DH), BF16),
            pltpu.VMEM((HD, D), BF16),
            pltpu.VMEM((D, FF), BF16),
            pltpu.VMEM((D, FF), BF16),
            pltpu.VMEM((FF, D), BF16),
            pltpu.VMEM((D // 2, 3 * HD), U32),
            pltpu.VMEM((HD // 2, D), U32),
            pltpu.VMEM((16 * H, DH), F32),
            pltpu.VMEM((PAD + S, D), F32),
            pltpu.VMEM((PAD + S, D), F32),
            pltpu.VMEM((PAD + S, D), F32),
            pltpu.VMEM((PAD + S, D), F32),
            pltpu.VMEM((PAD + S, 128), F32),
            pltpu.VMEM((PAIR, D), F32),
            pltpu.SemaphoreType.DMA((10,)),
        ],
        compiler_params=pltpu.CompilerParams(vmem_limit_bytes=110 * 1024 * 1024),
    )


@functools.partial(jax.jit, static_argnames=("A_seg_len",))
def pallas_interleave_layers__memory_aug_recurrent_mem_tr__moe_arch_mod__prompt_kernel(
    A_x: jax.Array,
    A_mem0: jax.Array,
    A_Wq: jax.Array,
    A_Wk: jax.Array,
    A_Wv: jax.Array,
    A_Wo: jax.Array,
    A_seg_len,
    B_x: jax.Array,
    B_w_r: jax.Array,
    B_w_gate: jax.Array,
    B_w_up: jax.Array,
    B_w_down: jax.Array,
):
    assert A_seg_len == SEG and A_x.shape == (1, S, D)
    del B_x
    out = _build()(
        A_x.reshape(S, D),
        A_mem0.reshape(M, D),
        A_Wq.reshape(D * H, DH),
        A_Wk.reshape(D * H, DH),
        A_Wv.reshape(D * H, DH),
        A_Wo.reshape(HD, D),
        B_w_r.reshape(1, D),
        B_w_gate,
        B_w_up,
        B_w_down,
    )
    return out.reshape(1, S, D)
```

```python
import functools
import math

import jax
import jax.numpy as jnp
from jax import lax
import jax.experimental.pallas as pl
import jax.experimental.pallas.tpu as pltpu

F32 = jnp.float32
BF16 = jnp.bfloat16
U32 = jnp.uint32

S, D, H, DH, M, SEG = 2048, 512, 32, 128, 8, 32
FF = 1792
HD = H * DH
PAIR = 2 * SEG
NPAIR = S // PAIR
PAD = PAIR
LN_EPS = 1e-05
NEG = -1000000000.0
EXP2_SCALE = (DH ** -0.5) * math.log2(math.e)


def _rnd(x):
    return x.astype(BF16).astype(F32)


def _layernorm(x):
    mean = jnp.sum(x, axis=-1, keepdims=True) * (1.0 / D)
    c = x - mean
    var = jnp.sum(c * c, axis=-1, keepdims=True) * (1.0 / D)
    den = _rnd(jnp.sqrt(_rnd(_rnd(var) + _rnd(jnp.float32(LN_EPS)))))
    inv = 1.0 / den
    return _rnd(_rnd(x - _rnd(mean)) * inv)


def _dot(a, b):
    return jnp.dot(a, b, preferred_element_type=F32)


def _dot_nt(a, b):
    return lax.dot_general(a, b, (((1,), (1,)), ((), ())), preferred_element_type=F32)


def _softmax_bf16(s, mask):
    s = jnp.where(mask, s, NEG)
    m = jnp.max(s, axis=-1, keepdims=True)
    e = jnp.exp2((s - m) * EXP2_SCALE)
    l = jnp.sum(e, axis=-1, keepdims=True)
    r = pl.reciprocal(l, approx=True)
    r = r * (2.0 - l * r)
    return (e * r).astype(BF16)


def _kernel(x_hbm, mem0_hbm, wq_hbm, wk_hbm, wv_hbm, wo_hbm, wr_hbm, wg_hbm, wu_hbm, wd_hbm,
            out_hbm,
            x_raw, mem0_v, wr_v, stage, wo_raw, wg_v, wu_v, wd_v,
            wqkv, wo, tmp, xres, x1buf, lbuf, hbuf, rbest, ibest, obuf, ostage,
            lhs_pre, pre, sems, osem, *, G, NPRE):
    NG = H // G
    GW = G * DH
    HC = 16
    GPC = HC // G
    NCH = 3 * H // HC

    cp_x = pltpu.make_async_copy(x_hbm, x_raw, sems.at[0])
    cp_m = pltpu.make_async_copy(mem0_hbm, mem0_v, sems.at[1])
    cp_r = pltpu.make_async_copy(wr_hbm, wr_v, sems.at[2])
    cp_o = pltpu.make_async_copy(wo_hbm, wo_raw, sems.at[3])
    cp_mlp = [pltpu.make_async_copy(s_, d_, sems.at[4 + i])
              for i, (s_, d_) in enumerate(((wg_hbm, wg_v), (wu_hbm, wu_v), (wd_hbm, wd_v)))]
    cp_x.start()
    for c in range(NCH):
        w = (wq_hbm, wk_hbm, wv_hbm)[c // 2]
        pltpu.make_async_copy(w.at[:, pl.ds((c % 2) * HC, HC), :], stage.at[c],
                              sems.at[7 + c]).start()
    cp_o.start()
    cp_m.start()
    cp_r.start()
    for c in cp_mlp:
        c.start()

    xres[0:PAD, :] = jnp.zeros((PAD, D), F32)
    cp_x.wait()

    def ln0(i, carry):
        for c in range(8):
            r0 = pl.multiple_of(i * 128 + c * 16, 16)
            xv = x_raw[pl.ds(r0, 16), :].astype(F32)
            xres[pl.ds(PAD + r0, 16), :] = xv
            hbuf[pl.ds(PAD + r0, 16), :] = _layernorm(xv)
        return carry

    lax.fori_loop(0, S // 128, ln0, 0)

    for p_ in range(NPRE):
        r0 = PAD + p_ * PAIR + 24
        lhs_pre[p_ * 8:(p_ + 1) * 8, :] = pltpu.bitcast(hbuf[r0:r0 + 16, :].astype(BF16), U32)

    TP = 20
    TSZ = 8 * TP

    def chunk(c, carry):
        pltpu.make_async_copy(wq_hbm.at[:, pl.ds(0, HC), :], stage.at[c], sems.at[7 + c]).wait()

        def relay(it, carry2):
            for u in range(4):
                d0 = pl.multiple_of(it * 64 + u * 16, 16)
                raw = pltpu.bitcast(stage[c, pl.ds(d0, 16), :, :], U32)
                for i in range(8):
                    ev, od = raw[2 * i], raw[2 * i + 1]
                    lo = (ev & jnp.uint32(0xFFFF)) | (od << 16)
                    hi = (ev >> 16) | (od & jnp.uint32(0xFFFF0000))
                    tmp[pl.ds(u * TSZ + i * TP, 8, stride=2), :] = lo
                    tmp[pl.ds(u * TSZ + i * TP + 1, 8, stride=2), :] = hi
            for u in range(4):
                o0 = pl.multiple_of(it * 32 + u * 8, 8)
                for hh in range(HC):
                    t = tmp[pl.ds(u * TSZ + hh, 8, stride=TP), :]
                    col = (hh % G) * DH
                    wqkv[c * GPC + hh // G, pl.ds(o0, 8), col:col + DH] = t
            return carry2

        lax.fori_loop(0, D // 64, relay, 0)
        if NPRE:
            lhs = pltpu.bitcast(lhs_pre[...], BF16)
            for gg in range(GPC):
                y = _dot(lhs, pltpu.bitcast(wqkv[c * GPC + gg], BF16)).astype(BF16)
                pre[c * GPC + gg] = pltpu.bitcast(y, U32)
        return carry

    lax.fori_loop(0, NCH, chunk, 0)

    cp_o.wait()

    def relay_o(c, carry):
        r0 = pl.multiple_of(c * 128, 128)
        o0 = pl.multiple_of(c * 64, 64)
        wo[pl.ds(o0, 64), :] = pltpu.bitcast(wo_raw[pl.ds(r0, 128), :], U32)
        return carry

    lax.fori_loop(0, HD // 128, relay_o, 0)

    cp_m.wait()
    cp_r.wait()
    wr = wr_v[...].astype(F32)

    qi = lax.broadcasted_iota(jnp.int32, (32, 48), 0)
    kj = lax.broadcasted_iota(jnp.int32, (32, 48), 1)
    mask_a = (kj < 40) & ((qi < M) | (kj <= qi))
    qi = lax.broadcasted_iota(jnp.int32, (48, 80), 0)
    kj = lax.broadcasted_iota(jnp.int32, (48, 80), 1)
    kb0 = (kj >= 40) & (kj < 48)
    m_mem = (qi < M) & ((kj < 32) | kb0)
    m_xb = (qi >= M) & (qi < 32) & ((kj <= qi) | kb0)
    m_xa = (qi >= 32) & (qi < 40) & ((kj >= 48) | ((kj >= 32) & (kj <= qi)))
    m_b0 = (qi >= 40) & ((kj < M) | (kb0 & (kj <= qi)))
    mask_b = m_mem | m_xb | m_xa | m_b0

    def w_cols(mi, g):
        return pltpu.bitcast(wqkv[mi * NG + g], BF16)

    def wo_rows(g):
        r0 = g * GW // 2
        return pltpu.bitcast(wo[r0:r0 + GW // 2, :], BF16)

    def seg_step(lhs, extra, mask):
        q, k, v, p, o = {}, {}, {}, {}, {}
        acc = [None]

        def proj(mi, g):
            y = _dot(lhs[mi], w_cols(mi, g)).astype(BF16)
            ex = extra(mi, g)
            return jnp.concatenate([y] + ex, axis=0) if ex else y

        def qk(g):
            q[g] = proj(0, g)
            k[g] = proj(1, g)

        def sc(g):
            for j in range(G):
                sl = slice(j * DH, (j + 1) * DH)
                p[g, j] = _softmax_bf16(_dot_nt(q[g][:, sl], k[g][:, sl]), mask)

        def vv(g):
            v[g] = proj(2, g)

        def pv(g):
            o[g] = jnp.concatenate(
                [_dot(p[g, j], v[g][:, j * DH:(j + 1) * DH]) for j in range(G)],
                axis=1).astype(BF16)

        def op(g):
            y = _dot(o[g], wo_rows(g))
            acc[0] = y if acc[0] is None else acc[0] + y

        qk(0)
        for g in range(1, NG):
            qk(g)
            sc(g - 1)
        vv(0)
        sc(NG - 1)
        for g in range(1, NG + 2):
            if g < NG:
                vv(g)
            if g - 1 < NG:
                pv(g - 1)
            if g >= 2:
                op(g - 2)
        return acc[0], (q, k, v)

    sub16 = lax.broadcasted_iota(jnp.int32, (16, 128), 0)

    def post(base, valid):
        rb = rbest[...]
        ib = ibest[...]
        for c in range(PAIR // 16):
            rows = pl.ds(base + c * 16, 16)
            x1 = _rnd(xres[rows, :] + _rnd(obuf[c * 16:(c + 1) * 16, :]))
            ln = _layernorm(x1)
            r = _rnd(jnp.sum(ln * wr, axis=-1, keepdims=True))
            r = jnp.broadcast_to(jnp.where(valid, r, -jnp.inf), (16, 128))
            better = r > rb
            rb = jnp.where(better, r, rb)
            ib = jnp.where(better, sub16 + (base + (c * 16 - PAD)), ib)
            x2 = _rnd(x1 + ln)
            x1buf[rows, :] = x1
            lbuf[rows, :] = ln
            xres[rows, :] = x2
            ostage[rows, :] = x2.astype(BF16)
            hbuf[rows, :] = _layernorm(x2)
        rbest[...] = rb
        ibest[...] = ib

    def out_copy(row0, nrows):
        return pltpu.make_async_copy(ostage.at[pl.ds(PAD + row0, nrows)],
                                     out_hbm.at[pl.ds(row0, nrows)], osem)

    def pair_body(pi, mem, li, light):
        base = pl.multiple_of(pi * PAIR, PAIR)
        hb = hbuf[pl.ds(base + PAD + 40, 24), :]
        if light:
            ha = hbuf[pl.ds(base + PAD, 24), :]
            lhs_a = jnp.concatenate([mem, ha], axis=0).astype(BF16)
            p0 = pl.multiple_of(pi * 8, 8)
            pre_rows = lambda mi, g: pltpu.bitcast(pre[mi * NG + g, pl.ds(p0, 8), :], BF16)
            post(base, pi > 0)
            acc_a, prj = seg_step((lhs_a,) * 3,
                                  lambda mi, g: [pre_rows(mi, g)] if mi else [], mask_a)
            lhs_b = jnp.concatenate([acc_a[0:8], hb], axis=0).astype(BF16)
            lhs_bq = lhs_b
            extra_q = lambda g: [pre_rows(0, g)]
        else:
            ha = hbuf[pl.ds(base + PAD, 40), :]
            lhs_a = jnp.concatenate([mem, ha], axis=0).astype(BF16)
            post(base, pi > 0)
            acc_a, prj = seg_step((lhs_a[0:32], lhs_a, lhs_a), lambda mi, g: [], mask_a)
            lhs_b = jnp.concatenate([acc_a[0:8], hb], axis=0).astype(BF16)
            lhs_bq = jnp.concatenate([lhs_b, lhs_a[32:48]], axis=0)
            extra_q = lambda g: []
        acc_b, _ = seg_step(
            (lhs_bq, lhs_b, lhs_b),
            lambda mi, g: [prj[mi][g][32:48], prj[mi][g][0:32]] if mi else extra_q(g),
            mask_b)
        obuf[0:24, :] = acc_a[8:32]
        obuf[24:40, :] = acc_b[32:48]
        obuf[40:64, :] = acc_b[8:32]

        @pl.when(jnp.logical_and(li == 1, pi > 0))
        def _():
            out_copy(pl.multiple_of(base - PAIR, PAIR), PAIR).start()

        return acc_b[0:8]

    def layer(li, carry):
        obuf[...] = jnp.zeros((PAIR, D), F32)
        rbest[...] = jnp.full((16, 128), -jnp.inf, F32)
        ibest[...] = jnp.zeros((16, 128), jnp.int32)
        mem = mem0_v[...].astype(F32)
        nlight = NPRE * (1 - li)
        if NPRE:
            mem = lax.fori_loop(0, nlight, functools.partial(pair_body, li=li, light=True), mem)
        lax.fori_loop(nlight, NPAIR, functools.partial(pair_body, li=li, light=False), mem)

        @pl.when(li == 0)
        def _():
            for c in cp_mlp:
                c.wait()

        @pl.when(li == 1)
        def _():
            out_copy(0, S - PAIR).wait()

        post(S, True)

        rb = rbest[...]
        rmax = jnp.max(rb, axis=0, keepdims=True)
        idx = jnp.min(jnp.where(rb == rmax, ibest[...], S - 1))
        row = pl.ds(PAD + idx, 1)
        lsel = lbuf[row, :]
        xs = jnp.broadcast_to(lsel, (16, D)).astype(BF16)
        gpre = _rnd(_dot(xs, wg_v[...]))
        gate = _rnd(gpre * _rnd(jax.nn.sigmoid(gpre)))
        up = _rnd(_dot(xs, wu_v[...]))
        y = _rnd(_dot((gate * up).astype(BF16), wd_v[...]))[0:1]
        rsel = _rnd(jax.nn.sigmoid(rmax[:, 0:1]))
        y = _rnd(y * rsel)
        x2 = _rnd(x1buf[row, :] + _rnd(lsel + y))
        xres[row, :] = x2
        hbuf[row, :] = _layernorm(x2)

        @pl.when(li == 1)
        def _():
            t0 = pl.multiple_of((idx // 16) * 16, 16)
            ostage[pl.ds(PAD + t0, 16), :] = xres[pl.ds(PAD + t0, 16), :].astype(BF16)
            t1 = pl.multiple_of(jnp.minimum(t0, S - PAIR - 16), 16)
            out_copy(S - PAIR, PAIR).start()
            out_copy(t1, 16).start()
            out_copy(0, PAIR + 16).wait()

        return carry

    lax.fori_loop(0, 2, layer, 0)


CFG = dict(G=4, NPRE=15)


def _build():
    G, NPRE = CFG['G'], CFG['NPRE']
    any_spec = pl.BlockSpec(memory_space=pl.ANY)
    return pl.pallas_call(
        functools.partial(_kernel, **CFG),
        out_shape=jax.ShapeDtypeStruct((S, D), BF16),
        in_specs=[any_spec] * 10,
        out_specs=any_spec,
        scratch_shapes=[
            pltpu.VMEM((S, D), BF16),
            pltpu.VMEM((M, D), BF16),
            pltpu.VMEM((1, D), BF16),
            pltpu.VMEM((6, D, 16, DH), BF16),
            pltpu.VMEM((HD, D), BF16),
            pltpu.VMEM((D, FF), BF16),
            pltpu.VMEM((D, FF), BF16),
            pltpu.VMEM((FF, D), BF16),
            pltpu.VMEM((3 * H // G, D // 2, G * DH), U32),
            pltpu.VMEM((HD // 2, D), U32),
            pltpu.VMEM((4 * 160, DH), U32),
            pltpu.VMEM((PAD + S, D), F32),
            pltpu.VMEM((PAD + S, D), F32),
            pltpu.VMEM((PAD + S, D), F32),
            pltpu.VMEM((PAD + S, D), F32),
            pltpu.VMEM((16, 128), F32),
            pltpu.VMEM((16, 128), jnp.int32),
            pltpu.VMEM((PAIR, D), F32),
            pltpu.VMEM((PAD + S, D), BF16),
            pltpu.VMEM((8 * max(NPRE, 1), D), U32),
            pltpu.VMEM((3 * H // G, 8 * max(NPRE, 1), G * DH), U32),
            pltpu.SemaphoreType.DMA((13,)),
            pltpu.SemaphoreType.DMA(()),
        ],
        compiler_params=pltpu.CompilerParams(vmem_limit_bytes=110 * 1024 * 1024),
    )


@functools.partial(jax.jit, static_argnames=("A_seg_len",))
def pallas_interleave_layers__memory_aug_recurrent_mem_tr__moe_arch_mod__prompt_kernel(
    A_x: jax.Array,
    A_mem0: jax.Array,
    A_Wq: jax.Array,
    A_Wk: jax.Array,
    A_Wv: jax.Array,
    A_Wo: jax.Array,
    A_seg_len,
    B_x: jax.Array,
    B_w_r: jax.Array,
    B_w_gate: jax.Array,
    B_w_up: jax.Array,
    B_w_down: jax.Array,
):
    assert A_seg_len == SEG and A_x.shape == (1, S, D)
    del B_x
    out = _build()(
        A_x.reshape(S, D),
        A_mem0.reshape(M, D),
        A_Wq,
        A_Wk,
        A_Wv,
        A_Wo.reshape(HD, D),
        B_w_r.reshape(1, D),
        B_w_gate,
        B_w_up,
        B_w_down,
    )
    return out.reshape(1, S, D)
```

```python
import functools
import math

import jax
import jax.numpy as jnp
from jax import lax
import jax.experimental.pallas as pl
import jax.experimental.pallas.tpu as pltpu

F32 = jnp.float32
BF16 = jnp.bfloat16
U32 = jnp.uint32

S, D, H, DH, M, SEG = 2048, 512, 32, 128, 8, 32
FF = 1792
HD = H * DH
PAIR = 2 * SEG
NPAIR = S // PAIR
PAD = PAIR
LN_EPS = 1e-05
NEG = -1000000000.0
EXP2_SCALE = (DH ** -0.5) * math.log2(math.e)


def _rnd(x):
    return x.astype(BF16).astype(F32)


def _layernorm(x):
    mean = jnp.sum(x, axis=-1, keepdims=True) * (1.0 / D)
    c = x - mean
    var = jnp.sum(c * c, axis=-1, keepdims=True) * (1.0 / D)
    den = _rnd(jnp.sqrt(_rnd(_rnd(var) + _rnd(jnp.float32(LN_EPS)))))
    inv = 1.0 / den
    return _rnd(_rnd(x - _rnd(mean)) * inv)


def _dot(a, b):
    return jnp.dot(a, b, preferred_element_type=F32)


def _dot_nt(a, b):
    return lax.dot_general(a, b, (((1,), (1,)), ((), ())), preferred_element_type=F32)


def _softmax_bf16(s, mask):
    s = jnp.where(mask, s, NEG)
    m = jnp.max(s, axis=-1, keepdims=True)
    e = jnp.exp2((s - m) * EXP2_SCALE)
    l = jnp.sum(e, axis=-1, keepdims=True)
    r = pl.reciprocal(l, approx=True)
    r = r * (2.0 - l * r)
    return (e * r).astype(BF16)


def _kernel(x_hbm, mem0_hbm, wq_hbm, wk_hbm, wv_hbm, wo_hbm, wr_hbm, wg_hbm, wu_hbm, wd_hbm,
            out_hbm,
            x_raw, mem0_v, wr_v, stage, wo_raw, wg_v, wu_v, wd_v,
            wqkv, wo, tmp, xres, x1buf, lbuf, hbuf, rbest, ibest, obuf, ostage,
            lhs_pre, pre, sems, osem, *, G, NPRE, KSPLIT, UNROLL):
    NG = H // G
    GW = G * DH
    HC = 16
    GPC = HC // G
    NCH = 3 * H // HC

    cp_x = pltpu.make_async_copy(x_hbm, x_raw, sems.at[0])
    cp_m = pltpu.make_async_copy(mem0_hbm, mem0_v, sems.at[1])
    cp_r = pltpu.make_async_copy(wr_hbm, wr_v, sems.at[2])
    cp_o = pltpu.make_async_copy(wo_hbm, wo_raw, sems.at[3])
    cp_mlp = [pltpu.make_async_copy(s_, d_, sems.at[4 + i])
              for i, (s_, d_) in enumerate(((wg_hbm, wg_v), (wu_hbm, wu_v), (wd_hbm, wd_v)))]
    cp_x.start()
    for c in range(NCH):
        w = (wq_hbm, wk_hbm, wv_hbm)[c // 2]
        pltpu.make_async_copy(w.at[:, pl.ds((c % 2) * HC, HC), :], stage.at[c],
                              sems.at[7 + c]).start()
    cp_o.start()
    cp_m.start()
    cp_r.start()
    for c in cp_mlp:
        c.start()

    xres[0:PAD, :] = jnp.zeros((PAD, D), F32)
    cp_x.wait()

    def ln0(i, carry):
        for c in range(8):
            r0 = pl.multiple_of(i * 128 + c * 16, 16)
            xv = x_raw[pl.ds(r0, 16), :].astype(F32)
            xres[pl.ds(PAD + r0, 16), :] = xv
            hbuf[pl.ds(PAD + r0, 16), :] = _layernorm(xv)
        return carry

    lax.fori_loop(0, S // 128, ln0, 0)

    for p_ in range(NPRE):
        r0 = PAD + p_ * PAIR + 24
        lhs_pre[p_ * 8:(p_ + 1) * 8, :] = pltpu.bitcast(hbuf[r0:r0 + 16, :].astype(BF16), U32)

    TP = 20
    TSZ = 8 * TP

    def chunk(c, carry):
        pltpu.make_async_copy(wq_hbm.at[:, pl.ds(0, HC), :], stage.at[c], sems.at[7 + c]).wait()

        def relay(it, carry2):
            for u in range(4):
                d0 = pl.multiple_of(it * 64 + u * 16, 16)
                raw = pltpu.bitcast(stage[c, pl.ds(d0, 16), :, :], U32)
                for i in range(8):
                    ev, od = raw[2 * i], raw[2 * i + 1]
                    lo = (ev & jnp.uint32(0xFFFF)) | (od << 16)
                    hi = (ev >> 16) | (od & jnp.uint32(0xFFFF0000))
                    tmp[pl.ds(u * TSZ + i * TP, 8, stride=2), :] = lo
                    tmp[pl.ds(u * TSZ + i * TP + 1, 8, stride=2), :] = hi
            for u in range(4):
                o0 = pl.multiple_of(it * 32 + u * 8, 8)
                for hh in range(HC):
                    t = tmp[pl.ds(u * TSZ + hh, 8, stride=TP), :]
                    col = (hh % G) * DH
                    wqkv[c * GPC + hh // G, pl.ds(o0, 8), col:col + DH] = t
            return carry2

        lax.fori_loop(0, D // 64, relay, 0)
        if NPRE:
            lhs = pltpu.bitcast(lhs_pre[...], BF16)
            for gg in range(GPC):
                pre[c * GPC + gg] = _dot(lhs, pltpu.bitcast(wqkv[c * GPC + gg], BF16))
        return carry

    lax.fori_loop(0, NCH, chunk, 0)

    cp_o.wait()

    def relay_o(c, carry):
        r0 = pl.multiple_of(c * 128, 128)
        o0 = pl.multiple_of(c * 64, 64)
        wo[pl.ds(o0, 64), :] = pltpu.bitcast(wo_raw[pl.ds(r0, 128), :], U32)
        return carry

    lax.fori_loop(0, HD // 128, relay_o, 0)

    cp_m.wait()
    cp_r.wait()
    wr = wr_v[...].astype(F32)

    qi = lax.broadcasted_iota(jnp.int32, (32, 48), 0)
    kj = lax.broadcasted_iota(jnp.int32, (32, 48), 1)
    mask_a = (kj < 40) & ((qi < M) | (kj <= qi))
    qi = lax.broadcasted_iota(jnp.int32, (48, 80), 0)
    kj = lax.broadcasted_iota(jnp.int32, (48, 80), 1)
    kb0 = (kj >= 40) & (kj < 48)
    m_mem = (qi < M) & ((kj < 32) | kb0)
    m_xb = (qi >= M) & (qi < 32) & ((kj <= qi) | kb0)
    m_xa = (qi >= 32) & (qi < 40) & ((kj >= 48) | ((kj >= 32) & (kj <= qi)))
    m_b0 = (qi >= 40) & ((kj < M) | (kb0 & (kj <= qi)))
    mask_b = m_mem | m_xb | m_xa | m_b0

    def w_cols(mi, g):
        return pltpu.bitcast(wqkv[mi * NG + g], BF16)

    def wo_rows(g):
        r0 = g * GW // 2
        return pltpu.bitcast(wo[r0:r0 + GW // 2, :], BF16)

    def seg_step(lhs, lhs_f32, extra, mask):
        q, k, v, p, o = {}, {}, {}, {}, {}
        raw = ({}, {}, {})
        acc = [None]

        def proj(mi, g, dst):
            if KSPLIT and mi == 0 and g == 0:
                y = None
                lp = jnp.concatenate([lhs_f32[16:], lhs_f32[0:16]], axis=0)
                for kt in range(D // 128):
                    w = pltpu.bitcast(wqkv[0, kt * 64:(kt + 1) * 64, :], BF16)
                    t = _dot(lp[:, kt * 128:(kt + 1) * 128].astype(BF16), w)
                    y = t if y is None else y + t
                nr = y.shape[0]
                y = jnp.concatenate([y[nr - 16:], y[0:nr - 16]], axis=0)
            else:
                y = _dot(lhs[mi], w_cols(mi, g))
            for j in range(G):
                h = g * G + j
                yh = y[:, j * DH:(j + 1) * DH]
                ex = extra(mi, h)
                if ex:
                    yh = jnp.concatenate([yh] + ex, axis=0)
                raw[mi][h] = yh
                dst[h] = yh.astype(BF16)

        def qk(g):
            proj(0, g, q)
            proj(1, g, k)

        def sc(g):
            for h in range(g * G, (g + 1) * G):
                p[h] = _softmax_bf16(_dot_nt(q[h], k[h]), mask)

        def vv(g):
            proj(2, g, v)

        def pv(g):
            o[g] = jnp.concatenate(
                [_dot(p[h], v[h]) for h in range(g * G, (g + 1) * G)], axis=1).astype(BF16)

        def op(g):
            y = _dot(o[g], wo_rows(g))
            acc[0] = y if acc[0] is None else acc[0] + y

        qk(0)
        for g in range(1, NG):
            qk(g)
            sc(g - 1)
        vv(0)
        sc(NG - 1)
        for g in range(1, NG + 2):
            if g < NG:
                vv(g)
            if g - 1 < NG:
                pv(g - 1)
            if g >= 2:
                op(g - 2)
        return acc[0], raw

    sub16 = lax.broadcasted_iota(jnp.int32, (16, 128), 0)

    def post(base, valid):
        rb = rbest[...]
        ib = ibest[...]
        for c in range(PAIR // 16):
            rows = pl.ds(base + c * 16, 16)
            x1 = _rnd(xres[rows, :] + _rnd(obuf[c * 16:(c + 1) * 16, :]))
            ln = _layernorm(x1)
            r = _rnd(jnp.sum(ln * wr, axis=-1, keepdims=True))
            r = jnp.broadcast_to(jnp.where(valid, r, -jnp.inf), (16, 128))
            better = r > rb
            rb = jnp.where(better, r, rb)
            ib = jnp.where(better, sub16 + (base + (c * 16 - PAD)), ib)
            x2 = _rnd(x1 + ln)
            x1buf[rows, :] = x1
            lbuf[rows, :] = ln
            xres[rows, :] = x2
            ostage[rows, :] = x2.astype(BF16)
            hbuf[rows, :] = _layernorm(x2)
        rbest[...] = rb
        ibest[...] = ib

    def out_copy(row0, nrows):
        return pltpu.make_async_copy(ostage.at[pl.ds(PAD + row0, nrows)],
                                     out_hbm.at[pl.ds(row0, nrows)], osem)

    def pair_body(pi, mem, light):
        base = pl.multiple_of(pi * PAIR, PAIR)
        hb = hbuf[pl.ds(base + PAD + 40, 24), :]
        if light:
            ha = hbuf[pl.ds(base + PAD, 24), :]
            aq = jnp.concatenate([mem, ha], axis=0)
            lhs_a = aq.astype(BF16)
            p0 = pl.multiple_of(pi * 16, 16)
            pre_rows = lambda mi, h: pre[mi * NG + h // G, pl.ds(p0, 16),
                                         (h % G) * DH:(h % G + 1) * DH]
            post(base, pi > 0)
            acc_a, prj = seg_step((lhs_a,) * 3, aq,
                                  lambda mi, g: [pre_rows(mi, g)] if mi else [], mask_a)
            bq = jnp.concatenate([acc_a[0:8], hb], axis=0)
            lhs_b = bq.astype(BF16)
            lhs_bq = lhs_b
            extra_q = lambda g: [pre_rows(0, g)]
        else:
            ha = hbuf[pl.ds(base + PAD, 40), :]
            lhs_a = jnp.concatenate([mem, ha], axis=0).astype(BF16)
            aq = jnp.concatenate([mem, ha[0:24]], axis=0)
            post(base, pi > 0)
            acc_a, prj = seg_step((aq.astype(BF16), lhs_a, lhs_a), aq, lambda mi, g: [], mask_a)
            lhs_b = jnp.concatenate([acc_a[0:8], hb], axis=0).astype(BF16)
            bq = jnp.concatenate([acc_a[0:8], hb, ha[24:40]], axis=0)
            lhs_bq = bq.astype(BF16)
            extra_q = lambda g: []
        acc_b, _ = seg_step(
            (lhs_bq, lhs_b, lhs_b), bq,
            lambda mi, g: [prj[mi][g][32:48], prj[mi][g][0:32]] if mi else extra_q(g),
            mask_b)
        obuf[0:24, :] = acc_a[8:32]
        obuf[24:40, :] = acc_b[32:48]
        obuf[40:64, :] = acc_b[8:32]

        return acc_b[0:8]

    def loop_body(it, mem, li, light):
        for u in range(UNROLL):
            mem = pair_body(it * UNROLL + u, mem, light)

        @pl.when(jnp.logical_and(li == 1, it > 0))
        def _():
            out_copy(pl.multiple_of(it * (UNROLL * PAIR) - PAIR, PAIR), UNROLL * PAIR).start()

        if UNROLL > 1:
            @pl.when(jnp.logical_and(li == 1, it == 0))
            def _():
                out_copy(0, (UNROLL - 1) * PAIR).start()

        return mem

    def layer(li, carry):
        obuf[...] = jnp.zeros((PAIR, D), F32)
        rbest[...] = jnp.full((16, 128), -jnp.inf, F32)
        ibest[...] = jnp.zeros((16, 128), jnp.int32)
        mem = mem0_v[...].astype(F32)
        nlight = (NPRE // UNROLL) * (1 - li)
        if NPRE:
            mem = lax.fori_loop(0, nlight, functools.partial(loop_body, li=li, light=True), mem)
        lax.fori_loop(nlight, NPAIR // UNROLL,
                      functools.partial(loop_body, li=li, light=False), mem)

        @pl.when(li == 0)
        def _():
            for c in cp_mlp:
                c.wait()

        @pl.when(li == 1)
        def _():
            out_copy(0, S - PAIR).wait()

        post(S, True)

        rb = rbest[...]
        rmax = jnp.max(rb, axis=0, keepdims=True)
        idx = jnp.min(jnp.where(rb == rmax, ibest[...], S - 1))
        row = pl.ds(PAD + idx, 1)
        lsel = lbuf[row, :]
        xs = jnp.broadcast_to(lsel, (16, D)).astype(BF16)
        gpre = _rnd(_dot(xs, wg_v[...]))
        gate = _rnd(gpre * _rnd(jax.nn.sigmoid(gpre)))
        up = _rnd(_dot(xs, wu_v[...]))
        y = _rnd(_dot((gate * up).astype(BF16), wd_v[...]))[0:1]
        rsel = _rnd(jax.nn.sigmoid(rmax[:, 0:1]))
        y = _rnd(y * rsel)
        x2 = _rnd(x1buf[row, :] + _rnd(lsel + y))
        xres[row, :] = x2
        hbuf[row, :] = _layernorm(x2)

        @pl.when(li == 1)
        def _():
            t0 = pl.multiple_of((idx // 16) * 16, 16)
            ostage[pl.ds(PAD + t0, 16), :] = xres[pl.ds(PAD + t0, 16), :].astype(BF16)
            t1 = pl.multiple_of(jnp.minimum(t0, S - PAIR - 16), 16)
            out_copy(S - PAIR, PAIR).start()
            out_copy(t1, 16).start()
            out_copy(0, PAIR + 16).wait()

        return carry

    lax.fori_loop(0, 2, layer, 0)


CFG = dict(G=4, NPRE=14, KSPLIT=True, UNROLL=2)


def _build():
    G, NPRE = CFG['G'], CFG['NPRE']
    any_spec = pl.BlockSpec(memory_space=pl.ANY)
    return pl.pallas_call(
        functools.partial(_kernel, **CFG),
        out_shape=jax.ShapeDtypeStruct((S, D), BF16),
        in_specs=[any_spec] * 10,
        out_specs=any_spec,
        scratch_shapes=[
            pltpu.VMEM((S, D), BF16),
            pltpu.VMEM((M, D), BF16),
            pltpu.VMEM((1, D), BF16),
            pltpu.VMEM((6, D, 16, DH), BF16),
            pltpu.VMEM((HD, D), BF16),
            pltpu.VMEM((D, FF), BF16),
            pltpu.VMEM((D, FF), BF16),
            pltpu.VMEM((FF, D), BF16),
            pltpu.VMEM((3 * H // G, D // 2, G * DH), U32),
            pltpu.VMEM((HD // 2, D), U32),
            pltpu.VMEM((4 * 160, DH), U32),
            pltpu.VMEM((PAD + S, D), F32),
            pltpu.VMEM((PAD + S, D), F32),
            pltpu.VMEM((PAD + S, D), F32),
            pltpu.VMEM((PAD + S, D), F32),
            pltpu.VMEM((16, 128), F32),
            pltpu.VMEM((16, 128), jnp.int32),
            pltpu.VMEM((PAIR, D), F32),
            pltpu.VMEM((PAD + S, D), BF16),
            pltpu.VMEM((8 * max(NPRE, 1), D), U32),
            pltpu.VMEM((3 * H // G, 16 * max(NPRE, 1), G * DH), F32),
            pltpu.SemaphoreType.DMA((13,)),
            pltpu.SemaphoreType.DMA(()),
        ],
        compiler_params=pltpu.CompilerParams(vmem_limit_bytes=110 * 1024 * 1024),
    )


@functools.partial(jax.jit, static_argnames=("A_seg_len",))
def pallas_interleave_layers__memory_aug_recurrent_mem_tr__moe_arch_mod__prompt_kernel(
    A_x: jax.Array,
    A_mem0: jax.Array,
    A_Wq: jax.Array,
    A_Wk: jax.Array,
    A_Wv: jax.Array,
    A_Wo: jax.Array,
    A_seg_len,
    B_x: jax.Array,
    B_w_r: jax.Array,
    B_w_gate: jax.Array,
    B_w_up: jax.Array,
    B_w_down: jax.Array,
):
    assert A_seg_len == SEG and A_x.shape == (1, S, D)
    del B_x
    out = _build()(
        A_x.reshape(S, D),
        A_mem0.reshape(M, D),
        A_Wq,
        A_Wk,
        A_Wv,
        A_Wo.reshape(HD, D),
        B_w_r.reshape(1, D),
        B_w_gate,
        B_w_up,
        B_w_down,
    )
    return out.reshape(1, S, D)
```

```python
import functools
import math

import jax
import jax.numpy as jnp
from jax import lax
import jax.experimental.pallas as pl
import jax.experimental.pallas.tpu as pltpu

F32 = jnp.float32
BF16 = jnp.bfloat16
U32 = jnp.uint32

S, D, H, DH, M, SEG = 2048, 512, 32, 128, 8, 32
FF = 1792
HD = H * DH
PAIR = 2 * SEG
NPAIR = S // PAIR
PAD = PAIR
G = 4
NG = H // G
GW = G * DH
HC = 16
GPC = HC // G
NCH = 3 * H // HC
TP = 20
TSZ = 8 * TP
NTMP = 8
RC = 8
LN_EPS = 1e-05
NEG = -1000000000.0
EXP2_SCALE = (DH ** -0.5) * math.log2(math.e)


def _rnd(x):
    return x.astype(BF16).astype(F32)


def _layernorm(x):
    mean = jnp.sum(x, axis=-1, keepdims=True) * (1.0 / D)
    c = x - mean
    var = jnp.sum(c * c, axis=-1, keepdims=True) * (1.0 / D)
    den = _rnd(jnp.sqrt(_rnd(_rnd(var) + _rnd(jnp.float32(LN_EPS)))))
    inv = 1.0 / den
    return _rnd(_rnd(x - _rnd(mean)) * inv)


def _dot(a, b):
    return jnp.dot(a, b, preferred_element_type=F32)


def _dot_nt(a, b):
    return lax.dot_general(a, b, (((1,), (1,)), ((), ())), preferred_element_type=F32)


def _softmax_bf16(s, mask):
    s = jnp.where(mask, s, NEG)
    m = jnp.max(s, axis=-1, keepdims=True)
    e = jnp.exp2((s - m) * EXP2_SCALE)
    l = jnp.sum(e, axis=-1, keepdims=True)
    r = pl.reciprocal(l, approx=True)
    r = r * (2.0 - l * r)
    return (e * r).astype(BF16)


def _kernel(x_hbm, mem0_hbm, wq_hbm, wk_hbm, wv_hbm, wo_hbm, wr_hbm, wg_hbm, wu_hbm, wd_hbm,
            out_hbm,
            x_raw, mem0_v, wr_v, stage, wo_raw, wg_v, wu_v, wd_v,
            wk0, wk1, wv0, wv1, wq0, wq1, wo, tmp,
            xres, x1buf, lbuf, hbuf, rbest, ibest, obuf, ostage,
            lhs_pre, pre, anchor, sems, osem, *,
            UNROLL, LAGA, LAGB, FILL, SMID, LNROWS):
    wch = (wk0, wk1, wv0, wv1, wq0, wq1)
    NXP = 4
    XP = S // NXP
    SEM_X, SEM_W, SEM_O, SEM_MISC = 0, NXP, NXP + NCH, NXP + NCH + 2

    def cp_x(i):
        return pltpu.make_async_copy(x_hbm.at[pl.ds(i * XP, XP)],
                                     x_raw.at[pl.ds(PAD + i * XP, XP)], sems.at[SEM_X + i])

    def cp_w(c):
        w = (wk_hbm, wv_hbm, wq_hbm)[c // 2]
        return pltpu.make_async_copy(w.at[:, pl.ds((c % 2) * HC, HC), :], stage.at[c],
                                     sems.at[SEM_W + c])

    def cp_o(i):
        return pltpu.make_async_copy(wo_hbm.at[pl.ds(i * (HD // 2), HD // 2)],
                                     wo_raw.at[pl.ds(i * (HD // 2), HD // 2)],
                                     sems.at[SEM_O + i])

    cp_small = [pltpu.make_async_copy(s_, d_, sems.at[SEM_MISC + i])
                for i, (s_, d_) in enumerate(((mem0_hbm, mem0_v), (wr_hbm, wr_v)))]
    cp_mlp = [pltpu.make_async_copy(s_, d_, sems.at[SEM_MISC + 2 + i])
              for i, (s_, d_) in enumerate(((wg_hbm, wg_v), (wu_hbm, wu_v), (wd_hbm, wd_v)))]
    for i in range(NXP):
        cp_x(i).start()
    for c in range(NCH):
        cp_w(c).start()
    for i in range(2):
        cp_o(i).start()
    for c in cp_small + cp_mlp:
        c.start()

    anchor[0] = PAIR
    x_raw[0:PAD, :] = jnp.zeros((PAD, D), BF16)
    xres[0:PAD, :] = jnp.zeros((PAD, D), F32)

    def ln0(i, carry):
        @pl.when(i % (XP // LNROWS) == 0)
        def _():
            cp_x(i // (XP // LNROWS)).wait()

        for pp in range(LNROWS // PAIR):
            r0 = pl.multiple_of(PAD + i * LNROWS + pp * PAIR, PAIR)
            ln = []
            for c in range(PAIR // 16):
                ln.append(_layernorm(x_raw[pl.ds(r0 + c * 16, 16), :].astype(F32)))
                hbuf[pl.ds(r0 + c * 16, 16), :] = ln[c]
            mid = jnp.concatenate([ln[1][8:16], ln[2][0:8]], axis=0).astype(BF16)
            p0 = pl.multiple_of((i * (LNROWS // PAIR) + pp) * 8, 8)
            lhs_pre[pl.ds(p0, 8), :] = pltpu.bitcast(mid, U32)
        return carry

    lax.fori_loop(0, S // LNROWS, ln0, 0)

    def relayout(c, blk0, nblk, slot0=0):
        def scatter(u):
            t0 = ((slot0 + u) % NTMP) * TSZ
            d0 = pl.multiple_of((blk0 + u) * 16, 16)
            raw = pltpu.bitcast(stage[c, pl.ds(d0, 16), :, :], U32)
            for i in range(8):
                ev, od = raw[2 * i], raw[2 * i + 1]
                lo = (ev & jnp.uint32(0xFFFF)) | (od << 16)
                hi = (ev >> 16) | (od & jnp.uint32(0xFFFF0000))
                tmp[pl.ds(t0 + i * TP, 8, stride=2), :] = lo
                tmp[pl.ds(t0 + i * TP + 1, 8, stride=2), :] = hi

        def gather(u):
            t0 = ((slot0 + u) % NTMP) * TSZ
            o0 = pl.multiple_of((blk0 + u) * 8, 8)
            for hh in range(HC):
                col = (hh % G) * DH
                wch[c][hh // G, pl.ds(o0, 8), col:col + DH] = tmp[pl.ds(t0 + hh, 8, stride=TP), :]

        scatter(0)
        for u in range(nblk):
            if u + 1 < nblk:
                scatter(u + 1)
            gather(u)

    def repack_wo(half):
        for c in range(HD // 2 // 128):
            r0 = pl.multiple_of(half * (HD // 2) + c * 128, 128)
            o0 = pl.multiple_of(half * (HD // 4) + c * 64, 64)
            wo[pl.ds(o0, 64), :] = pltpu.bitcast(wo_raw[pl.ds(r0, 128), :], U32)

    def precompute(c, it):
        lhs = pltpu.bitcast(lhs_pre[...], BF16)
        for gg in range(2):
            pre[c * GPC + it * 2 + gg] = _dot(lhs, pltpu.bitcast(wch[c][it * 2 + gg], BF16))

    NBLK = D // 16
    cp_w(0).wait()
    lax.fori_loop(0, NBLK // 8, lambda it, cr: (relayout(0, it * 8, 8), cr)[1], 0)
    precompute(0, 0)
    cp_w(1).wait()
    precompute(0, 1)
    relayout(1, 0, NBLK)

    def phase(c, chunks, with_wo):
        for cc in chunks:
            cp_w(cc).wait()

        def body(it, carry):
            if with_wo:
                cp_o(it).wait()
            precompute(c, it)
            for n, cc in enumerate(chunks):
                relayout(cc, it * (NBLK // 2), NBLK // 2, n * (NTMP // 2))
            if with_wo:
                repack_wo(it)
            return carry

        lax.fori_loop(0, 2, body, 0)

    phase(1, (2,), False)
    phase(2, (3, 4), False)
    phase(3, (5,), True)

    for c in cp_small:
        c.wait()
    wr = wr_v[...].astype(F32)

    qi = lax.broadcasted_iota(jnp.int32, (32, 48), 0)
    kj = lax.broadcasted_iota(jnp.int32, (32, 48), 1)
    mask_a = (kj < 40) & ((qi < M) | (kj <= qi))
    qi = lax.broadcasted_iota(jnp.int32, (48, 80), 0)
    kj = lax.broadcasted_iota(jnp.int32, (48, 80), 1)
    kb0 = (kj >= 40) & (kj < 48)
    m_mem = (qi < M) & ((kj < 32) | kb0)
    m_xb = (qi >= M) & (qi < 32) & ((kj <= qi) | kb0)
    m_xa = (qi >= 32) & (qi < 40) & ((kj >= 48) | ((kj >= 32) & (kj <= qi)))
    m_b0 = (qi >= 40) & ((kj < M) | (kb0 & (kj <= qi)))
    mask_b = m_mem | m_xb | m_xa | m_b0

    def w_ref(mi, g):
        return wch[(4, 0, 2)[mi] + g // GPC].at[g % GPC]

    def wo_rows(g):
        r0 = g * GW // 2
        return pltpu.bitcast(wo[r0:r0 + GW // 2, :], BF16)

    def seg_step(lhs, lhs_f32, extra, mask, lags, s_mid, filler):
        q, k, v, p, o = {}, {}, {}, {}, {}
        raw = ({}, {}, {})
        acc = [None]

        def proj(mi, g, dst):
            if mi == 0 and g == 0:
                y = None
                lp = jnp.concatenate([lhs_f32[16:], lhs_f32[0:16]], axis=0)
                for kt in range(D // 128):
                    w = pltpu.bitcast(w_ref(0, 0)[kt * 64:(kt + 1) * 64, :], BF16)
                    t = _dot(lp[:, kt * 128:(kt + 1) * 128].astype(BF16), w)
                    y = t if y is None else y + t
                nr = y.shape[0]
                y = jnp.concatenate([y[nr - 16:], y[0:nr - 16]], axis=0)
            else:
                y = _dot(lhs[mi], pltpu.bitcast(w_ref(mi, g)[...], BF16))
            for j in range(G):
                h = g * G + j
                yh = y[:, j * DH:(j + 1) * DH]
                ex = extra(mi, h)
                if ex:
                    yh = jnp.concatenate([yh] + ex, axis=0)
                raw[mi][h] = yh
                dst[h] = yh.astype(BF16)

        def sc(g):
            for h in range(g * G, (g + 1) * G):
                p[h] = _softmax_bf16(_dot_nt(q[h], k[h]), mask)

        def pv(g):
            o[g] = jnp.concatenate(
                [_dot(p[h], v[h]) for h in range(g * G, (g + 1) * G)], axis=1).astype(BF16)

        def op(g):
            y = _dot(o[g], wo_rows(g))
            acc[0] = y if acc[0] is None else acc[0] + y

        ls, lp, lo = lags
        for t in range(2 * NG + lp + lo):
            if t < NG:
                proj(0, t, q)
                if s_mid and 0 <= t - ls < NG:
                    sc(t - ls)
                proj(1, t, k)
            elif t < 2 * NG:
                proj(2, t - NG, v)
            if 0 <= t - ls < NG and not s_mid:
                sc(t - ls)
            if 0 <= t - NG - lp < NG:
                pv(t - NG - lp)
            if s_mid and t == NG + lp:
                for g in range(NG - ls, NG):
                    sc(g)
            if 0 <= t - NG - lp - lo < NG:
                op(t - NG - lp - lo)
            if t in filler:
                src = raw[1][t * G] if t < NG else raw[2][min(t - NG, NG - 1) * G]
                filler[t](src[0:8])
        return acc[0], raw

    subr = lax.broadcasted_iota(jnp.int32, (RC, 128), 0)

    def post_chunk(li, base, valid, c, tie=None):
        if tie is not None:
            obuf[pl.ds(pl.multiple_of(anchor[0], 8), 8), 0:DH] = tie
        rows = pl.ds(base + c * RC, RC)
        x0 = x_raw[rows, :].astype(F32) if li == 0 else xres[rows, :]
        x1 = _rnd(x0 + _rnd(obuf[c * RC:(c + 1) * RC, :]))
        ln = _layernorm(x1)
        r = _rnd(jnp.sum(ln * wr, axis=-1, keepdims=True))
        r = jnp.broadcast_to(jnp.where(valid, r, -jnp.inf), (RC, 128))
        rb = rbest[...]
        better = r > rb
        rbest[...] = jnp.where(better, r, rb)
        ibest[...] = jnp.where(better, subr + (base + (c * RC - PAD)), ibest[...])
        x1buf[rows, :] = x1
        lbuf[rows, :] = ln
        if li == 0:
            x2 = _rnd(x1 + ln)
            xres[rows, :] = x2
            hbuf[rows, :] = _layernorm(x2)
        else:
            ostage[rows, :] = (x1 + ln).astype(BF16)

    def out_copy(row0, nrows):
        return pltpu.make_async_copy(ostage.at[pl.ds(PAD + row0, nrows)],
                                     out_hbm.at[pl.ds(row0, nrows)], osem)

    def pair_body(li, pi, mem):
        base = pl.multiple_of(pi * PAIR, PAIR)
        ha = hbuf[pl.ds(base + PAD, 40), :]
        hb = hbuf[pl.ds(base + PAD + 40, 24), :]
        fill = ({}, {})
        for c, (st, t) in enumerate(FILL[li]):
            fill[st][t] = functools.partial(post_chunk, li, base, pi > 0, c)
        aq = jnp.concatenate([mem, ha[0:24]], axis=0)
        lhs_aq = aq.astype(BF16)
        if li == 0:
            p0 = pl.multiple_of(pi * 16, 16)
            lhs_akv = lhs_aq
            extra_a = lambda mi, h: [pre[(mi - 1) * NG + h // G, pl.ds(p0, 16),
                                         (h % G) * DH:(h % G + 1) * DH]] if mi else []
        else:
            lhs_akv = jnp.concatenate([mem, ha], axis=0).astype(BF16)
            extra_a = lambda mi, h: []
        acc_a, prj = seg_step((lhs_aq, lhs_akv, lhs_akv), aq, extra_a, mask_a,
                              LAGA, SMID[0], fill[0])
        lhs_b = jnp.concatenate([acc_a[0:8], hb], axis=0).astype(BF16)
        bq = jnp.concatenate([acc_a[0:8], hb, ha[24:40]], axis=0)
        acc_b, _ = seg_step(
            (bq.astype(BF16), lhs_b, lhs_b), bq,
            lambda mi, h: [prj[mi][h][32:48], prj[mi][h][0:32]] if mi else [],
            mask_b, LAGB, SMID[1], fill[1])
        obuf[0:24, :] = acc_a[8:32]
        obuf[24:40, :] = acc_b[32:48]
        obuf[40:64, :] = acc_b[8:32]
        return acc_b[0:8]

    def loop_body(li, it, mem):
        for u in range(UNROLL):
            mem = pair_body(li, it * UNROLL + u, mem)

        if li == 1:
            @pl.when(it > 0)
            def _():
                out_copy(pl.multiple_of(it * (UNROLL * PAIR) - PAIR, PAIR),
                         UNROLL * PAIR).start()

            if UNROLL > 1:
                @pl.when(it == 0)
                def _():
                    out_copy(0, (UNROLL - 1) * PAIR).start()

        return mem

    for li in range(2):
        obuf[0:PAIR, :] = jnp.zeros((PAIR, D), F32)
        rbest[...] = jnp.full((RC, 128), -jnp.inf, F32)
        ibest[...] = jnp.zeros((RC, 128), jnp.int32)
        lax.fori_loop(0, NPAIR // UNROLL, functools.partial(loop_body, li),
                      mem0_v[...].astype(F32))

        if li == 0:
            for c in cp_mlp:
                c.wait()
        else:
            out_copy(0, S - PAIR).wait()

        for c in range(PAIR // RC):
            post_chunk(li, S, True, c)

        rb = rbest[...]
        rmax = jnp.max(rb, axis=0, keepdims=True)
        idx = jnp.min(jnp.where(rb == rmax, ibest[...], S - 1))
        row = pl.ds(PAD + idx, 1)
        lsel = lbuf[row, :]
        xs = jnp.broadcast_to(lsel, (16, D)).astype(BF16)
        gpre = _rnd(_dot(xs, wg_v[...]))
        gate = _rnd(gpre * _rnd(jax.nn.sigmoid(gpre)))
        up = _rnd(_dot(xs, wu_v[...]))
        y = _rnd(_dot((gate * up).astype(BF16), wd_v[...]))[0:1]
        rsel = _rnd(jax.nn.sigmoid(rmax[:, 0:1]))
        y = _rnd(y * rsel)
        if li == 0:
            x2 = _rnd(x1buf[row, :] + _rnd(lsel + y))
            xres[row, :] = x2
            hbuf[row, :] = _layernorm(x2)
        else:
            t0 = pl.multiple_of((idx // 16) * 16, 16)
            tile = pl.ds(PAD + t0, 16)
            sel = lax.broadcasted_iota(jnp.int32, (16, D), 0) == idx - t0
            upd = jnp.where(sel, jnp.broadcast_to(y, (16, D)), 0.0)
            ostage[tile, :] = (x1buf[tile, :] + _rnd(lbuf[tile, :] + upd)).astype(BF16)
            t1 = pl.multiple_of(jnp.minimum(t0, S - PAIR - 16), 16)
            out_copy(S - PAIR, PAIR).start()
            out_copy(t1, 16).start()
            out_copy(0, PAIR + 16).wait()


_FILL = ((0, 9), (0, 11), (0, 13), (0, 15), (1, 8), (1, 10), (1, 12), (1, 14))
CFG = dict(UNROLL=2, LAGA=(1, 1, 1), LAGB=(1, 1, 1), FILL=(_FILL, _FILL),
           SMID=(False, True), LNROWS=256)


def _build():
    any_spec = pl.BlockSpec(memory_space=pl.ANY)
    return pl.pallas_call(
        functools.partial(_kernel, **CFG),
        out_shape=jax.ShapeDtypeStruct((S, D), BF16),
        in_specs=[any_spec] * 10,
        out_specs=any_spec,
        scratch_shapes=[
            pltpu.VMEM((PAD + S, D), BF16),
            pltpu.VMEM((M, D), BF16),
            pltpu.VMEM((1, D), BF16),
            pltpu.VMEM((NCH, D, HC, DH), BF16),
            pltpu.VMEM((HD, D), BF16),
            pltpu.VMEM((D, FF), BF16),
            pltpu.VMEM((D, FF), BF16),
            pltpu.VMEM((FF, D), BF16),
        ] + [pltpu.VMEM((GPC, D // 2, GW), U32)] * NCH + [
            pltpu.VMEM((HD // 2, D), U32),
            pltpu.VMEM((NTMP * TSZ, DH), U32),
            pltpu.VMEM((PAD + S, D), F32),
            pltpu.VMEM((PAD + S, D), F32),
            pltpu.VMEM((PAD + S, D), F32),
            pltpu.VMEM((PAD + S, D), F32),
            pltpu.VMEM((RC, 128), F32),
            pltpu.VMEM((RC, 128), jnp.int32),
            pltpu.VMEM((PAIR + 8, D), F32),
            pltpu.VMEM((PAD + S, D), BF16),
            pltpu.VMEM((8 * NPAIR, D), U32),
            pltpu.VMEM((2 * NG, 16 * NPAIR, GW), F32),
            pltpu.SMEM((1,), jnp.int32),
            pltpu.SemaphoreType.DMA((17,)),
            pltpu.SemaphoreType.DMA(()),
        ],
        compiler_params=pltpu.CompilerParams(vmem_limit_bytes=120 * 1024 * 1024),
    )


@functools.partial(jax.jit, static_argnames=("A_seg_len",))
def pallas_interleave_layers__memory_aug_recurrent_mem_tr__moe_arch_mod__prompt_kernel(
    A_x: jax.Array,
    A_mem0: jax.Array,
    A_Wq: jax.Array,
    A_Wk: jax.Array,
    A_Wv: jax.Array,
    A_Wo: jax.Array,
    A_seg_len,
    B_x: jax.Array,
    B_w_r: jax.Array,
    B_w_gate: jax.Array,
    B_w_up: jax.Array,
    B_w_down: jax.Array,
):
    assert A_seg_len == SEG and A_x.shape == (1, S, D)
    del B_x
    out = _build()(
        A_x.reshape(S, D),
        A_mem0.reshape(M, D),
        A_Wq,
        A_Wk,
        A_Wv,
        A_Wo.reshape(HD, D),
        B_w_r.reshape(1, D),
        B_w_gate,
        B_w_up,
        B_w_down,
    )
    return out.reshape(1, S, D)
```

```python
import functools
import math

import jax
import jax.numpy as jnp
from jax import lax
import jax.experimental.pallas as pl
import jax.experimental.pallas.tpu as pltpu

F32 = jnp.float32
BF16 = jnp.bfloat16
U32 = jnp.uint32

S, D, H, DH, M, SEG = 2048, 512, 32, 128, 8, 32
FF = 1792
HD = H * DH
PAIR = 2 * SEG
NPAIR = S // PAIR
PAD = PAIR
G = 4
NG = H // G
GW = G * DH
HC = 16
GPC = HC // G
NCH = 3 * H // HC
TP = 20
TSZ = 8 * TP
NTMP = 8
RC = 8
LN_EPS = 1e-05
NEG = -1000000000.0
EXP2_SCALE = (DH ** -0.5) * math.log2(math.e)


def _rnd(x):
    return x.astype(BF16).astype(F32)


def _layernorm(x):
    mean = jnp.sum(x, axis=-1, keepdims=True) * (1.0 / D)
    c = x - mean
    var = jnp.sum(c * c, axis=-1, keepdims=True) * (1.0 / D)
    den = _rnd(jnp.sqrt(_rnd(_rnd(var) + _rnd(jnp.float32(LN_EPS)))))
    inv = 1.0 / den
    return _rnd(_rnd(x - _rnd(mean)) * inv)


def _dot(a, b):
    return jnp.dot(a, b, preferred_element_type=F32)


def _dot_nt(a, b):
    return lax.dot_general(a, b, (((1,), (1,)), ((), ())), preferred_element_type=F32)


def _softmax_bf16(s, mask):
    s = jnp.where(mask, s, NEG)
    m = jnp.max(s, axis=-1, keepdims=True)
    e = jnp.exp2((s - m) * EXP2_SCALE)
    l = jnp.sum(e, axis=-1, keepdims=True)
    r = pl.reciprocal(l, approx=True)
    r = r * (2.0 - l * r)
    return (e * r).astype(BF16)


def _kernel(x_hbm, mem0_hbm, wq_hbm, wk_hbm, wv_hbm, wo_hbm, wr_hbm, wg_hbm, wu_hbm, wd_hbm,
            out_hbm,
            x_raw, mem0_v, wr_v, stage, wo_raw, wg_v, wu_v, wd_v,
            wk0, wk1, wv0, wv1, wq0, wq1, wo, tmp,
            xres, x1buf, lbuf, hbuf, rbest, ibest, obuf, ostage,
            lhs_pre, pre, anchor, sems, osem, *,
            UNROLLS, LAGA, LAGB, FILL, SMID, LNROWS, SLACK):
    wch = (wk0, wk1, wv0, wv1, wq0, wq1)
    NXP = 4
    XP = S // NXP
    SEM_X, SEM_W, SEM_O, SEM_MISC = 0, NXP, NXP + NCH + 1, NXP + NCH + 3

    def cp_x(i):
        return pltpu.make_async_copy(x_hbm.at[pl.ds(i * XP, XP)],
                                     x_raw.at[pl.ds(PAD + i * XP, XP)], sems.at[SEM_X + i])

    def cp_w(c, half=None):
        w = (wk_hbm, wv_hbm, wq_hbm)[c // 2]
        heads = pl.ds((c % 2) * HC, HC)
        if half is None:
            return pltpu.make_async_copy(w.at[:, heads, :], stage.at[pl.ds(c * D, D)],
                                         sems.at[SEM_W + 1 + c])
        return pltpu.make_async_copy(w.at[pl.ds(half * (D // 2), D // 2), heads, :],
                                     stage.at[pl.ds(c * D + half * (D // 2), D // 2)],
                                     sems.at[SEM_W + half])

    def cp_o(i):
        return pltpu.make_async_copy(wo_hbm.at[pl.ds(i * (HD // 2), HD // 2)],
                                     wo_raw.at[pl.ds(i * (HD // 2), HD // 2)],
                                     sems.at[SEM_O + i])

    cp_small = [pltpu.make_async_copy(s_, d_, sems.at[SEM_MISC + i])
                for i, (s_, d_) in enumerate(((mem0_hbm, mem0_v), (wr_hbm, wr_v)))]
    cp_mlp = [pltpu.make_async_copy(s_, d_, sems.at[SEM_MISC + 2 + i])
              for i, (s_, d_) in enumerate(((wg_hbm, wg_v), (wu_hbm, wu_v), (wd_hbm, wd_v)))]
    for i in range(NXP):
        cp_x(i).start()
    cp_w(0, 0).start()
    cp_w(0, 1).start()
    for c in range(1, NCH):
        cp_w(c).start()
    for i in range(2):
        cp_o(i).start()
    for c in cp_small + cp_mlp:
        c.start()

    anchor[0] = PAIR
    anchor[1] = NCH * D
    anchor[2] = HD
    x_raw[0:PAD, :] = jnp.zeros((PAD, D), BF16)
    xres[0:PAD, :] = jnp.zeros((PAD, D), F32)

    def ln0(i, carry):
        @pl.when(i % (XP // LNROWS) == 0)
        def _():
            cp_x(i // (XP // LNROWS)).wait()

        for pp in range(LNROWS // PAIR):
            r0 = pl.multiple_of(PAD + i * LNROWS + pp * PAIR, PAIR)
            ln = []
            for c in range(PAIR // 16):
                ln.append(_layernorm(x_raw[pl.ds(r0 + c * 16, 16), :].astype(F32)))
                hbuf[pl.ds(r0 + c * 16, 16), :] = ln[c]
            mid = jnp.concatenate([ln[1][8:16], ln[2][0:8]], axis=0).astype(BF16)
            p0 = pl.multiple_of((i * (LNROWS // PAIR) + pp) * 8, 8)
            lhs_pre[pl.ds(p0, 8), :] = pltpu.bitcast(mid, U32)
        return carry

    lax.fori_loop(0, S // LNROWS, ln0, 0)

    def relayout_jobs(c, blk0, nblk, slot0=0):
        def job(u):
            t0 = ((slot0 + u) % NTMP) * TSZ
            d0 = pl.multiple_of(c * D + (blk0 + u) * 16, 16)
            raw = pltpu.bitcast(stage[pl.ds(d0, 16), :, :], U32)
            for i in range(8):
                ev, od = raw[2 * i], raw[2 * i + 1]
                lo = (ev & jnp.uint32(0xFFFF)) | (od << 16)
                hi = (ev >> 16) | (od & jnp.uint32(0xFFFF0000))
                tmp[pl.ds(t0 + i * TP, 8, stride=2), :] = lo
                tmp[pl.ds(t0 + i * TP + 1, 8, stride=2), :] = hi
            o0 = pl.multiple_of((blk0 + u) * 8, 8)
            for hh in range(HC):
                col = (hh % G) * DH
                wch[c][hh // G, pl.ds(o0, 8), col:col + DH] = tmp[pl.ds(t0 + hh, 8, stride=TP), :]

        return [('stage', functools.partial(job, u)) for u in range(nblk)]

    def repack_jobs(half):
        def job(c):
            r0 = pl.multiple_of(half * (HD // 2) + c * 128, 128)
            o0 = pl.multiple_of(half * (HD // 4) + c * 64, 64)
            wo[pl.ds(o0, 64), :] = pltpu.bitcast(wo_raw[pl.ds(r0, 128), :], U32)

        return [('wo_raw', functools.partial(job, c)) for c in range(HD // 2 // 128)]

    def precompute(c, g0, ng, jobs):
        lhs = pltpu.bitcast(lhs_pre[...], BF16)
        ys = [_dot(lhs, pltpu.bitcast(wch[c][g0 + gg], BF16)) for gg in range(ng)]
        nrow = 16 * NPAIR
        for u, (kind, job) in enumerate(jobs):
            if u > 0:
                pos = (u * ng * G * nrow // len(jobs)) // 16 * 16 - 16 * SLACK
                pos = max(pos, 0)
                nt, r0 = pos // nrow, pos % nrow
                tie = ys[nt // G][r0:r0 + 16, (nt % G) * DH:(nt % G + 1) * DH].astype(BF16)
                if kind == 'stage':
                    stage[anchor[1]] = tie
                else:
                    wo_raw[pl.ds(pl.multiple_of(anchor[2], 16), 16), 0:DH] = tie
            job()
        for gg in range(ng):
            pre[c * GPC + g0 + gg] = ys[gg]

    def run(jobs):
        for _, job in jobs:
            job()

    NBLK = D // 16

    def relay0(it, carry):
        @pl.when(it % 2 == 0)
        def _():
            cp_w(0, it // 2).wait()
        run(relayout_jobs(0, it * 8, 8))
        return carry

    lax.fori_loop(0, NBLK // 8, relay0, 0)
    lax.fori_loop(0, 2, lambda it, cr: (precompute(0, it, 1, []), cr)[1], 0)
    cp_w(1).wait()
    lax.fori_loop(0, 2, lambda it, cr: (
        precompute(0, 2 + it, 1, relayout_jobs(1, it * (NBLK // 2), NBLK // 2)), cr)[1], 0)

    def phase(c, chunks, with_wo):
        for cc in chunks:
            cp_w(cc).wait()

        def body(it, carry):
            if with_wo:
                cp_o(it).wait()
            jl = [relayout_jobs(cc, it * (NBLK // 2), NBLK // 2, n * (NTMP // 2))
                  for n, cc in enumerate(chunks)]
            if with_wo:
                jl.append(repack_jobs(it))
            jobs = [j for group in zip(*jl) for j in group]
            precompute(c, it * 2, 2, jobs)
            return carry

        lax.fori_loop(0, 2, body, 0)

    phase(1, (2,), False)
    phase(2, (3, 4), False)
    phase(3, (5,), True)

    for c in cp_small:
        c.wait()
    wr = wr_v[...].astype(F32)

    qi = lax.broadcasted_iota(jnp.int32, (32, 48), 0)
    kj = lax.broadcasted_iota(jnp.int32, (32, 48), 1)
    mask_a = (kj < 40) & ((qi < M) | (kj <= qi))
    qi = lax.broadcasted_iota(jnp.int32, (48, 80), 0)
    kj = lax.broadcasted_iota(jnp.int32, (48, 80), 1)
    kb0 = (kj >= 40) & (kj < 48)
    m_mem = (qi < M) & ((kj < 32) | kb0)
    m_xb = (qi >= M) & (qi < 32) & ((kj <= qi) | kb0)
    m_xa = (qi >= 32) & (qi < 40) & ((kj >= 48) | ((kj >= 32) & (kj <= qi)))
    m_b0 = (qi >= 40) & ((kj < M) | (kb0 & (kj <= qi)))
    mask_b = m_mem | m_xb | m_xa | m_b0

    def w_ref(mi, g):
        return wch[(4, 0, 2)[mi] + g // GPC].at[g % GPC]

    def wo_rows(g):
        r0 = g * GW // 2
        return pltpu.bitcast(wo[r0:r0 + GW // 2, :], BF16)

    def seg_step(lhs, lhs_f32, extra, mask, lags, s_mid, filler):
        q, k, v, p, o = {}, {}, {}, {}, {}
        raw = ({}, {}, {})
        acc = [None]

        def proj(mi, g, dst):
            if mi == 0 and g == 0:
                y = None
                lp = jnp.concatenate([lhs_f32[16:], lhs_f32[0:16]], axis=0)
                for kt in range(D // 128):
                    w = pltpu.bitcast(w_ref(0, 0)[kt * 64:(kt + 1) * 64, :], BF16)
                    t = _dot(lp[:, kt * 128:(kt + 1) * 128].astype(BF16), w)
                    y = t if y is None else y + t
                nr = y.shape[0]
                y = jnp.concatenate([y[nr - 16:], y[0:nr - 16]], axis=0)
            else:
                y = _dot(lhs[mi], pltpu.bitcast(w_ref(mi, g)[...], BF16))
            for j in range(G):
                h = g * G + j
                yh = y[:, j * DH:(j + 1) * DH]
                ex = extra(mi, h)
                if ex:
                    yh = jnp.concatenate([yh] + ex, axis=0)
                raw[mi][h] = yh
                dst[h] = yh.astype(BF16)

        def sc(g):
            for h in range(g * G, (g + 1) * G):
                p[h] = _softmax_bf16(_dot_nt(q[h], k[h]), mask)

        def pv(g):
            o[g] = jnp.concatenate(
                [_dot(p[h], v[h]) for h in range(g * G, (g + 1) * G)], axis=1).astype(BF16)

        def op(g):
            y = _dot(o[g], wo_rows(g))
            acc[0] = y if acc[0] is None else acc[0] + y

        ls, lp, lo = lags
        for t in range(2 * NG + lp + lo):
            if t < NG:
                proj(0, t, q)
                if s_mid and 0 <= t - ls < NG:
                    sc(t - ls)
                proj(1, t, k)
            elif t < 2 * NG:
                proj(2, t - NG, v)
            if 0 <= t - ls < NG and not s_mid:
                sc(t - ls)
            if 0 <= t - NG - lp < NG:
                pv(t - NG - lp)
            if s_mid and t == NG + lp:
                for g in range(NG - ls, NG):
                    sc(g)
            if 0 <= t - NG - lp - lo < NG:
                op(t - NG - lp - lo)
            if t in filler:
                src = raw[1][t * G] if t < NG else raw[2][min(t - NG, NG - 1) * G]
                filler[t](src[0:8])
        return acc[0], raw

    subr = lax.broadcasted_iota(jnp.int32, (RC, 128), 0)

    def post_chunk(li, base, valid, c, tie=None):
        if tie is not None:
            obuf[pl.ds(pl.multiple_of(anchor[0], 8), 8), 0:DH] = tie
        rows = pl.ds(base + c * RC, RC)
        x0 = x_raw[rows, :].astype(F32) if li == 0 else xres[rows, :]
        x1 = _rnd(x0 + _rnd(obuf[c * RC:(c + 1) * RC, :]))
        ln = _layernorm(x1)
        r = _rnd(jnp.sum(ln * wr, axis=-1, keepdims=True))
        r = jnp.broadcast_to(jnp.where(valid, r, -jnp.inf), (RC, 128))
        rb = rbest[...]
        better = r > rb
        rbest[...] = jnp.where(better, r, rb)
        ibest[...] = jnp.where(better, subr + (base + (c * RC - PAD)), ibest[...])
        x1buf[rows, :] = x1
        lbuf[rows, :] = ln
        if li == 0:
            x2 = _rnd(x1 + ln)
            xres[rows, :] = x2
            hbuf[rows, :] = _layernorm(x2)
        else:
            ostage[rows, :] = (x1 + ln).astype(BF16)

    def out_copy(row0, nrows):
        return pltpu.make_async_copy(ostage.at[pl.ds(PAD + row0, nrows)],
                                     out_hbm.at[pl.ds(row0, nrows)], osem)

    def pair_body(li, pi, mem):
        base = pl.multiple_of(pi * PAIR, PAIR)
        ha = hbuf[pl.ds(base + PAD, 40), :]
        hb = hbuf[pl.ds(base + PAD + 40, 24), :]
        fill = ({}, {})
        for c, (st, t) in enumerate(FILL[li]):
            fill[st][t] = functools.partial(post_chunk, li, base, pi > 0, c)
        aq = jnp.concatenate([mem, ha[0:24]], axis=0)
        lhs_aq = aq.astype(BF16)
        if li == 0:
            p0 = pl.multiple_of(pi * 16, 16)
            lhs_akv = lhs_aq
            extra_a = lambda mi, h: [pre[(mi - 1) * NG + h // G, pl.ds(p0, 16),
                                         (h % G) * DH:(h % G + 1) * DH]] if mi else []
        else:
            lhs_akv = jnp.concatenate([mem, ha], axis=0).astype(BF16)
            extra_a = lambda mi, h: []
        acc_a, prj = seg_step((lhs_aq, lhs_akv, lhs_akv), aq, extra_a, mask_a,
                              LAGA, SMID[0], fill[0])
        lhs_b = jnp.concatenate([acc_a[0:8], hb], axis=0).astype(BF16)
        bq = jnp.concatenate([acc_a[0:8], hb, ha[24:40]], axis=0)
        acc_b, _ = seg_step(
            (bq.astype(BF16), lhs_b, lhs_b), bq,
            lambda mi, h: [prj[mi][h][32:48], prj[mi][h][0:32]] if mi else [],
            mask_b, LAGB, SMID[1], fill[1])
        obuf[0:24, :] = acc_a[8:32]
        obuf[24:40, :] = acc_b[32:48]
        obuf[40:64, :] = acc_b[8:32]
        return acc_b[0:8]

    def loop_body(li, it, mem):
        UNROLL = UNROLLS[li]
        for u in range(UNROLL):
            mem = pair_body(li, it * UNROLL + u, mem)

        if li == 1:
            @pl.when(it > 0)
            def _():
                out_copy(pl.multiple_of(it * (UNROLL * PAIR) - PAIR, PAIR),
                         UNROLL * PAIR).start()

            if UNROLL > 1:
                @pl.when(it == 0)
                def _():
                    out_copy(0, (UNROLL - 1) * PAIR).start()

        return mem

    for li in range(2):
        obuf[0:PAIR, :] = jnp.zeros((PAIR, D), F32)
        rbest[...] = jnp.full((RC, 128), -jnp.inf, F32)
        ibest[...] = jnp.zeros((RC, 128), jnp.int32)
        lax.fori_loop(0, NPAIR // UNROLLS[li], functools.partial(loop_body, li),
                      mem0_v[...].astype(F32))

        if li == 0:
            for c in cp_mlp:
                c.wait()
        else:
            out_copy(0, S - PAIR).wait()

        for c in range(PAIR // RC):
            post_chunk(li, S, True, c)

        rb = rbest[...]
        rmax = jnp.max(rb, axis=0, keepdims=True)
        idx = jnp.min(jnp.where(rb == rmax, ibest[...], S - 1))
        row = pl.ds(PAD + idx, 1)
        lsel = lbuf[row, :]
        xs = jnp.broadcast_to(lsel, (16, D)).astype(BF16)
        gpre = _rnd(_dot(xs, wg_v[...]))
        gate = _rnd(gpre * _rnd(jax.nn.sigmoid(gpre)))
        up = _rnd(_dot(xs, wu_v[...]))
        y = _rnd(_dot((gate * up).astype(BF16), wd_v[...]))[0:1]
        rsel = _rnd(jax.nn.sigmoid(rmax[:, 0:1]))
        y = _rnd(y * rsel)
        if li == 0:
            x2 = _rnd(x1buf[row, :] + _rnd(lsel + y))
            xres[row, :] = x2
            hbuf[row, :] = _layernorm(x2)
        else:
            t0 = pl.multiple_of((idx // 16) * 16, 16)
            tile = pl.ds(PAD + t0, 16)
            sel = lax.broadcasted_iota(jnp.int32, (16, D), 0) == idx - t0
            upd = jnp.where(sel, jnp.broadcast_to(y, (16, D)), 0.0)
            ostage[tile, :] = (x1buf[tile, :] + _rnd(lbuf[tile, :] + upd)).astype(BF16)
            t1 = pl.multiple_of(jnp.minimum(t0, S - PAIR - 16), 16)
            out_copy(S - PAIR, PAIR).start()
            out_copy(t1, 16).start()
            out_copy(0, PAIR + 16).wait()


_FILL = ((0, 9), (0, 11), (0, 13), (0, 15), (1, 8), (1, 10), (1, 12), (1, 14))
CFG = dict(UNROLLS=(2, 2), LAGA=(1, 1, 1), LAGB=(1, 1, 1), FILL=(_FILL, _FILL),
           SMID=(False, True), LNROWS=256, SLACK=8)


def _build():
    any_spec = pl.BlockSpec(memory_space=pl.ANY)
    return pl.pallas_call(
        functools.partial(_kernel, **CFG),
        out_shape=jax.ShapeDtypeStruct((S, D), BF16),
        in_specs=[any_spec] * 10,
        out_specs=any_spec,
        scratch_shapes=[
            pltpu.VMEM((PAD + S, D), BF16),
            pltpu.VMEM((M, D), BF16),
            pltpu.VMEM((1, D), BF16),
            pltpu.VMEM((NCH * D + 1, HC, DH), BF16),
            pltpu.VMEM((HD + 16, D), BF16),
            pltpu.VMEM((D, FF), BF16),
            pltpu.VMEM((D, FF), BF16),
            pltpu.VMEM((FF, D), BF16),
        ] + [pltpu.VMEM((GPC, D // 2, GW), U32)] * NCH + [
            pltpu.VMEM((HD // 2, D), U32),
            pltpu.VMEM((NTMP * TSZ, DH), U32),
            pltpu.VMEM((PAD + S, D), F32),
            pltpu.VMEM((PAD + S, D), F32),
            pltpu.VMEM((PAD + S, D), F32),
            pltpu.VMEM((PAD + S, D), F32),
            pltpu.VMEM((RC, 128), F32),
            pltpu.VMEM((RC, 128), jnp.int32),
            pltpu.VMEM((PAIR + 8, D), F32),
            pltpu.VMEM((PAD + S, D), BF16),
            pltpu.VMEM((8 * NPAIR, D), U32),
            pltpu.VMEM((2 * NG, 16 * NPAIR, GW), F32),
            pltpu.SMEM((3,), jnp.int32),
            pltpu.SemaphoreType.DMA((18,)),
            pltpu.SemaphoreType.DMA(()),
        ],
        compiler_params=pltpu.CompilerParams(vmem_limit_bytes=120 * 1024 * 1024),
    )


@functools.partial(jax.jit, static_argnames=("A_seg_len",))
def pallas_interleave_layers__memory_aug_recurrent_mem_tr__moe_arch_mod__prompt_kernel(
    A_x: jax.Array,
    A_mem0: jax.Array,
    A_Wq: jax.Array,
    A_Wk: jax.Array,
    A_Wv: jax.Array,
    A_Wo: jax.Array,
    A_seg_len,
    B_x: jax.Array,
    B_w_r: jax.Array,
    B_w_gate: jax.Array,
    B_w_up: jax.Array,
    B_w_down: jax.Array,
):
    assert A_seg_len == SEG and A_x.shape == (1, S, D)
    del B_x
    out = _build()(
        A_x.reshape(S, D),
        A_mem0.reshape(M, D),
        A_Wq,
        A_Wk,
        A_Wv,
        A_Wo.reshape(HD, D),
        B_w_r.reshape(1, D),
        B_w_gate,
        B_w_up,
        B_w_down,
    )
    return out.reshape(1, S, D)
```

```python
import functools
import math

import jax
import jax.numpy as jnp
from jax import lax
import jax.experimental.pallas as pl
import jax.experimental.pallas.tpu as pltpu

F32 = jnp.float32
BF16 = jnp.bfloat16
U32 = jnp.uint32

S, D, H, DH, M, SEG = 2048, 512, 32, 128, 8, 32
FF = 1792
HD = H * DH
PAIR = 2 * SEG
NPAIR = S // PAIR
PAD = PAIR
G = 4
NG = H // G
GW = G * DH
HC = 16
GPC = HC // G
NCH = 3 * H // HC
TP = 20
TSZ = 8 * TP
NTMP = 8
RC = 8
LN_EPS = 1e-05
NEG = -1000000000.0
EXP2_SCALE = (DH ** -0.5) * math.log2(math.e)


def _rnd(x):
    return x.astype(BF16).astype(F32)


def _layernorm(x):
    mean = jnp.sum(x, axis=-1, keepdims=True) * (1.0 / D)
    c = x - mean
    var = jnp.sum(c * c, axis=-1, keepdims=True) * (1.0 / D)
    den = _rnd(jnp.sqrt(_rnd(_rnd(var) + _rnd(jnp.float32(LN_EPS)))))
    inv = 1.0 / den
    return _rnd(_rnd(x - _rnd(mean)) * inv)


def _dot(a, b):
    return jnp.dot(a, b, preferred_element_type=F32)


def _dot_nt(a, b):
    return lax.dot_general(a, b, (((1,), (1,)), ((), ())), preferred_element_type=F32)


def _softmax_bf16(s, mask):
    s = jnp.where(mask, s, NEG)
    m = jnp.max(s, axis=-1, keepdims=True)
    e = jnp.exp2((s - m) * EXP2_SCALE)
    l = jnp.sum(e, axis=-1, keepdims=True)
    r = pl.reciprocal(l, approx=True)
    r = r * (2.0 - l * r)
    return (e * r).astype(BF16)


def _kernel(x_hbm, mem0_hbm, wq_hbm, wk_hbm, wv_hbm, wo_hbm, wr_hbm, wg_hbm, wu_hbm, wd_hbm,
            out_hbm,
            x_raw, mem0_v, wr_v, stage, wo_raw, wg_v, wu_v, wd_v,
            wk0, wk1, wv0, wv1, wq0, wq1, wo, tmp,
            xres, x1buf, lbuf, hbuf, rbest, ibest, obuf, ostage,
            lhs_pre, pre, anchor, sems, osem, *,
            UNROLLS, LAGA, LAGB, FILL, SMID, LNP, LNA, SLACK):
    wch = (wk0, wk1, wv0, wv1, wq0, wq1)
    NWO = 4
    WOP = HD // NWO
    SEM_X, SEM_W, SEM_O, SEM_MISC = 0, 3, 3 + NCH + 1, 3 + NCH + 1 + NWO

    def cp_x(i):
        r0, nr = ((24, 16), (0, 24), (40, 24))[i]
        return pltpu.make_async_copy(x_hbm.at[:, pl.ds(r0, nr), :],
                                     x_raw.at[pl.ds(1, NPAIR), pl.ds(r0, nr), :],
                                     sems.at[SEM_X + i])

    def cp_w(c, half=None):
        w = (wk_hbm, wv_hbm, wq_hbm)[c // 2]
        heads = pl.ds((c % 2) * HC, HC)
        if half is None:
            return pltpu.make_async_copy(w.at[:, heads, :], stage.at[pl.ds(c * D, D)],
                                         sems.at[SEM_W + 1 + c])
        return pltpu.make_async_copy(w.at[pl.ds(half * (D // 2), D // 2), heads, :],
                                     stage.at[pl.ds(c * D + half * (D // 2), D // 2)],
                                     sems.at[SEM_W + half])

    def cp_o(i):
        return pltpu.make_async_copy(wo_hbm.at[pl.ds(i * WOP, WOP)],
                                     wo_raw.at[pl.ds(i * WOP, WOP)], sems.at[SEM_O + i])

    cp_small = [pltpu.make_async_copy(s_, d_, sems.at[SEM_MISC + i])
                for i, (s_, d_) in enumerate(((mem0_hbm, mem0_v), (wr_hbm, wr_v)))]
    cp_mlp = [pltpu.make_async_copy(s_, d_, sems.at[SEM_MISC + 2 + i])
              for i, (s_, d_) in enumerate(((wg_hbm, wg_v), (wu_hbm, wu_v), (wd_hbm, wd_v)))]
    cp_x(0).start()
    cp_w(0, 0).start()
    cp_w(0, 1).start()
    cp_w(1).start()
    cp_w(2).start()
    cp_x(1).start()
    cp_x(2).start()
    for c in range(3, NCH):
        cp_w(c).start()
    for i in range(NWO):
        cp_o(i).start()
    for c in cp_small + cp_mlp:
        c.start()

    anchor[0] = PAIR
    anchor[1] = NCH * D
    anchor[2] = HD
    anchor[3] = NPAIR + 1
    x_raw[0] = jnp.zeros((PAIR, D), BF16)
    xres[0:PAD, :] = jnp.zeros((PAD, D), F32)

    cp_x(0).wait()

    def ln_mid(i, carry):
        for pp in range(LNP):
            pr = i * LNP + pp
            ln = _layernorm(x_raw[1 + pr, 24:40, :].astype(F32))
            hbuf[pl.ds(pl.multiple_of(PAD + pr * PAIR + 24, 8), 16), :] = ln
            lhs_pre[pl.ds(pl.multiple_of(pr * 8, 8), 8), :] = pltpu.bitcast(ln.astype(BF16), U32)
        return carry

    lax.fori_loop(0, NPAIR // LNP, ln_mid, 0)

    def ln_jobs(p0, npairs):
        def job(pp, r0):
            ln = _layernorm(x_raw[1 + p0 + pp, r0:r0 + 8, :].astype(F32))
            hbuf[pl.ds(pl.multiple_of(PAD + (p0 + pp) * PAIR + r0, 8), 8), :] = ln

        return [('x_raw', functools.partial(job, pp, r0))
                for pp in range(npairs) for r0 in (0, 8, 16, 40, 48, 56)]

    def relayout_jobs(c, blk0, nblk, slot0=0):
        def job(u):
            t0 = ((slot0 + u) % NTMP) * TSZ
            d0 = pl.multiple_of(c * D + (blk0 + u) * 16, 16)
            raw = pltpu.bitcast(stage[pl.ds(d0, 16), :, :], U32)
            for i in range(8):
                ev, od = raw[2 * i], raw[2 * i + 1]
                lo = (ev & jnp.uint32(0xFFFF)) | (od << 16)
                hi = (ev >> 16) | (od & jnp.uint32(0xFFFF0000))
                tmp[pl.ds(t0 + i * TP, 8, stride=2), :] = lo
                tmp[pl.ds(t0 + i * TP + 1, 8, stride=2), :] = hi
            o0 = pl.multiple_of((blk0 + u) * 8, 8)
            for hh in range(HC):
                col = (hh % G) * DH
                wch[c][hh // G, pl.ds(o0, 8), col:col + DH] = tmp[pl.ds(t0 + hh, 8, stride=TP), :]

        return [('stage', functools.partial(job, u)) for u in range(nblk)]

    def repack_jobs(part):
        def job(c):
            r0 = pl.multiple_of(part * WOP + c * 128, 128)
            o0 = pl.multiple_of(part * (WOP // 2) + c * 64, 64)
            wo[pl.ds(o0, 64), :] = pltpu.bitcast(wo_raw[pl.ds(r0, 128), :], U32)

        return [('wo_raw', functools.partial(job, c)) for c in range(WOP // 128)]

    def interleave(*lists):
        keyed = [((i + 0.5) / len(l), n, j) for n, l in enumerate(lists) for i, j in enumerate(l)]
        return [j for _, _, j in sorted(keyed, key=lambda t: t[:2])]

    def precompute(c, g0, ng, jobs):
        lhs = pltpu.bitcast(lhs_pre[...], BF16)
        ys = [_dot(lhs, pltpu.bitcast(wch[c][g0 + gg], BF16)) for gg in range(ng)]
        nrow = 16 * NPAIR
        has_ln = any(kind == 'x_raw' for kind, _ in jobs)
        for u, (kind, job) in enumerate(jobs):
            if u > 0:
                span = ng * G * nrow - (SLACK[1] if has_ln else SLACK[0])
                pos = max((u * span // len(jobs)) // 16 * 16 - 128, 0)
                nt, r0 = pos // nrow, pos % nrow
                tie = ys[nt // G][r0:r0 + 16, (nt % G) * DH:(nt % G + 1) * DH].astype(BF16)
                if kind == 'stage':
                    stage[anchor[1]] = tie
                elif kind == 'x_raw':
                    x_raw[anchor[3], 0:16, 0:DH] = tie
                else:
                    wo_raw[pl.ds(pl.multiple_of(anchor[2], 16), 16), 0:DH] = tie
            job()
        for gg in range(ng):
            pre[c * GPC + g0 + gg] = ys[gg]

    def run(jobs):
        for _, job in jobs:
            job()

    NBLK = D // 16

    def relay0(it, carry):
        @pl.when(it % 2 == 0)
        def _():
            cp_w(0, it // 2).wait()
        run(relayout_jobs(0, it * 8, 8))
        return carry

    lax.fori_loop(0, NBLK // 8, relay0, 0)
    lax.fori_loop(0, 2, lambda it, cr: (precompute(0, it, 1, []), cr)[1], 0)
    cp_w(1).wait()
    lax.fori_loop(0, 2, lambda it, cr: (
        precompute(0, 2 + it, 1, relayout_jobs(1, it * (NBLK // 2), NBLK // 2)), cr)[1], 0)

    HB, QB = NBLK // 2, NBLK // 4
    cp_w(2).wait()
    lax.fori_loop(0, 2, lambda it, cr: (
        precompute(1, it * 2, 2, relayout_jobs(2, it * HB, HB)), cr)[1], 0)
    cp_x(1).wait()
    cp_x(2).wait()
    cp_w(3).wait()
    lax.fori_loop(0, 2, lambda it, cr: (
        precompute(2, it * 2, 2, interleave(relayout_jobs(3, it * HB, HB),
                                            ln_jobs(it * LNA, LNA))), cr)[1], 0)
    cp_w(4).wait()
    cp_w(5).wait()
    LNB = (NPAIR - 2 * LNA) // 4

    def last_phase(it, carry):
        cp_o(it).wait()
        precompute(3, it, 1, interleave(relayout_jobs(4, it * QB, QB),
                                        relayout_jobs(5, it * QB, QB, NTMP // 2),
                                        repack_jobs(it),
                                        ln_jobs(2 * LNA + it * LNB, LNB)))
        return carry

    lax.fori_loop(0, 4, last_phase, 0)

    for c in cp_small:
        c.wait()
    wr = wr_v[...].astype(F32).reshape(1, D)

    qi = lax.broadcasted_iota(jnp.int32, (32, 48), 0)
    kj = lax.broadcasted_iota(jnp.int32, (32, 48), 1)
    mask_a = (kj < 40) & ((qi < M) | (kj <= qi))
    qi = lax.broadcasted_iota(jnp.int32, (48, 80), 0)
    kj = lax.broadcasted_iota(jnp.int32, (48, 80), 1)
    kb0 = (kj >= 40) & (kj < 48)
    m_mem = (qi < M) & ((kj < 32) | kb0)
    m_xb = (qi >= M) & (qi < 32) & ((kj <= qi) | kb0)
    m_xa = (qi >= 32) & (qi < 40) & ((kj >= 48) | ((kj >= 32) & (kj <= qi)))
    m_b0 = (qi >= 40) & ((kj < M) | (kb0 & (kj <= qi)))
    mask_b = m_mem | m_xb | m_xa | m_b0

    def w_ref(mi, g):
        return wch[(4, 0, 2)[mi] + g // GPC].at[g % GPC]

    def wo_rows(g, n=1):
        r0 = g * GW // 2
        return pltpu.bitcast(wo[r0:r0 + n * GW // 2, :], BF16)

    def seg_step(lhs, lhs_f32, extra, mask, lags, s_mid, filler):
        q, k, v, p, o = {}, {}, {}, {}, {}
        raw = ({}, {}, {})
        acc = [None]

        def proj(mi, g, dst):
            if mi == 0 and g == 0:
                y = None
                lp = jnp.concatenate([lhs_f32[16:], lhs_f32[0:16]], axis=0)
                for kt in range(D // 128):
                    w = pltpu.bitcast(w_ref(0, 0)[kt * 64:(kt + 1) * 64, :], BF16)
                    t = _dot(lp[:, kt * 128:(kt + 1) * 128].astype(BF16), w)
                    y = t if y is None else y + t
                nr = y.shape[0]
                y = jnp.concatenate([y[nr - 16:], y[0:nr - 16]], axis=0)
            else:
                y = _dot(lhs[mi], pltpu.bitcast(w_ref(mi, g)[...], BF16))
            for j in range(G):
                h = g * G + j
                yh = y[:, j * DH:(j + 1) * DH]
                ex = extra(mi, h)
                if ex:
                    yh = jnp.concatenate([yh] + ex, axis=0)
                raw[mi][h] = yh
                dst[h] = yh.astype(BF16)

        def sc(g):
            for h in range(g * G, (g + 1) * G):
                p[h] = _softmax_bf16(_dot_nt(q[h], k[h]), mask)

        def pv(g):
            o[g] = jnp.concatenate(
                [_dot(p[h], v[h]) for h in range(g * G, (g + 1) * G)], axis=1)

        def op(g):
            if merge and g == NG - 2:
                return
            if merge and g == NG - 1:
                y = _dot(jnp.concatenate([o[g - 1], o[g]], axis=1).astype(BF16),
                         wo_rows(g - 1, 2))
            else:
                y = _dot(o[g].astype(BF16), wo_rows(g))
            acc[0] = y if acc[0] is None else acc[0] + y

        ls, lp, lo, merge = lags
        for t in range(2 * NG + lp + lo):
            if t < NG:
                proj(0, t, q)
                if s_mid and 0 <= t - ls < NG:
                    sc(t - ls)
                proj(1, t, k)
            elif t < 2 * NG:
                proj(2, t - NG, v)
            if 0 <= t - ls < NG and not s_mid:
                sc(t - ls)
            if 0 <= t - NG - lp < NG:
                pv(t - NG - lp)
            if s_mid and t == NG + lp:
                for g in range(NG - ls, NG):
                    sc(g)
            if 0 <= t - NG - lp - lo < NG:
                op(t - NG - lp - lo)
            if t in filler:
                src = raw[1][t * G] if t < NG else raw[2][min(t - NG, NG - 1) * G]
                filler[t](src[0:8])
        return acc[0], raw

    subr = lax.broadcasted_iota(jnp.int32, (RC, 128), 0).astype(F32)

    def post_chunk(li, pi, valid, c, tie=None):
        if tie is not None:
            obuf[pl.ds(pl.multiple_of(anchor[0], 8), 8), 0:DH] = tie
        base = pi * PAIR if isinstance(pi, int) else pl.multiple_of(pi * PAIR, PAIR)
        rows = pl.ds(base + c * RC, RC)
        x0 = x_raw[pi, c * RC:(c + 1) * RC, :].astype(F32) if li == 0 else xres[rows, :]
        x1 = _rnd(x0 + _rnd(obuf[c * RC:(c + 1) * RC, :]))
        ln = _layernorm(x1)
        r = _rnd(jnp.sum(ln * wr, axis=-1, keepdims=True))
        r = jnp.broadcast_to(jnp.where(valid, r, -jnp.inf), (RC, 128))
        rb = rbest[...]
        better = r > rb
        rbest[...] = jnp.where(better, r, rb)
        row0 = jnp.asarray(base + (c * RC - PAD), jnp.int32).astype(F32)
        ibest[...] = jnp.where(better, subr + row0, ibest[...])
        x1buf[rows, :] = x1
        lbuf[rows, :] = ln
        if li == 0:
            x2 = _rnd(x1 + ln)
            xres[rows, :] = x2
            hbuf[rows, :] = _layernorm(x2)
        else:
            ostage[rows, :] = (x1 + ln).astype(BF16)

    def out_copy(row0, nrows):
        return pltpu.make_async_copy(ostage.at[pl.ds(PAD + row0, nrows)],
                                     out_hbm.at[pl.ds(row0, nrows)], osem)

    def pair_body(li, pi, mem):
        base = pl.multiple_of(pi * PAIR, PAIR)
        ha = hbuf[pl.ds(base + PAD, 40), :]
        hb = hbuf[pl.ds(base + PAD + 40, 24), :]
        fill = ({}, {})
        for c, (st, t) in enumerate(FILL[li]):
            fill[st][t] = functools.partial(post_chunk, li, pi, pi > 0, c)
        aq = jnp.concatenate([mem, ha[0:24]], axis=0)
        lhs_aq = aq.astype(BF16)
        if li == 0:
            p0 = pl.multiple_of(pi * 16, 16)
            lhs_akv = lhs_aq
            extra_a = lambda mi, h: [pre[(mi - 1) * NG + h // G, pl.ds(p0, 16),
                                         (h % G) * DH:(h % G + 1) * DH]] if mi else []
        else:
            lhs_akv = jnp.concatenate([mem, ha], axis=0).astype(BF16)
            extra_a = lambda mi, h: []
        acc_a, prj = seg_step((lhs_aq, lhs_akv, lhs_akv), aq, extra_a, mask_a,
                              LAGA, SMID[0], fill[0])
        lhs_b = jnp.concatenate([acc_a[0:8], hb], axis=0).astype(BF16)
        bq = jnp.concatenate([acc_a[0:8], hb, ha[24:40]], axis=0)
        acc_b, _ = seg_step(
            (bq.astype(BF16), lhs_b, lhs_b), bq,
            lambda mi, h: [prj[mi][h][32:48], prj[mi][h][0:32]] if mi else [],
            mask_b, LAGB, SMID[1], fill[1])
        obuf[0:24, :] = acc_a[8:32]
        obuf[24:40, :] = acc_b[32:48]
        obuf[40:64, :] = acc_b[8:32]
        return acc_b[0:8]

    def loop_body(li, it, mem):
        UNROLL = UNROLLS[li]
        for u in range(UNROLL):
            mem = pair_body(li, it * UNROLL + u, mem)

        if li == 1:
            @pl.when(it > 0)
            def _():
                out_copy(pl.multiple_of(it * (UNROLL * PAIR) - PAIR, PAIR),
                         UNROLL * PAIR).start()

            if UNROLL > 1:
                @pl.when(it == 0)
                def _():
                    out_copy(0, (UNROLL - 1) * PAIR).start()

        return mem

    for li in range(2):
        obuf[0:PAIR, :] = jnp.zeros((PAIR, D), F32)
        rbest[...] = jnp.full((RC, 128), -jnp.inf, F32)
        ibest[...] = jnp.zeros((RC, 128), F32)
        lax.fori_loop(0, NPAIR // UNROLLS[li], functools.partial(loop_body, li),
                      mem0_v[...].astype(F32))

        if li == 0:
            for c in cp_mlp:
                c.wait()
        else:
            out_copy(0, S - PAIR).wait()

        for c in range(PAIR // RC):
            post_chunk(li, NPAIR, True, c)

        rb = rbest[...]
        rmax = jnp.max(rb, axis=0, keepdims=True)
        imin = jnp.min(jnp.where(rb == rmax, ibest[...], S - 1.0), axis=0, keepdims=True)
        idx = imin.astype(jnp.int32)[0, 0]
        row = pl.ds(PAD + idx, 1)
        lsel = lbuf[row, :]
        xs = jnp.broadcast_to(lsel, (16, D)).astype(BF16)
        gpre = _rnd(_dot(xs, wg_v[...]))
        gate = _rnd(gpre * _rnd(jax.nn.sigmoid(gpre)))
        up = _rnd(_dot(xs, wu_v[...]))
        y = _rnd(_dot((gate * up).astype(BF16), wd_v[...]))[0:1]
        rsel = _rnd(jax.nn.sigmoid(rmax[:, 0:1]))
        y = _rnd(y * rsel)
        if li == 0:
            x2 = _rnd(x1buf[row, :] + _rnd(lsel + y))
            xres[row, :] = x2
            hbuf[row, :] = _layernorm(x2)
        else:
            t0 = pl.multiple_of((idx // 16) * 16, 16)
            tile = pl.ds(PAD + t0, 16)
            sel = lax.broadcasted_iota(jnp.int32, (16, D), 0) == idx - t0
            upd = jnp.where(sel, jnp.broadcast_to(y, (16, D)), 0.0)
            ostage[tile, :] = (x1buf[tile, :] + _rnd(lbuf[tile, :] + upd)).astype(BF16)
            t1 = pl.multiple_of(jnp.minimum(t0, S - PAIR - 16), 16)
            out_copy(S - PAIR, PAIR).start()
            out_copy(t1, 16).start()
            out_copy(0, PAIR + 16).wait()


_FILL = ((0, 9), (0, 11), (0, 13), (0, 15), (1, 8), (1, 10), (1, 12), (1, 14))
CFG = dict(UNROLLS=(2, 2), LAGA=(1, 1, 2, True), LAGB=(1, 1, 1, False), FILL=(_FILL, _FILL),
           SMID=(False, True), LNP=16, LNA=16, SLACK=(128, 256))


def _build():
    any_spec = pl.BlockSpec(memory_space=pl.ANY)
    return pl.pallas_call(
        functools.partial(_kernel, **CFG),
        out_shape=jax.ShapeDtypeStruct((S, D), BF16),
        in_specs=[any_spec] * 10,
        out_specs=any_spec,
        scratch_shapes=[
            pltpu.VMEM((NPAIR + 2, PAIR, D), BF16),
            pltpu.VMEM((M, D), BF16),
            pltpu.VMEM((D,), BF16),
            pltpu.VMEM((NCH * D + 1, HC, DH), BF16),
            pltpu.VMEM((HD + 16, D), BF16),
            pltpu.VMEM((D, FF), BF16),
            pltpu.VMEM((D, FF), BF16),
            pltpu.VMEM((FF, D), BF16),
        ] + [pltpu.VMEM((GPC, D // 2, GW), U32)] * NCH + [
            pltpu.VMEM((HD // 2, D), U32),
            pltpu.VMEM((NTMP * TSZ, DH), U32),
            pltpu.VMEM((PAD + S, D), F32),
            pltpu.VMEM((PAD + S, D), F32),
            pltpu.VMEM((PAD + S, D), F32),
            pltpu.VMEM((PAD + S, D), F32),
            pltpu.VMEM((RC, 128), F32),
            pltpu.VMEM((RC, 128), F32),
            pltpu.VMEM((PAIR + 8, D), F32),
            pltpu.VMEM((PAD + S, D), BF16),
            pltpu.VMEM((8 * NPAIR, D), U32),
            pltpu.VMEM((2 * NG, 16 * NPAIR, GW), F32),
            pltpu.SMEM((4,), jnp.int32),
            pltpu.SemaphoreType.DMA((19,)),
            pltpu.SemaphoreType.DMA(()),
        ],
        compiler_params=pltpu.CompilerParams(vmem_limit_bytes=120 * 1024 * 1024),
    )


@functools.partial(jax.jit, static_argnames=("A_seg_len",))
def pallas_interleave_layers__memory_aug_recurrent_mem_tr__moe_arch_mod__prompt_kernel(
    A_x: jax.Array,
    A_mem0: jax.Array,
    A_Wq: jax.Array,
    A_Wk: jax.Array,
    A_Wv: jax.Array,
    A_Wo: jax.Array,
    A_seg_len,
    B_x: jax.Array,
    B_w_r: jax.Array,
    B_w_gate: jax.Array,
    B_w_up: jax.Array,
    B_w_down: jax.Array,
):
    assert A_seg_len == SEG and A_x.shape == (1, S, D)
    del B_x
    out = _build()(
        A_x.reshape(NPAIR, PAIR, D),
        A_mem0.reshape(M, D),
        A_Wq,
        A_Wk,
        A_Wv,
        A_Wo.reshape(HD, D),
        B_w_r,
        B_w_gate,
        B_w_up,
        B_w_down,
    )
    return out.reshape(1, S, D)
```

```python
import functools
import math

import jax
import jax.numpy as jnp
from jax import lax
import jax.experimental.pallas as pl
import jax.experimental.pallas.tpu as pltpu

F32 = jnp.float32
BF16 = jnp.bfloat16
U32 = jnp.uint32

S, D, H, DH, M, SEG = 2048, 512, 32, 128, 8, 32
FF = 1792
HD = H * DH
PAIR = 2 * SEG
NPAIR = S // PAIR
PAD = PAIR
G = 4
NG = H // G
GW = G * DH
HC = 16
GPC = HC // G
NCH = 3 * H // HC
TP = 20
TSZ = 8 * TP
NTMP = 8
RC = 8
LN_EPS = 1e-05
NEG = -1000000000.0
EXP2_SCALE = (DH ** -0.5) * math.log2(math.e)


def _rnd(x):
    return x.astype(BF16).astype(F32)


def _layernorm(x):
    mean = jnp.sum(x, axis=-1, keepdims=True) * (1.0 / D)
    c = x - mean
    var = jnp.sum(c * c, axis=-1, keepdims=True) * (1.0 / D)
    den = _rnd(jnp.sqrt(_rnd(_rnd(var) + _rnd(jnp.float32(LN_EPS)))))
    inv = 1.0 / den
    return _rnd(_rnd(x - _rnd(mean)) * inv)


def _dot(a, b):
    return jnp.dot(a, b, preferred_element_type=F32)


def _dot_nt(a, b):
    return lax.dot_general(a, b, (((1,), (1,)), ((), ())), preferred_element_type=F32)


def _softmax_bf16(s, mask):
    s = jnp.where(mask, s, NEG)
    m = jnp.max(s, axis=-1, keepdims=True)
    e = jnp.exp2((s - m) * EXP2_SCALE)
    l = jnp.sum(e, axis=-1, keepdims=True)
    r = pl.reciprocal(l, approx=True)
    r = r * (2.0 - l * r)
    return (e * r).astype(BF16)


def _kernel(x_hbm, mem0_hbm, wq_hbm, wk_hbm, wv_hbm, wo_hbm, wr_hbm, wg_hbm, wu_hbm, wd_hbm,
            out_hbm,
            x_raw, mem0_v, wr_v, stage, wo_raw, wg_v, wu_v, wd_v,
            wk0, wk1, wv0, wv1, wq0, wq1, wo, tmp,
            xres, x1buf, lbuf, hbuf, rbest, ibest, obuf, ostage,
            lhs_pre, pre, anchor, sems, osem, *,
            UNROLLS, LAGA, LAGB, FILL, SMID, LNP, LNA, SLACK, KS0):
    wch = (wk0, wk1, wv0, wv1, wq0, wq1)
    NWO = 4
    WOP = HD // NWO
    SEM_X, SEM_W, SEM_O, SEM_MISC = 0, 3, 3 + NCH + 1, 3 + NCH + 1 + NWO

    def cp_x(i):
        r0, nr = ((24, 16), (0, 24), (40, 24))[i]
        return pltpu.make_async_copy(x_hbm.at[:, pl.ds(r0, nr), :],
                                     x_raw.at[pl.ds(1, NPAIR), pl.ds(r0, nr), :],
                                     sems.at[SEM_X + i])

    def cp_w(c, half=None):
        w = (wk_hbm, wv_hbm, wq_hbm)[c // 2]
        heads = pl.ds((c % 2) * HC, HC)
        if half is None:
            return pltpu.make_async_copy(w.at[:, heads, :], stage.at[pl.ds(c * D, D)],
                                         sems.at[SEM_W + 1 + c])
        return pltpu.make_async_copy(w.at[pl.ds(half * (D // 2), D // 2), heads, :],
                                     stage.at[pl.ds(c * D + half * (D // 2), D // 2)],
                                     sems.at[SEM_W + half])

    def cp_o(i):
        return pltpu.make_async_copy(wo_hbm.at[pl.ds(i * WOP, WOP)],
                                     wo_raw.at[pl.ds(i * WOP, WOP)], sems.at[SEM_O + i])

    cp_small = [pltpu.make_async_copy(s_, d_, sems.at[SEM_MISC + i])
                for i, (s_, d_) in enumerate(((mem0_hbm, mem0_v), (wr_hbm, wr_v)))]
    cp_mlp = [pltpu.make_async_copy(s_, d_, sems.at[SEM_MISC + 2 + i])
              for i, (s_, d_) in enumerate(((wg_hbm, wg_v), (wu_hbm, wu_v), (wd_hbm, wd_v)))]
    cp_x(0).start()
    cp_w(0, 0).start()
    cp_w(0, 1).start()
    cp_w(1).start()
    cp_w(2).start()
    cp_x(1).start()
    cp_x(2).start()
    for c in range(3, NCH):
        cp_w(c).start()
    for i in range(NWO):
        cp_o(i).start()
    for c in cp_small + cp_mlp:
        c.start()

    anchor[0] = PAIR
    anchor[1] = NCH * D
    anchor[2] = HD
    anchor[3] = NPAIR + 1
    x_raw[0] = jnp.zeros((PAIR, D), BF16)
    xres[0:PAD, :] = jnp.zeros((PAD, D), F32)

    cp_x(0).wait()

    def ln_mid(i, carry):
        for pp in range(LNP):
            pr = i * LNP + pp
            ln = _layernorm(x_raw[1 + pr, 24:40, :].astype(F32))
            hbuf[pl.ds(pl.multiple_of(PAD + pr * PAIR + 24, 8), 16), :] = ln
            lhs_pre[pl.ds(pl.multiple_of(pr * 8, 8), 8), :] = pltpu.bitcast(ln.astype(BF16), U32)
        return carry

    lax.fori_loop(0, NPAIR // LNP, ln_mid, 0)

    def ln_jobs(p0, npairs):
        def job(pp, r0):
            ln = _layernorm(x_raw[1 + p0 + pp, r0:r0 + 8, :].astype(F32))
            hbuf[pl.ds(pl.multiple_of(PAD + (p0 + pp) * PAIR + r0, 8), 8), :] = ln

        return [('x_raw', functools.partial(job, pp, r0))
                for pp in range(npairs) for r0 in (0, 8, 16, 40, 48, 56)]

    def relayout_jobs(c, blk0, nblk, slot0=0):
        def job(u):
            t0 = ((slot0 + u) % NTMP) * TSZ
            d0 = pl.multiple_of(c * D + (blk0 + u) * 16, 16)
            raw = pltpu.bitcast(stage[pl.ds(d0, 16), :, :], U32)
            for i in range(8):
                ev, od = raw[2 * i], raw[2 * i + 1]
                lo = (ev & jnp.uint32(0xFFFF)) | (od << 16)
                hi = (ev >> 16) | (od & jnp.uint32(0xFFFF0000))
                tmp[pl.ds(t0 + i * TP, 8, stride=2), :] = lo
                tmp[pl.ds(t0 + i * TP + 1, 8, stride=2), :] = hi
            o0 = pl.multiple_of((blk0 + u) * 8, 8)
            for hh in range(HC):
                col = (hh % G) * DH
                wch[c][hh // G, pl.ds(o0, 8), col:col + DH] = tmp[pl.ds(t0 + hh, 8, stride=TP), :]

        return [('stage', functools.partial(job, u)) for u in range(nblk)]

    def repack_jobs(part):
        def job(c):
            r0 = pl.multiple_of(part * WOP + c * 128, 128)
            o0 = pl.multiple_of(part * (WOP // 2) + c * 64, 64)
            wo[pl.ds(o0, 64), :] = pltpu.bitcast(wo_raw[pl.ds(r0, 128), :], U32)

        return [('wo_raw', functools.partial(job, c)) for c in range(WOP // 128)]

    def interleave(*lists):
        keyed = [((i + 0.5) / len(l), n, j) for n, l in enumerate(lists) for i, j in enumerate(l)]
        return [j for _, _, j in sorted(keyed, key=lambda t: t[:2])]

    def precompute(c, g0, ng, jobs):
        lhs = pltpu.bitcast(lhs_pre[...], BF16)
        ys = [_dot(lhs, pltpu.bitcast(wch[c][g0 + gg], BF16)) for gg in range(ng)]
        nrow = 16 * NPAIR
        has_ln = any(kind == 'x_raw' for kind, _ in jobs)
        for u, (kind, job) in enumerate(jobs):
            if u > 0:
                span = ng * G * nrow - (SLACK[1] if has_ln else SLACK[0])
                pos = max((u * span // len(jobs)) // 16 * 16 - 128, 0)
                nt, r0 = pos // nrow, pos % nrow
                tie = ys[nt // G][r0:r0 + 16, (nt % G) * DH:(nt % G + 1) * DH].astype(BF16)
                if kind == 'stage':
                    stage[anchor[1]] = tie
                elif kind == 'x_raw':
                    x_raw[anchor[3], 0:16, 0:DH] = tie
                else:
                    wo_raw[pl.ds(pl.multiple_of(anchor[2], 16), 16), 0:DH] = tie
            job()
        for gg in range(ng):
            pre[c * GPC + g0 + gg] = ys[gg]

    def run(jobs):
        for _, job in jobs:
            job()

    NBLK = D // 16

    def relay0(it, carry):
        @pl.when(it % 2 == 0)
        def _():
            cp_w(0, it // 2).wait()
        run(relayout_jobs(0, it * 8, 8))
        return carry

    lax.fori_loop(0, NBLK // 8, relay0, 0)
    lax.fori_loop(0, 2, lambda it, cr: (precompute(0, it, 1, []), cr)[1], 0)
    cp_w(1).wait()
    lax.fori_loop(0, 2, lambda it, cr: (
        precompute(0, 2 + it, 1, relayout_jobs(1, it * (NBLK // 2), NBLK // 2)), cr)[1], 0)

    HB, QB = NBLK // 2, NBLK // 4
    cp_w(2).wait()
    lax.fori_loop(0, 2, lambda it, cr: (
        precompute(1, it * 2, 2, relayout_jobs(2, it * HB, HB)), cr)[1], 0)
    cp_x(1).wait()
    cp_x(2).wait()
    cp_w(3).wait()
    lax.fori_loop(0, 2, lambda it, cr: (
        precompute(2, it * 2, 2, interleave(relayout_jobs(3, it * HB, HB),
                                            ln_jobs(it * LNA, LNA))), cr)[1], 0)
    cp_w(4).wait()
    cp_w(5).wait()
    LNB = (NPAIR - 2 * LNA) // 4

    def last_phase(it, carry):
        cp_o(it).wait()
        precompute(3, it, 1, interleave(relayout_jobs(4, it * QB, QB),
                                        relayout_jobs(5, it * QB, QB, NTMP // 2),
                                        repack_jobs(it),
                                        ln_jobs(2 * LNA + it * LNB, LNB)))
        return carry

    lax.fori_loop(0, 4, last_phase, 0)

    for c in cp_small:
        c.wait()
    wr = wr_v[...].astype(F32).reshape(1, D)

    qi = lax.broadcasted_iota(jnp.int32, (32, 48), 0)
    kj = lax.broadcasted_iota(jnp.int32, (32, 48), 1)
    mask_a = (kj < 40) & ((qi < M) | (kj <= qi))
    qi = lax.broadcasted_iota(jnp.int32, (48, 80), 0)
    kj = lax.broadcasted_iota(jnp.int32, (48, 80), 1)
    kb0 = (kj >= 40) & (kj < 48)
    m_mem = (qi < M) & ((kj < 32) | kb0)
    m_xb = (qi >= M) & (qi < 32) & ((kj <= qi) | kb0)
    m_xa = (qi >= 32) & (qi < 40) & ((kj >= 48) | ((kj >= 32) & (kj <= qi)))
    m_b0 = (qi >= 40) & ((kj < M) | (kb0 & (kj <= qi)))
    mask_b = m_mem | m_xb | m_xa | m_b0

    def w_ref(mi, g):
        return wch[(4, 0, 2)[mi] + g // GPC].at[g % GPC]

    def wo_rows(g, n=1):
        r0 = g * GW // 2
        return pltpu.bitcast(wo[r0:r0 + n * GW // 2, :], BF16)

    def seg_step(lhs, lhs_f32, extra, mask, lags, s_mid, filler):
        q, k, v, p, o = {}, {}, {}, {}, {}
        raw = ({}, {}, {})
        acc = [None]

        def proj(mi, g, dst):
            if mi == 0 and g == 0 and lhs_f32 is not None:
                y = None
                lp = jnp.concatenate([lhs_f32[16:], lhs_f32[0:16]], axis=0)
                for kt in range(D // 128):
                    w = pltpu.bitcast(w_ref(0, 0)[kt * 64:(kt + 1) * 64, :], BF16)
                    t = _dot(lp[:, kt * 128:(kt + 1) * 128].astype(BF16), w)
                    y = t if y is None else y + t
                nr = y.shape[0]
                y = jnp.concatenate([y[nr - 16:], y[0:nr - 16]], axis=0)
            else:
                y = _dot(lhs[mi], pltpu.bitcast(w_ref(mi, g)[...], BF16))
            for j in range(G):
                h = g * G + j
                yh = y[:, j * DH:(j + 1) * DH]
                ex = extra(mi, h)
                if ex:
                    yh = jnp.concatenate([yh] + ex, axis=0)
                raw[mi][h] = yh
                dst[h] = yh.astype(BF16)

        def sc(g):
            for h in range(g * G, (g + 1) * G):
                p[h] = _softmax_bf16(_dot_nt(q[h], k[h]), mask)

        def pv(g):
            o[g] = jnp.concatenate(
                [_dot(p[h], v[h]) for h in range(g * G, (g + 1) * G)], axis=1)

        def op(g):
            if merge and g == NG - 2:
                return
            if merge and g == NG - 1:
                y = _dot(jnp.concatenate([o[g - 1], o[g]], axis=1).astype(BF16),
                         wo_rows(g - 1, 2))
            else:
                y = _dot(o[g].astype(BF16), wo_rows(g))
            acc[0] = y if acc[0] is None else acc[0] + y

        ls, lp, lo, merge, pv0 = lags
        for t in range(2 * NG + lp + lo):
            if t < NG:
                proj(0, t, q)
                if s_mid and 0 <= t - ls < NG:
                    sc(t - ls)
                proj(1, t, k)
            elif t < 2 * NG:
                proj(2, t - NG, v)
            if 0 <= t - ls < NG and not s_mid:
                sc(t - ls)
            if t == NG + lp + pv0:
                pv(0)
                if s_mid:
                    for g in range(NG - ls, NG):
                        sc(g)
            if 0 < t - NG - lp < NG:
                pv(t - NG - lp)
            if pv0 > lo - 1 and t == NG + lp + lo + 1:
                op(0)
            if (1 if pv0 > lo - 1 else 0) <= t - NG - lp - lo < NG:
                op(t - NG - lp - lo)
            if t in filler:
                src = raw[1][t * G] if t < NG else raw[2][min(t - NG, NG - 1) * G]
                filler[t](src[0:8])
        return acc[0], raw

    subr = lax.broadcasted_iota(jnp.int32, (RC, 128), 0).astype(F32)

    def post_chunk(li, pi, valid, c, tie=None):
        if tie is not None:
            obuf[pl.ds(pl.multiple_of(anchor[0], 8), 8), 0:DH] = tie
        base = pi * PAIR if isinstance(pi, int) else pl.multiple_of(pi * PAIR, PAIR)
        rows = pl.ds(base + c * RC, RC)
        x0 = x_raw[pi, c * RC:(c + 1) * RC, :].astype(F32) if li == 0 else xres[rows, :]
        x1 = _rnd(x0 + _rnd(obuf[c * RC:(c + 1) * RC, :]))
        ln = _layernorm(x1)
        r = _rnd(jnp.sum(ln * wr, axis=-1, keepdims=True))
        r = jnp.broadcast_to(jnp.where(valid, r, -jnp.inf), (RC, 128))
        rb = rbest[...]
        better = r > rb
        rbest[...] = jnp.where(better, r, rb)
        row0 = jnp.asarray(base + (c * RC - PAD), jnp.int32).astype(F32)
        ibest[...] = jnp.where(better, subr + row0, ibest[...])
        x1buf[rows, :] = x1
        lbuf[rows, :] = ln
        if li == 0:
            x2 = _rnd(x1 + ln)
            xres[rows, :] = x2
            hbuf[rows, :] = _layernorm(x2)
        else:
            ostage[rows, :] = (x1 + ln).astype(BF16)

    def out_copy(row0, nrows):
        return pltpu.make_async_copy(ostage.at[pl.ds(PAD + row0, nrows)],
                                     out_hbm.at[pl.ds(row0, nrows)], osem)

    def pair_body(li, pi, mem, first):
        base = pl.multiple_of(pi * PAIR, PAIR)
        ha = hbuf[pl.ds(base + PAD, 40), :]
        hb = hbuf[pl.ds(base + PAD + 40, 24), :]
        fill = ({}, {})
        for c, (st, t) in enumerate(FILL[li]):
            fill[st][t] = functools.partial(post_chunk, li, pi, pi > 0, c)
        aq = jnp.concatenate([mem, ha[0:24]], axis=0)
        lhs_aq = aq.astype(BF16)
        if li == 0:
            p0 = pl.multiple_of(pi * 16, 16)
            lhs_akv = lhs_aq
            extra_a = lambda mi, h: [pre[(mi - 1) * NG + h // G, pl.ds(p0, 16),
                                         (h % G) * DH:(h % G + 1) * DH]] if mi else []
        else:
            lhs_akv = jnp.concatenate([mem, ha], axis=0).astype(BF16)
            extra_a = lambda mi, h: []
        acc_a, prj = seg_step((lhs_aq, lhs_akv, lhs_akv), None if first else aq, extra_a, mask_a,
                              LAGA, SMID[0], fill[0])
        lhs_b = jnp.concatenate([acc_a[0:8], hb], axis=0).astype(BF16)
        bq = jnp.concatenate([acc_a[0:8], hb, ha[24:40]], axis=0)
        acc_b, _ = seg_step(
            (bq.astype(BF16), lhs_b, lhs_b), bq,
            lambda mi, h: [prj[mi][h][32:48], prj[mi][h][0:32]] if mi else [],
            mask_b, LAGB, SMID[1], fill[1])
        obuf[0:24, :] = acc_a[8:32]
        obuf[24:40, :] = acc_b[32:48]
        obuf[40:64, :] = acc_b[8:32]
        return acc_b[0:8]

    def loop_body(li, it, mem):
        UNROLL = UNROLLS[li]
        for u in range(UNROLL):
            mem = pair_body(li, it * UNROLL + u, mem, u == 0 and not KS0)

        if li == 1:
            @pl.when(it > 0)
            def _():
                out_copy(pl.multiple_of(it * (UNROLL * PAIR) - PAIR, PAIR),
                         UNROLL * PAIR).start()

            if UNROLL > 1:
                @pl.when(it == 0)
                def _():
                    out_copy(0, (UNROLL - 1) * PAIR).start()

        return mem

    for li in range(2):
        obuf[0:PAIR, :] = jnp.zeros((PAIR, D), F32)
        rbest[...] = jnp.full((RC, 128), -jnp.inf, F32)
        ibest[...] = jnp.zeros((RC, 128), F32)
        lax.fori_loop(0, NPAIR // UNROLLS[li], functools.partial(loop_body, li),
                      mem0_v[...].astype(F32))

        if li == 0:
            for c in cp_mlp:
                c.wait()
        else:
            out_copy(0, S - PAIR).wait()

        for c in range(PAIR // RC):
            post_chunk(li, NPAIR, True, c)

        rb = rbest[...]
        rmax = jnp.max(rb, axis=0, keepdims=True)
        imin = jnp.min(jnp.where(rb == rmax, ibest[...], S - 1.0), axis=0, keepdims=True)
        idx = imin.astype(jnp.int32)[0, 0]
        row = pl.ds(PAD + idx, 1)
        lsel = lbuf[row, :]
        xs = jnp.broadcast_to(lsel, (16, D)).astype(BF16)
        gpre = _rnd(_dot(xs, wg_v[...]))
        gate = _rnd(gpre * _rnd(jax.nn.sigmoid(gpre)))
        up = _rnd(_dot(xs, wu_v[...]))
        y = _rnd(_dot((gate * up).astype(BF16), wd_v[...]))[0:1]
        rsel = _rnd(jax.nn.sigmoid(rmax[:, 0:1]))
        y = _rnd(y * rsel)
        if li == 0:
            x2 = _rnd(x1buf[row, :] + _rnd(lsel + y))
            xres[row, :] = x2
            hbuf[row, :] = _layernorm(x2)
        else:
            t0 = pl.multiple_of((idx // 16) * 16, 16)
            tile = pl.ds(PAD + t0, 16)
            sel = lax.broadcasted_iota(jnp.int32, (16, D), 0) == idx - t0
            upd = jnp.where(sel, jnp.broadcast_to(y, (16, D)), 0.0)
            ostage[tile, :] = (x1buf[tile, :] + _rnd(lbuf[tile, :] + upd)).astype(BF16)
            t1 = pl.multiple_of(jnp.minimum(t0, S - PAIR - 16), 16)
            out_copy(S - PAIR, PAIR).start()
            out_copy(t1, 16).start()
            out_copy(0, PAIR + 16).wait()


_FILL = ((0, 9), (0, 11), (0, 13), (0, 15), (1, 9), (1, 11), (1, 13), (1, 14))
CFG = dict(UNROLLS=(2, 2), LAGA=(1, 1, 2, True, 0), LAGB=(1, 1, 2, False, 1), FILL=(_FILL, _FILL),
           SMID=(False, True), LNP=16, LNA=16, SLACK=(128, 256), KS0=False)


def _build():
    any_spec = pl.BlockSpec(memory_space=pl.ANY)
    return pl.pallas_call(
        functools.partial(_kernel, **CFG),
        out_shape=jax.ShapeDtypeStruct((S, D), BF16),
        in_specs=[any_spec] * 10,
        out_specs=any_spec,
        scratch_shapes=[
            pltpu.VMEM((NPAIR + 2, PAIR, D), BF16),
            pltpu.VMEM((M, D), BF16),
            pltpu.VMEM((D,), BF16),
            pltpu.VMEM((NCH * D + 1, HC, DH), BF16),
            pltpu.VMEM((HD + 16, D), BF16),
            pltpu.VMEM((D, FF), BF16),
            pltpu.VMEM((D, FF), BF16),
            pltpu.VMEM((FF, D), BF16),
        ] + [pltpu.VMEM((GPC, D // 2, GW), U32)] * NCH + [
            pltpu.VMEM((HD // 2, D), U32),
            pltpu.VMEM((NTMP * TSZ, DH), U32),
            pltpu.VMEM((PAD + S, D), F32),
            pltpu.VMEM((PAD + S, D), F32),
            pltpu.VMEM((PAD + S, D), F32),
            pltpu.VMEM((PAD + S, D), F32),
            pltpu.VMEM((RC, 128), F32),
            pltpu.VMEM((RC, 128), F32),
            pltpu.VMEM((PAIR + 8, D), F32),
            pltpu.VMEM((PAD + S, D), BF16),
            pltpu.VMEM((8 * NPAIR, D), U32),
            pltpu.VMEM((2 * NG, 16 * NPAIR, GW), F32),
            pltpu.SMEM((4,), jnp.int32),
            pltpu.SemaphoreType.DMA((19,)),
            pltpu.SemaphoreType.DMA(()),
        ],
        compiler_params=pltpu.CompilerParams(vmem_limit_bytes=120 * 1024 * 1024),
    )


@functools.partial(jax.jit, static_argnames=("A_seg_len",))
def pallas_interleave_layers__memory_aug_recurrent_mem_tr__moe_arch_mod__prompt_kernel(
    A_x: jax.Array,
    A_mem0: jax.Array,
    A_Wq: jax.Array,
    A_Wk: jax.Array,
    A_Wv: jax.Array,
    A_Wo: jax.Array,
    A_seg_len,
    B_x: jax.Array,
    B_w_r: jax.Array,
    B_w_gate: jax.Array,
    B_w_up: jax.Array,
    B_w_down: jax.Array,
):
    assert A_seg_len == SEG and A_x.shape == (1, S, D)
    del B_x
    out = _build()(
        A_x.reshape(NPAIR, PAIR, D),
        A_mem0.reshape(M, D),
        A_Wq,
        A_Wk,
        A_Wv,
        A_Wo.reshape(HD, D),
        B_w_r,
        B_w_gate,
        B_w_up,
        B_w_down,
    )
    return out.reshape(1, S, D)
```

```python
import functools
import math

import jax
import jax.numpy as jnp
from jax import lax
import jax.experimental.pallas as pl
import jax.experimental.pallas.tpu as pltpu

F32 = jnp.float32
BF16 = jnp.bfloat16
U32 = jnp.uint32

S, D, H, DH, M, SEG = 2048, 512, 32, 128, 8, 32
FF = 1792
HD = H * DH
PAIR = 2 * SEG
NPAIR = S // PAIR
PAD = PAIR
G = 4
NG = H // G
GW = G * DH
HC = 16
GPC = HC // G
NCH = 3 * H // HC
TP = 20
TSZ = 8 * TP
NTMP = 8
FSPLIT = ((0, 1024), (1024, FF))
RC = 8
LN_EPS = 1e-05
NEG = -1000000000.0
EXP2_SCALE = (DH ** -0.5) * math.log2(math.e)


def _rnd(x):
    return x.astype(BF16).astype(F32)


def _layernorm(x):
    mean = jnp.sum(x, axis=-1, keepdims=True) * (1.0 / D)
    c = x - mean
    var = jnp.sum(c * c, axis=-1, keepdims=True) * (1.0 / D)
    den = _rnd(jnp.sqrt(_rnd(_rnd(var) + _rnd(jnp.float32(LN_EPS)))))
    inv = 1.0 / den
    return _rnd(_rnd(x - _rnd(mean)) * inv)


def _dot(a, b):
    return jnp.dot(a, b, preferred_element_type=F32)


def _dot_nt(a, b):
    return lax.dot_general(a, b, (((1,), (1,)), ((), ())), preferred_element_type=F32)


def _softmax_bf16(s, mask):
    s = jnp.where(mask, s, NEG)
    m = jnp.max(s, axis=-1, keepdims=True)
    e = jnp.exp2((s - m) * EXP2_SCALE)
    l = jnp.sum(e, axis=-1, keepdims=True)
    r = pl.reciprocal(l, approx=True)
    r = r * (2.0 - l * r)
    return (e * r).astype(BF16)


def _kernel(x_hbm, mem0_hbm, wq_hbm, wk_hbm, wv_hbm, wo_hbm, wr_hbm, wg_hbm, wu_hbm, wd_hbm,
            out_hbm,
            x_raw, mem0_v, wr_v, stage, wo_raw, wg_v, wu_v, wd_v,
            wk0, wk1, wv0, wv1, wq0, wq1, wo, tmp,
            xres, x1buf, lbuf, hbuf, rbest, ibest, obuf, ostage,
            lhs_pre, pre, ybuf, anchor, sems, osem, *,
            UNROLLS, LAGA, LAGB, FILL, SMID, LNP, LNA, SLACK, KS0):
    wch = (wk0, wk1, wv0, wv1, wq0, wq1)
    NWO = 4
    WOP = HD // NWO
    SEM_X, SEM_W, SEM_O, SEM_MISC = 0, 3, 3 + NCH + 1, 3 + NCH + 1 + NWO

    def cp_x(i):
        r0, nr = ((24, 16), (0, 24), (40, 24))[i]
        return pltpu.make_async_copy(x_hbm.at[:, pl.ds(r0, nr), :],
                                     x_raw.at[pl.ds(1, NPAIR), pl.ds(r0, nr), :],
                                     sems.at[SEM_X + i])

    def cp_w(c, half=None):
        w = (wk_hbm, wv_hbm, wq_hbm)[c // 2]
        heads = pl.ds((c % 2) * HC, HC)
        if half is None:
            return pltpu.make_async_copy(w.at[:, heads, :], stage.at[pl.ds(c * D, D)],
                                         sems.at[SEM_W + 1 + c])
        return pltpu.make_async_copy(w.at[pl.ds(half * (D // 2), D // 2), heads, :],
                                     stage.at[pl.ds(c * D + half * (D // 2), D // 2)],
                                     sems.at[SEM_W + half])

    def cp_o(i):
        return pltpu.make_async_copy(wo_hbm.at[pl.ds(i * WOP, WOP)],
                                     wo_raw.at[pl.ds(i * WOP, WOP)], sems.at[SEM_O + i])

    cp_small = [pltpu.make_async_copy(s_, d_, sems.at[SEM_MISC + i])
                for i, (s_, d_) in enumerate(((mem0_hbm, mem0_v), (wr_hbm, wr_v)))]
    cp_mlp = [pltpu.make_async_copy(s_, d_, sems.at[SEM_MISC + 2 + i])
              for i, (s_, d_) in enumerate(((wg_hbm, wg_v), (wu_hbm, wu_v), (wd_hbm, wd_v)))]
    cp_x(0).start()
    cp_w(0, 0).start()
    cp_w(0, 1).start()
    cp_w(1).start()
    cp_w(2).start()
    cp_x(1).start()
    cp_x(2).start()
    for c in range(3, NCH):
        cp_w(c).start()
    for i in range(NWO):
        cp_o(i).start()
    for c in cp_small + cp_mlp:
        c.start()

    anchor[0] = PAIR
    anchor[1] = NCH * D
    anchor[2] = HD
    anchor[3] = NPAIR + 1
    x_raw[0] = jnp.zeros((PAIR, D), BF16)
    xres[0:PAD, :] = jnp.zeros((PAD, D), F32)

    cp_x(0).wait()

    def ln_mid(i, carry):
        for pp in range(LNP):
            pr = i * LNP + pp
            ln = _layernorm(x_raw[1 + pr, 24:40, :].astype(F32))
            hbuf[pl.ds(pl.multiple_of(PAD + pr * PAIR + 24, 8), 16), :] = ln
            lhs_pre[pl.ds(pl.multiple_of(pr * 8, 8), 8), :] = pltpu.bitcast(ln.astype(BF16), U32)
        return carry

    lax.fori_loop(0, NPAIR // LNP, ln_mid, 0)

    def ln_jobs(p0, npairs):
        def job(pp, r0):
            ln = _layernorm(x_raw[1 + p0 + pp, r0:r0 + 8, :].astype(F32))
            hbuf[pl.ds(pl.multiple_of(PAD + (p0 + pp) * PAIR + r0, 8), 8), :] = ln

        return [('x_raw', functools.partial(job, pp, r0))
                for pp in range(npairs) for r0 in (0, 8, 16, 40, 48, 56)]

    def relayout_jobs(c, blk0, nblk, slot0=0):
        def job(u):
            t0 = ((slot0 + u) % NTMP) * TSZ
            d0 = pl.multiple_of(c * D + (blk0 + u) * 16, 16)
            raw = pltpu.bitcast(stage[pl.ds(d0, 16), :, :], U32)
            for i in range(8):
                ev, od = raw[2 * i], raw[2 * i + 1]
                lo = (ev & jnp.uint32(0xFFFF)) | (od << 16)
                hi = (ev >> 16) | (od & jnp.uint32(0xFFFF0000))
                tmp[pl.ds(t0 + i * TP, 8, stride=2), :] = lo
                tmp[pl.ds(t0 + i * TP + 1, 8, stride=2), :] = hi
            o0 = pl.multiple_of((blk0 + u) * 8, 8)
            for hh in range(HC):
                col = (hh % G) * DH
                wch[c][hh // G, pl.ds(o0, 8), col:col + DH] = tmp[pl.ds(t0 + hh, 8, stride=TP), :]

        return [('stage', functools.partial(job, u)) for u in range(nblk)]

    def repack_jobs(part):
        def job(c):
            r0 = pl.multiple_of(part * WOP + c * 128, 128)
            o0 = pl.multiple_of(part * (WOP // 2) + c * 64, 64)
            wo[pl.ds(o0, 64), :] = pltpu.bitcast(wo_raw[pl.ds(r0, 128), :], U32)

        return [('wo_raw', functools.partial(job, c)) for c in range(WOP // 128)]

    def interleave(*lists):
        keyed = [((i + 0.5) / len(l), n, j) for n, l in enumerate(lists) for i, j in enumerate(l)]
        return [j for _, _, j in sorted(keyed, key=lambda t: t[:2])]

    def precompute(c, g0, ng, jobs):
        lhs = pltpu.bitcast(lhs_pre[...], BF16)
        ys = [_dot(lhs, pltpu.bitcast(wch[c][g0 + gg], BF16)) for gg in range(ng)]
        nrow = 16 * NPAIR
        has_ln = any(kind == 'x_raw' for kind, _ in jobs)
        for u, (kind, job) in enumerate(jobs):
            if u > 0:
                span = ng * G * nrow - (SLACK[1] if has_ln else SLACK[0])
                pos = max((u * span // len(jobs)) // 16 * 16 - 128, 0)
                nt, r0 = pos // nrow, pos % nrow
                tie = ys[nt // G][r0:r0 + 16, (nt % G) * DH:(nt % G + 1) * DH].astype(BF16)
                if kind == 'stage':
                    stage[anchor[1]] = tie
                elif kind == 'x_raw':
                    x_raw[anchor[3], 0:16, 0:DH] = tie
                else:
                    wo_raw[pl.ds(pl.multiple_of(anchor[2], 16), 16), 0:DH] = tie
            job()
        for gg in range(ng):
            pre[c * GPC + g0 + gg] = ys[gg]

    def run(jobs):
        for _, job in jobs:
            job()

    NBLK = D // 16

    def relay0(it, carry):
        @pl.when(it % 2 == 0)
        def _():
            cp_w(0, it // 2).wait()
        run(relayout_jobs(0, it * 8, 8))
        return carry

    lax.fori_loop(0, NBLK // 8, relay0, 0)
    lax.fori_loop(0, 2, lambda it, cr: (precompute(0, it, 1, []), cr)[1], 0)
    cp_w(1).wait()
    lax.fori_loop(0, 2, lambda it, cr: (
        precompute(0, 2 + it, 1, relayout_jobs(1, it * (NBLK // 2), NBLK // 2)), cr)[1], 0)

    HB, QB = NBLK // 2, NBLK // 4
    cp_w(2).wait()
    lax.fori_loop(0, 2, lambda it, cr: (
        precompute(1, it * 2, 2, relayout_jobs(2, it * HB, HB)), cr)[1], 0)
    cp_x(1).wait()
    cp_x(2).wait()
    cp_w(3).wait()
    lax.fori_loop(0, 2, lambda it, cr: (
        precompute(2, it * 2, 2, interleave(relayout_jobs(3, it * HB, HB),
                                            ln_jobs(it * LNA, LNA))), cr)[1], 0)
    cp_w(4).wait()
    cp_w(5).wait()
    LNB = (NPAIR - 2 * LNA) // 4

    def last_phase(it, carry):
        cp_o(it).wait()
        precompute(3, it, 1, interleave(relayout_jobs(4, it * QB, QB),
                                        relayout_jobs(5, it * QB, QB, NTMP // 2),
                                        repack_jobs(it),
                                        ln_jobs(2 * LNA + it * LNB, LNB)))
        return carry

    lax.fori_loop(0, 4, last_phase, 0)

    for c in cp_small:
        c.wait()
    wr = wr_v[...].astype(F32).reshape(1, D)

    qi = lax.broadcasted_iota(jnp.int32, (32, 48), 0)
    kj = lax.broadcasted_iota(jnp.int32, (32, 48), 1)
    mask_a = (kj < 40) & ((qi < M) | (kj <= qi))
    qi = lax.broadcasted_iota(jnp.int32, (48, 80), 0)
    kj = lax.broadcasted_iota(jnp.int32, (48, 80), 1)
    kb0 = (kj >= 40) & (kj < 48)
    m_mem = (qi < M) & ((kj < 32) | kb0)
    m_xb = (qi >= M) & (qi < 32) & ((kj <= qi) | kb0)
    m_xa = (qi >= 32) & (qi < 40) & ((kj >= 48) | ((kj >= 32) & (kj <= qi)))
    m_b0 = (qi >= 40) & ((kj < M) | (kb0 & (kj <= qi)))
    mask_b = m_mem | m_xb | m_xa | m_b0

    def w_ref(mi, g):
        return wch[(4, 0, 2)[mi] + g // GPC].at[g % GPC]

    def wo_rows(g, n=1):
        r0 = g * GW // 2
        return pltpu.bitcast(wo[r0:r0 + n * GW // 2, :], BF16)

    def seg_step(lhs, lhs_f32, extra, mask, lags, s_mid, filler):
        q, k, v, p, o = {}, {}, {}, {}, {}
        raw = ({}, {}, {})
        acc = [None]

        def proj(mi, g, dst):
            if mi == 0 and g == 0 and lhs_f32 is not None:
                y = None
                lp = jnp.concatenate([lhs_f32[16:], lhs_f32[0:16]], axis=0)
                for kt in range(D // 128):
                    w = pltpu.bitcast(w_ref(0, 0)[kt * 64:(kt + 1) * 64, :], BF16)
                    t = _dot(lp[:, kt * 128:(kt + 1) * 128].astype(BF16), w)
                    y = t if y is None else y + t
                nr = y.shape[0]
                y = jnp.concatenate([y[nr - 16:], y[0:nr - 16]], axis=0)
            else:
                y = _dot(lhs[mi], pltpu.bitcast(w_ref(mi, g)[...], BF16))
            for j in range(G):
                h = g * G + j
                yh = y[:, j * DH:(j + 1) * DH]
                ex = extra(mi, h)
                if ex:
                    yh = jnp.concatenate([yh] + ex, axis=0)
                raw[mi][h] = yh
                dst[h] = yh.astype(BF16)

        def sc(g):
            for h in range(g * G, (g + 1) * G):
                p[h] = _softmax_bf16(_dot_nt(q[h], k[h]), mask)

        def pv(g):
            o[g] = jnp.concatenate(
                [_dot(p[h], v[h]) for h in range(g * G, (g + 1) * G)], axis=1)

        def op(g):
            if merge and g == NG - 2:
                return
            if merge and g == NG - 1:
                y = _dot(jnp.concatenate([o[g - 1], o[g]], axis=1).astype(BF16),
                         wo_rows(g - 1, 2))
            else:
                y = _dot(o[g].astype(BF16), wo_rows(g))
            acc[0] = y if acc[0] is None else acc[0] + y

        ls, lp, lo, merge, pv0 = lags
        for t in range(2 * NG + lp + lo):
            if t < NG:
                proj(0, t, q)
                if s_mid and 0 <= t - ls < NG:
                    sc(t - ls)
                proj(1, t, k)
            elif t < 2 * NG:
                proj(2, t - NG, v)
            if 0 <= t - ls < NG and not s_mid:
                sc(t - ls)
            if t == NG + lp + pv0:
                pv(0)
                if s_mid:
                    for g in range(NG - ls, NG):
                        sc(g)
            if 0 < t - NG - lp < NG:
                pv(t - NG - lp)
            if pv0 > lo - 1 and t == NG + lp + lo + 1:
                op(0)
            if (1 if pv0 > lo - 1 else 0) <= t - NG - lp - lo < NG:
                op(t - NG - lp - lo)
            if t in filler:
                src = raw[1][t * G] if t < NG else raw[2][min(t - NG, NG - 1) * G]
                filler[t](src[0:8])
        return acc[0], raw

    subr = lax.broadcasted_iota(jnp.int32, (RC, 128), 0).astype(F32)

    def post_chunk(li, pi, valid, c, tie=None):
        if tie is not None:
            obuf[pl.ds(pl.multiple_of(anchor[0], 8), 8), 0:DH] = tie
        base = pi * PAIR if isinstance(pi, int) else pl.multiple_of(pi * PAIR, PAIR)
        rows = pl.ds(base + c * RC, RC)
        x0 = x_raw[pi, c * RC:(c + 1) * RC, :].astype(F32) if li == 0 else xres[rows, :]
        x1 = _rnd(x0 + _rnd(obuf[c * RC:(c + 1) * RC, :]))
        ln = _layernorm(x1)
        r = _rnd(jnp.sum(ln * wr, axis=-1, keepdims=True))
        r = jnp.broadcast_to(jnp.where(valid, r, -jnp.inf), (RC, 128))
        rb = rbest[...]
        better = r > rb
        rbest[...] = jnp.where(better, r, rb)
        row0 = jnp.asarray(base + (c * RC - PAD), jnp.int32).astype(F32)
        ibest[...] = jnp.where(better, subr + row0, ibest[...])
        x1buf[rows, :] = x1
        lbuf[rows, :] = ln
        if li == 0:
            x2 = _rnd(x1 + ln)
            xres[rows, :] = x2
            hbuf[rows, :] = _layernorm(x2)
        else:
            ostage[rows, :] = (x1 + ln).astype(BF16)

    def out_copy(row0, nrows):
        return pltpu.make_async_copy(ostage.at[pl.ds(PAD + row0, nrows)],
                                     out_hbm.at[pl.ds(row0, nrows)], osem)

    def pair_body(li, pi, mem, first):
        base = pl.multiple_of(pi * PAIR, PAIR)
        ha = hbuf[pl.ds(base + PAD, 40), :]
        hb = hbuf[pl.ds(base + PAD + 40, 24), :]
        fill = ({}, {})
        for c, (st, t) in enumerate(FILL[li]):
            fill[st][t] = functools.partial(post_chunk, li, pi, pi > 0, c)
        aq = jnp.concatenate([mem, ha[0:24]], axis=0)
        lhs_aq = aq.astype(BF16)
        if li == 0:
            p0 = pl.multiple_of(pi * 16, 16)
            lhs_akv = lhs_aq
            extra_a = lambda mi, h: [pre[(mi - 1) * NG + h // G, pl.ds(p0, 16),
                                         (h % G) * DH:(h % G + 1) * DH]] if mi else []
        else:
            lhs_akv = jnp.concatenate([mem, ha], axis=0).astype(BF16)
            extra_a = lambda mi, h: []
        acc_a, prj = seg_step((lhs_aq, lhs_akv, lhs_akv), None if first else aq, extra_a, mask_a,
                              LAGA, SMID[0], fill[0])
        lhs_b = jnp.concatenate([acc_a[0:8], hb], axis=0).astype(BF16)
        bq = jnp.concatenate([acc_a[0:8], hb, ha[24:40]], axis=0)
        acc_b, _ = seg_step(
            (bq.astype(BF16), lhs_b, lhs_b), bq,
            lambda mi, h: [prj[mi][h][32:48], prj[mi][h][0:32]] if mi else [],
            mask_b, LAGB, SMID[1], fill[1])
        obuf[0:24, :] = acc_a[8:32]
        obuf[24:40, :] = acc_b[32:48]
        obuf[40:64, :] = acc_b[8:32]
        return acc_b[0:8]

    def loop_body(li, it, mem):
        UNROLL = UNROLLS[li]
        for u in range(UNROLL):
            mem = pair_body(li, it * UNROLL + u, mem, u == 0 and not KS0)

        if li == 1:
            @pl.when(it > 0)
            def _():
                out_copy(pl.multiple_of(it * (UNROLL * PAIR) - PAIR, PAIR),
                         UNROLL * PAIR).start()

            if UNROLL > 1:
                @pl.when(it == 0)
                def _():
                    out_copy(0, (UNROLL - 1) * PAIR).start()

        return mem

    for li in range(2):
        obuf[0:PAIR, :] = jnp.zeros((PAIR, D), F32)
        rbest[...] = jnp.full((RC, 128), -jnp.inf, F32)
        ibest[...] = jnp.zeros((RC, 128), F32)
        lax.fori_loop(0, NPAIR // UNROLLS[li], functools.partial(loop_body, li),
                      mem0_v[...].astype(F32))

        if li == 0:
            for c in cp_mlp:
                c.wait()
        else:
            out_copy(0, S - PAIR).wait()

        def top1():
            rb = rbest[...]
            rmax = jnp.max(rb, axis=0, keepdims=True)
            imin = jnp.min(jnp.where(rb == rmax, ibest[...], S - 1.0), axis=0, keepdims=True)
            return rmax, imin.astype(jnp.int32)[0, 0]

        def mod_trip(carry, li=li):
            rmax, idx = top1()
            lsel = lbuf[pl.ds(PAD + idx, 1), :]
            for c in range(PAIR // RC):
                post_chunk(li, NPAIR, True, c)
            xs = jnp.broadcast_to(lsel, (16, D)).astype(BF16)
            acts = []
            for f0, f1 in FSPLIT:
                gpre = _rnd(_dot(xs, wg_v[:, f0:f1]))
                gate = _rnd(gpre * _rnd(jax.nn.sigmoid(gpre)))
                up = _rnd(_dot(xs, wu_v[:, f0:f1]))
                acts.append((gate * up).astype(BF16))
            y = None
            for (f0, f1), act in zip(FSPLIT, acts):
                t = _dot(act, wd_v[f0:f1, :])
                y = t if y is None else y + t
            y = _rnd(y)[0:8]
            rsel = _rnd(jax.nn.sigmoid(rmax[:, 0:1]))
            ybuf[...] = _rnd(y * rsel)
            return idx, top1()[1]

        idx, _ = lax.while_loop(lambda cr: cr[0] != cr[1], mod_trip,
                                (jnp.int32(-1), jnp.int32(0)))
        row = pl.ds(PAD + idx, 1)
        lsel = lbuf[row, :]
        y = ybuf[0:1, :]
        if li == 0:
            x2 = _rnd(x1buf[row, :] + _rnd(lsel + y))
            xres[row, :] = x2
            hbuf[row, :] = _layernorm(x2)
        else:
            t0 = pl.multiple_of((idx // 16) * 16, 16)
            tile = pl.ds(PAD + t0, 16)
            sel = lax.broadcasted_iota(jnp.int32, (16, D), 0) == idx - t0
            upd = jnp.where(sel, jnp.broadcast_to(y, (16, D)), 0.0)
            ostage[tile, :] = (x1buf[tile, :] + _rnd(lbuf[tile, :] + upd)).astype(BF16)
            t1 = pl.multiple_of(jnp.minimum(t0, S - PAIR - 16), 16)
            out_copy(S - PAIR, PAIR).start()
            out_copy(t1, 16).start()
            out_copy(0, PAIR + 16).wait()


_FILL = ((0, 9), (0, 11), (0, 13), (0, 15), (1, 9), (1, 11), (1, 13), (1, 14))
CFG = dict(UNROLLS=(2, 2), LAGA=(1, 1, 2, True, 0), LAGB=(1, 1, 2, False, 1), FILL=(_FILL, _FILL),
           SMID=(False, True), LNP=16, LNA=16, SLACK=(128, 256), KS0=False)


def _build():
    any_spec = pl.BlockSpec(memory_space=pl.ANY)
    return pl.pallas_call(
        functools.partial(_kernel, **CFG),
        out_shape=jax.ShapeDtypeStruct((S, D), BF16),
        in_specs=[any_spec] * 10,
        out_specs=any_spec,
        scratch_shapes=[
            pltpu.VMEM((NPAIR + 2, PAIR, D), BF16),
            pltpu.VMEM((M, D), BF16),
            pltpu.VMEM((D,), BF16),
            pltpu.VMEM((NCH * D + 1, HC, DH), BF16),
            pltpu.VMEM((HD + 16, D), BF16),
            pltpu.VMEM((D, FF), BF16),
            pltpu.VMEM((D, FF), BF16),
            pltpu.VMEM((FF, D), BF16),
        ] + [pltpu.VMEM((GPC, D // 2, GW), U32)] * NCH + [
            pltpu.VMEM((HD // 2, D), U32),
            pltpu.VMEM((NTMP * TSZ, DH), U32),
            pltpu.VMEM((PAD + S, D), F32),
            pltpu.VMEM((PAD + S, D), F32),
            pltpu.VMEM((PAD + S, D), F32),
            pltpu.VMEM((PAD + S, D), F32),
            pltpu.VMEM((RC, 128), F32),
            pltpu.VMEM((RC, 128), F32),
            pltpu.VMEM((PAIR + 8, D), F32),
            pltpu.VMEM((PAD + S, D), BF16),
            pltpu.VMEM((8 * NPAIR, D), U32),
            pltpu.VMEM((2 * NG, 16 * NPAIR, GW), F32),
            pltpu.VMEM((8, D), F32),
            pltpu.SMEM((4,), jnp.int32),
            pltpu.SemaphoreType.DMA((19,)),
            pltpu.SemaphoreType.DMA(()),
        ],
        compiler_params=pltpu.CompilerParams(vmem_limit_bytes=120 * 1024 * 1024),
    )


@functools.partial(jax.jit, static_argnames=("A_seg_len",))
def pallas_interleave_layers__memory_aug_recurrent_mem_tr__moe_arch_mod__prompt_kernel(
    A_x: jax.Array,
    A_mem0: jax.Array,
    A_Wq: jax.Array,
    A_Wk: jax.Array,
    A_Wv: jax.Array,
    A_Wo: jax.Array,
    A_seg_len,
    B_x: jax.Array,
    B_w_r: jax.Array,
    B_w_gate: jax.Array,
    B_w_up: jax.Array,
    B_w_down: jax.Array,
):
    assert A_seg_len == SEG and A_x.shape == (1, S, D)
    del B_x
    out = _build()(
        A_x.reshape(NPAIR, PAIR, D),
        A_mem0.reshape(M, D),
        A_Wq,
        A_Wk,
        A_Wv,
        A_Wo.reshape(HD, D),
        B_w_r,
        B_w_gate,
        B_w_up,
        B_w_down,
    )
    return out.reshape(1, S, D)
```

```python
import functools
import math

import jax
import jax.numpy as jnp
from jax import lax
import jax.experimental.pallas as pl
import jax.experimental.pallas.tpu as pltpu

F32 = jnp.float32
BF16 = jnp.bfloat16
U32 = jnp.uint32

S, D, H, DH, M, SEG = 2048, 512, 32, 128, 8, 32
FF = 1792
HD = H * DH
PAIR = 2 * SEG
NPAIR = S // PAIR
PAD = PAIR
G = 4
NG = H // G
GW = G * DH
HC = 16
GPC = HC // G
NCH = 3 * H // HC
TP = 20
TSZ = 8 * TP
NTMP = 8
FSPLIT = ((0, 1024), (1024, FF))
RC = 8
LN_EPS = 1e-05
NEG = -1000000000.0
EXP2_SCALE = (DH ** -0.5) * math.log2(math.e)


def _rnd(x):
    return x.astype(BF16).astype(F32)


def _layernorm(x):
    mean = jnp.sum(x, axis=-1, keepdims=True) * (1.0 / D)
    c = x - mean
    var = jnp.sum(c * c, axis=-1, keepdims=True) * (1.0 / D)
    z = _rnd(_rnd(var) + _rnd(jnp.float32(LN_EPS)))
    den = _rnd(z * lax.rsqrt(z))
    inv = pl.reciprocal(den, approx=True)
    inv = inv * (2.0 - den * inv)
    return _rnd(_rnd(x - _rnd(mean)) * inv)


def _dot(a, b):
    return jnp.dot(a, b, preferred_element_type=F32)


def _dot_nt(a, b):
    return lax.dot_general(a, b, (((1,), (1,)), ((), ())), preferred_element_type=F32)


def _softmax_bf16(s, mask):
    s = jnp.where(mask, s, NEG)
    m = jnp.max(s, axis=-1, keepdims=True)
    e = jnp.exp2((s - m) * EXP2_SCALE)
    l = jnp.sum(e, axis=-1, keepdims=True)
    r = pl.reciprocal(l, approx=True)
    r = r * (2.0 - l * r)
    return (e * r).astype(BF16)


def _kernel(x_hbm, mem0_hbm, wq_hbm, wk_hbm, wv_hbm, wo_hbm, wr_hbm, wg_hbm, wu_hbm, wd_hbm,
            out_hbm,
            x_raw, mem0_v, wr_v, stage, wo_raw, wg_v, wu_v, wd_v,
            wk0, wk1, wv0, wv1, wq0, wq1, wo, tmp,
            xres, x1buf, lbuf, hbuf, rbest, ibest, obuf, ostage,
            lhs_pre, pre, ybuf, anchor, sems, osem, *,
            UNROLLS, LAGA, LAGB, FILL, SMID, LNP, LNA, SLACK, KS0, LNTIE):
    wch = (wk0, wk1, wv0, wv1, wq0, wq1)
    NWO = 4
    WOP = HD // NWO
    WPARTS = (2, 2, 2, 1, 4, 4)
    SEM_X = 0
    SEM_W = [3 + sum(WPARTS[:c]) for c in range(NCH)]
    SEM_O = 3 + sum(WPARTS)
    SEM_MISC = SEM_O + NWO

    def cp_x(i):
        r0, nr = ((24, 16), (0, 24), (40, 24))[i]
        return pltpu.make_async_copy(x_hbm.at[:, pl.ds(r0, nr), :],
                                     x_raw.at[pl.ds(1, NPAIR), pl.ds(r0, nr), :],
                                     sems.at[SEM_X + i])

    def cp_w(c, part):
        w = (wk_hbm, wv_hbm, wq_hbm)[c // 2]
        nd = D // WPARTS[c]
        return pltpu.make_async_copy(
            w.at[pl.ds(part * nd, nd), pl.ds((c % 2) * HC, HC), :],
            stage.at[pl.ds(c * D + part * nd, nd)], sems.at[SEM_W[c] + part])

    def cp_o(i):
        return pltpu.make_async_copy(wo_hbm.at[pl.ds(i * WOP, WOP)],
                                     wo_raw.at[pl.ds(i * WOP, WOP)], sems.at[SEM_O + i])

    cp_small = [pltpu.make_async_copy(s_, d_, sems.at[SEM_MISC + i])
                for i, (s_, d_) in enumerate(((mem0_hbm, mem0_v), (wr_hbm, wr_v)))]
    cp_mlp = [pltpu.make_async_copy(s_, d_, sems.at[SEM_MISC + 2 + i])
              for i, (s_, d_) in enumerate(((wg_hbm, wg_v), (wu_hbm, wu_v), (wd_hbm, wd_v)))]
    cp_x(0).start()
    for c in range(3):
        cp_w(c, 0).start()
        cp_w(c, 1).start()
    cp_x(1).start()
    cp_x(2).start()
    cp_w(3, 0).start()
    for i in range(NWO):
        cp_w(4, i).start()
        cp_w(5, i).start()
        cp_o(i).start()
    for c in cp_small + cp_mlp:
        c.start()

    anchor[0] = PAIR
    anchor[1] = NCH * D
    anchor[2] = HD
    anchor[3] = NPAIR + 1
    x_raw[0] = jnp.zeros((PAIR, D), BF16)
    xres[0:PAD, :] = jnp.zeros((PAD, D), F32)

    cp_x(0).wait()

    def ln_mid(i, carry):
        for pp in range(LNP):
            pr = i * LNP + pp
            ln = _layernorm(x_raw[1 + pr, 24:40, :].astype(F32))
            hbuf[pl.ds(pl.multiple_of(PAD + pr * PAIR + 24, 8), 16), :] = ln
            lhs_pre[pl.ds(pl.multiple_of(pr * 8, 8), 8), :] = pltpu.bitcast(ln.astype(BF16), U32)
        return carry

    lax.fori_loop(0, NPAIR // LNP, ln_mid, 0)

    def ln_jobs(p0, npairs):
        def job(pp, r0):
            ln = _layernorm(x_raw[1 + p0 + pp, r0:r0 + 8, :].astype(F32))
            hbuf[pl.ds(pl.multiple_of(PAD + (p0 + pp) * PAIR + r0, 8), 8), :] = ln

        return [('x_raw', functools.partial(job, pp, r0))
                for pp in range(npairs) for r0 in (0, 8, 16, 40, 48, 56)]

    def relayout_jobs(c, blk0, nblk, slot0=0):
        def job(u):
            t0 = ((slot0 + u) % NTMP) * TSZ
            d0 = pl.multiple_of(c * D + (blk0 + u) * 16, 16)
            raw = pltpu.bitcast(stage[pl.ds(d0, 16), :, :], U32)
            for i in range(8):
                ev, od = raw[2 * i], raw[2 * i + 1]
                lo = (ev & jnp.uint32(0xFFFF)) | (od << 16)
                hi = (ev >> 16) | (od & jnp.uint32(0xFFFF0000))
                tmp[pl.ds(t0 + i * TP, 8, stride=2), :] = lo
                tmp[pl.ds(t0 + i * TP + 1, 8, stride=2), :] = hi
            o0 = pl.multiple_of((blk0 + u) * 8, 8)
            for hh in range(HC):
                col = (hh % G) * DH
                wch[c][hh // G, pl.ds(o0, 8), col:col + DH] = tmp[pl.ds(t0 + hh, 8, stride=TP), :]

        return [('stage', functools.partial(job, u)) for u in range(nblk)]

    def repack_jobs(part):
        def job(c):
            r0 = pl.multiple_of(part * WOP + c * 128, 128)
            o0 = pl.multiple_of(part * (WOP // 2) + c * 64, 64)
            wo[pl.ds(o0, 64), :] = pltpu.bitcast(wo_raw[pl.ds(r0, 128), :], U32)

        return [('wo_raw', functools.partial(job, c)) for c in range(WOP // 128)]

    def interleave(*lists):
        keyed = [((i + 0.5) / len(l), n, j) for n, l in enumerate(lists) for i, j in enumerate(l)]
        return [j for _, _, j in sorted(keyed, key=lambda t: t[:2])]

    def precompute(c, g0, ng, jobs, khalf=None):
        if khalf is None:
            lhs = pltpu.bitcast(lhs_pre[...], BF16)
            ys = [_dot(lhs, pltpu.bitcast(wch[c][g0 + gg], BF16)) for gg in range(ng)]
        else:
            k0 = khalf * (D // 2)
            lhs = pltpu.bitcast(lhs_pre[:, k0:k0 + D // 2], BF16)
            ys = [_dot(lhs, pltpu.bitcast(wch[c][g0 + gg, k0 // 2:k0 // 2 + D // 4, :], BF16))
                  for gg in range(ng)]
        nrow = 16 * NPAIR
        has_ln = any(kind == 'x_raw' for kind, _ in jobs)
        nln = 0
        for u, (kind, job) in enumerate(jobs):
            nln += kind == 'x_raw'
            if u > 0 and (kind != 'x_raw' or nln % LNTIE == 0):
                par = 1 if khalf is None else 2
                span = ng * G * nrow // par - (SLACK[1] if has_ln else SLACK[0])
                pos = max((u * span // len(jobs)) // 16 * 16 - 128, 0)
                nt, r0 = pos // nrow * par, pos % nrow
                tie = ys[nt // G][r0:r0 + 16, (nt % G) * DH:(nt % G + 1) * DH].astype(BF16)
                if kind == 'stage':
                    stage[anchor[1]] = tie
                elif kind == 'x_raw':
                    x_raw[anchor[3], 0:16, 0:DH] = tie
                else:
                    wo_raw[pl.ds(pl.multiple_of(anchor[2], 16), 16), 0:DH] = tie
            job()
        for gg in range(ng):
            if khalf == 1:
                pre[c * GPC + g0 + gg] += ys[gg]
            else:
                pre[c * GPC + g0 + gg] = ys[gg]

    def run(jobs):
        for _, job in jobs:
            job()

    NBLK = D // 16

    HB, QB = NBLK // 2, NBLK // 4
    cp_w(0, 0).wait()
    lax.fori_loop(0, HB // 8, lambda it, cr: (run(relayout_jobs(0, it * 8, 8)), cr)[1], 0)
    precompute(0, 0, 2, [], khalf=0)
    cp_w(0, 1).wait()
    precompute(0, 2, 2, relayout_jobs(0, HB, HB), khalf=0)

    def phase01(c, khalf, it, carry):
        cp_w(c + 1, it).wait()
        precompute(c, it * 2, 2, relayout_jobs(c + 1, it * HB, HB), khalf)
        return carry

    lax.fori_loop(0, 2, functools.partial(phase01, 0, 1), 0)
    lax.fori_loop(0, 2, functools.partial(phase01, 1, None), 0)
    cp_x(1).wait()
    cp_x(2).wait()
    cp_w(3, 0).wait()
    lax.fori_loop(0, 2, lambda it, cr: (
        precompute(2, it * 2, 2, interleave(relayout_jobs(3, it * HB, HB),
                                            ln_jobs(it * LNA, LNA))), cr)[1], 0)
    LNB = (NPAIR - 2 * LNA) // 4

    def last_phase(it, carry):
        cp_w(4, it).wait()
        cp_w(5, it).wait()
        cp_o(it).wait()
        precompute(3, it, 1, interleave(relayout_jobs(4, it * QB, QB),
                                        relayout_jobs(5, it * QB, QB, NTMP // 2),
                                        repack_jobs(it),
                                        ln_jobs(2 * LNA + it * LNB, LNB)))
        return carry

    lax.fori_loop(0, 4, last_phase, 0)

    for c in cp_small:
        c.wait()
    wr = wr_v[...].astype(F32).reshape(1, D)

    qi = lax.broadcasted_iota(jnp.int32, (32, 48), 0)
    kj = lax.broadcasted_iota(jnp.int32, (32, 48), 1)
    mask_a = (kj < 40) & ((qi < M) | (kj <= qi))
    qi = lax.broadcasted_iota(jnp.int32, (48, 80), 0)
    kj = lax.broadcasted_iota(jnp.int32, (48, 80), 1)
    kb0 = (kj >= 40) & (kj < 48)
    m_mem = (qi < M) & ((kj < 32) | kb0)
    m_xb = (qi >= M) & (qi < 32) & ((kj <= qi) | kb0)
    m_xa = (qi >= 32) & (qi < 40) & ((kj >= 48) | ((kj >= 32) & (kj <= qi)))
    m_b0 = (qi >= 40) & ((kj < M) | (kb0 & (kj <= qi)))
    mask_b = m_mem | m_xb | m_xa | m_b0

    def w_ref(mi, g):
        return wch[(4, 0, 2)[mi] + g // GPC].at[g % GPC]

    def wo_rows(g, n=1):
        r0 = g * GW // 2
        return pltpu.bitcast(wo[r0:r0 + n * GW // 2, :], BF16)

    def seg_step(lhs, lhs_f32, extra, mask, lags, s_mid, filler):
        q, k, v, p, o = {}, {}, {}, {}, {}
        raw = ({}, {}, {})
        acc = [None]

        def proj(mi, g, dst):
            if mi == 0 and g == 0 and lhs_f32 is not None:
                y = None
                lp = jnp.concatenate([lhs_f32[16:], lhs_f32[0:16]], axis=0)
                for kt in range(D // 128):
                    w = pltpu.bitcast(w_ref(0, 0)[kt * 64:(kt + 1) * 64, :], BF16)
                    t = _dot(lp[:, kt * 128:(kt + 1) * 128].astype(BF16), w)
                    y = t if y is None else y + t
                nr = y.shape[0]
                y = jnp.concatenate([y[nr - 16:], y[0:nr - 16]], axis=0)
            else:
                y = _dot(lhs[mi], pltpu.bitcast(w_ref(mi, g)[...], BF16))
            for j in range(G):
                h = g * G + j
                yh = y[:, j * DH:(j + 1) * DH]
                ex = extra(mi, h)
                if ex:
                    yh = jnp.concatenate([yh] + ex, axis=0)
                raw[mi][h] = yh
                dst[h] = yh.astype(BF16)

        def sc(g):
            for h in range(g * G, (g + 1) * G):
                p[h] = _softmax_bf16(_dot_nt(q[h], k[h]), mask)

        def pv(g):
            o[g] = jnp.concatenate(
                [_dot(p[h], v[h]) for h in range(g * G, (g + 1) * G)], axis=1)

        def op(g):
            if merge and g == NG - 2:
                return
            if merge and g == NG - 1:
                y = _dot(jnp.concatenate([o[g - 1], o[g]], axis=1).astype(BF16),
                         wo_rows(g - 1, 2))
            else:
                y = _dot(o[g].astype(BF16), wo_rows(g))
            acc[0] = y if acc[0] is None else acc[0] + y

        ls, lp, lo, merge, pv0 = lags
        for t in range(2 * NG + lp + lo):
            if t < NG:
                proj(0, t, q)
                if s_mid and 0 <= t - ls < NG:
                    sc(t - ls)
                proj(1, t, k)
            elif t < 2 * NG:
                proj(2, t - NG, v)
            if 0 <= t - ls < NG and not s_mid:
                sc(t - ls)
            if t == NG + lp + pv0:
                pv(0)
                if s_mid:
                    for g in range(NG - ls, NG):
                        sc(g)
            if 0 < t - NG - lp < NG:
                pv(t - NG - lp)
            if pv0 > lo - 1 and t == NG + lp + lo + 1:
                op(0)
            if (1 if pv0 > lo - 1 else 0) <= t - NG - lp - lo < NG:
                op(t - NG - lp - lo)
            if t in filler:
                src = raw[1][t * G] if t < NG else raw[2][min(t - NG, NG - 1) * G]
                filler[t](src[0:8])
        return acc[0], raw

    subr = lax.broadcasted_iota(jnp.int32, (RC, 128), 0).astype(F32)

    def post_chunk(li, pi, valid, c, tie=None):
        if tie is not None:
            obuf[pl.ds(pl.multiple_of(anchor[0], 8), 8), 0:DH] = tie
        base = pi * PAIR if isinstance(pi, int) else pl.multiple_of(pi * PAIR, PAIR)
        rows = pl.ds(base + c * RC, RC)
        x0 = x_raw[pi, c * RC:(c + 1) * RC, :].astype(F32) if li == 0 else xres[rows, :]
        x1 = _rnd(x0 + _rnd(obuf[c * RC:(c + 1) * RC, :]))
        ln = _layernorm(x1)
        r = _rnd(jnp.sum(ln * wr, axis=-1, keepdims=True))
        r = jnp.broadcast_to(jnp.where(valid, r, -jnp.inf), (RC, 128))
        rb = rbest[...]
        better = r > rb
        rbest[...] = jnp.where(better, r, rb)
        row0 = jnp.asarray(base + (c * RC - PAD), jnp.int32).astype(F32)
        ibest[...] = jnp.where(better, subr + row0, ibest[...])
        x1buf[rows, :] = x1
        lbuf[rows, :] = ln
        if li == 0:
            x2 = _rnd(x1 + ln)
            xres[rows, :] = x2
            hbuf[rows, :] = _layernorm(x2)
        else:
            ostage[rows, :] = (x1 + ln).astype(BF16)

    def out_copy(row0, nrows):
        return pltpu.make_async_copy(ostage.at[pl.ds(PAD + row0, nrows)],
                                     out_hbm.at[pl.ds(row0, nrows)], osem)

    def pair_body(li, pi, mem, first):
        base = pl.multiple_of(pi * PAIR, PAIR)
        ha = hbuf[pl.ds(base + PAD, 40), :]
        hb = hbuf[pl.ds(base + PAD + 40, 24), :]
        fill = ({}, {})
        for c, (st, t) in enumerate(FILL[li]):
            fill[st][t] = functools.partial(post_chunk, li, pi, pi > 0, c)
        aq = jnp.concatenate([mem, ha[0:24]], axis=0)
        lhs_aq = aq.astype(BF16)
        if li == 0:
            p0 = pl.multiple_of(pi * 16, 16)
            lhs_akv = lhs_aq
            extra_a = lambda mi, h: [pre[(mi - 1) * NG + h // G, pl.ds(p0, 16),
                                         (h % G) * DH:(h % G + 1) * DH]] if mi else []
        else:
            lhs_akv = jnp.concatenate([mem, ha], axis=0).astype(BF16)
            extra_a = lambda mi, h: []
        acc_a, prj = seg_step((lhs_aq, lhs_akv, lhs_akv), None if first else aq, extra_a, mask_a,
                              LAGA, SMID[0], fill[0])
        lhs_b = jnp.concatenate([acc_a[0:8], hb], axis=0).astype(BF16)
        bq = jnp.concatenate([acc_a[0:8], hb, ha[24:40]], axis=0)
        acc_b, _ = seg_step(
            (bq.astype(BF16), lhs_b, lhs_b), bq,
            lambda mi, h: [prj[mi][h][32:48], prj[mi][h][0:32]] if mi else [],
            mask_b, LAGB, SMID[1], fill[1])
        obuf[0:24, :] = acc_a[8:32]
        obuf[24:40, :] = acc_b[32:48]
        obuf[40:64, :] = acc_b[8:32]
        return acc_b[0:8]

    def loop_body(li, it, mem):
        UNROLL = UNROLLS[li]
        for u in range(UNROLL):
            mem = pair_body(li, it * UNROLL + u, mem, u == 0 and not KS0)

        if li == 1:
            @pl.when(it > 0)
            def _():
                out_copy(pl.multiple_of(it * (UNROLL * PAIR) - PAIR, PAIR),
                         UNROLL * PAIR).start()

            if UNROLL > 1:
                @pl.when(it == 0)
                def _():
                    out_copy(0, (UNROLL - 1) * PAIR).start()

        return mem

    for li in range(2):
        obuf[0:PAIR, :] = jnp.zeros((PAIR, D), F32)
        rbest[...] = jnp.full((RC, 128), -jnp.inf, F32)
        ibest[...] = jnp.zeros((RC, 128), F32)
        lax.fori_loop(0, NPAIR // UNROLLS[li], functools.partial(loop_body, li),
                      mem0_v[...].astype(F32))

        if li == 0:
            for c in cp_mlp:
                c.wait()
        else:
            out_copy(0, S - PAIR).wait()

        def top1():
            rb = rbest[...]
            rmax = jnp.max(rb, axis=0, keepdims=True)
            imin = jnp.min(jnp.where(rb == rmax, ibest[...], S - 1.0), axis=0, keepdims=True)
            return rmax, imin.astype(jnp.int32)[0, 0]

        def mod_trip(carry, li=li):
            rmax, idx = top1()
            lsel = lbuf[pl.ds(PAD + idx, 1), :]
            for c in range(PAIR // RC):
                post_chunk(li, NPAIR, True, c)
            xs = jnp.broadcast_to(lsel, (16, D)).astype(BF16)
            acts = []
            for f0, f1 in FSPLIT:
                gpre = _rnd(_dot(xs, wg_v[:, f0:f1]))
                gate = _rnd(gpre * _rnd(jax.nn.sigmoid(gpre)))
                up = _rnd(_dot(xs, wu_v[:, f0:f1]))
                acts.append((gate * up).astype(BF16))
            y = None
            for (f0, f1), act in zip(FSPLIT, acts):
                t = _dot(act, wd_v[f0:f1, :])
                y = t if y is None else y + t
            y = _rnd(y)[0:8]
            rsel = _rnd(jax.nn.sigmoid(rmax[:, 0:1]))
            ybuf[...] = _rnd(y * rsel)
            return idx, top1()[1]

        idx, _ = lax.while_loop(lambda cr: cr[0] != cr[1], mod_trip,
                                (jnp.int32(-1), jnp.int32(0)))
        row = pl.ds(PAD + idx, 1)
        lsel = lbuf[row, :]
        y = ybuf[0:1, :]
        if li == 0:
            x2 = _rnd(x1buf[row, :] + _rnd(lsel + y))
            xres[row, :] = x2
            hbuf[row, :] = _layernorm(x2)
        else:
            t0 = pl.multiple_of((idx // 16) * 16, 16)
            tile = pl.ds(PAD + t0, 16)
            sel = lax.broadcasted_iota(jnp.int32, (16, D), 0) == idx - t0
            upd = jnp.where(sel, jnp.broadcast_to(y, (16, D)), 0.0)
            ostage[tile, :] = (x1buf[tile, :] + _rnd(lbuf[tile, :] + upd)).astype(BF16)
            t1 = pl.multiple_of(jnp.minimum(t0, S - PAIR - 16), 16)
            out_copy(S - PAIR, PAIR).start()
            out_copy(t1, 16).start()
            out_copy(0, PAIR + 16).wait()


_FILL = ((0, 9), (0, 11), (0, 13), (0, 15), (1, 9), (1, 11), (1, 13), (1, 14))
CFG = dict(UNROLLS=(2, 2), LAGA=(1, 1, 2, True, 0), LAGB=(1, 1, 2, False, 1), FILL=(_FILL, _FILL),
           SMID=(False, True), LNP=16, LNA=16, SLACK=(128, 256), KS0=False, LNTIE=1)


def _build():
    any_spec = pl.BlockSpec(memory_space=pl.ANY)
    return pl.pallas_call(
        functools.partial(_kernel, **CFG),
        out_shape=jax.ShapeDtypeStruct((S, D), BF16),
        in_specs=[any_spec] * 10,
        out_specs=any_spec,
        scratch_shapes=[
            pltpu.VMEM((NPAIR + 2, PAIR, D), BF16),
            pltpu.VMEM((M, D), BF16),
            pltpu.VMEM((D,), BF16),
            pltpu.VMEM((NCH * D + 1, HC, DH), BF16),
            pltpu.VMEM((HD + 16, D), BF16),
            pltpu.VMEM((D, FF), BF16),
            pltpu.VMEM((D, FF), BF16),
            pltpu.VMEM((FF, D), BF16),
        ] + [pltpu.VMEM((GPC, D // 2, GW), U32)] * NCH + [
            pltpu.VMEM((HD // 2, D), U32),
            pltpu.VMEM((NTMP * TSZ, DH), U32),
            pltpu.VMEM((PAD + S, D), F32),
            pltpu.VMEM((PAD + S, D), F32),
            pltpu.VMEM((PAD + S, D), F32),
            pltpu.VMEM((PAD + S, D), F32),
            pltpu.VMEM((RC, 128), F32),
            pltpu.VMEM((RC, 128), F32),
            pltpu.VMEM((PAIR + 8, D), F32),
            pltpu.VMEM((PAD + S, D), BF16),
            pltpu.VMEM((8 * NPAIR, D), U32),
            pltpu.VMEM((2 * NG, 16 * NPAIR, GW), F32),
            pltpu.VMEM((8, D), F32),
            pltpu.SMEM((4,), jnp.int32),
            pltpu.SemaphoreType.DMA((27,)),
            pltpu.SemaphoreType.DMA(()),
        ],
        compiler_params=pltpu.CompilerParams(vmem_limit_bytes=120 * 1024 * 1024),
    )


@functools.partial(jax.jit, static_argnames=("A_seg_len",))
def pallas_interleave_layers__memory_aug_recurrent_mem_tr__moe_arch_mod__prompt_kernel(
    A_x: jax.Array,
    A_mem0: jax.Array,
    A_Wq: jax.Array,
    A_Wk: jax.Array,
    A_Wv: jax.Array,
    A_Wo: jax.Array,
    A_seg_len,
    B_x: jax.Array,
    B_w_r: jax.Array,
    B_w_gate: jax.Array,
    B_w_up: jax.Array,
    B_w_down: jax.Array,
):
    assert A_seg_len == SEG and A_x.shape == (1, S, D)
    del B_x
    out = _build()(
        A_x.reshape(NPAIR, PAIR, D),
        A_mem0.reshape(M, D),
        A_Wq,
        A_Wk,
        A_Wv,
        A_Wo.reshape(HD, D),
        B_w_r,
        B_w_gate,
        B_w_up,
        B_w_down,
    )
    return out.reshape(1, S, D)
```

```python
import functools
import math

import jax
import jax.numpy as jnp
from jax import lax
import jax.experimental.pallas as pl
import jax.experimental.pallas.tpu as pltpu

F32 = jnp.float32
BF16 = jnp.bfloat16
U32 = jnp.uint32

S, D, H, DH, M, SEG = 2048, 512, 32, 128, 8, 32
FF = 1792
HD = H * DH
PAIR = 2 * SEG
NPAIR = S // PAIR
PAD = PAIR
G = 4
NG = H // G
GW = G * DH
HC = 16
GPC = HC // G
NCH = 3 * H // HC
TP = 20
TSZ = 8 * TP
NTMP = 8
FSPLIT = ((0, 1024), (1024, FF))
RC = 8
LN_EPS = 1e-05
NEG = -1000000000.0 * DH ** 0.5
EXP2_SCALE = (DH ** -0.5) * math.log2(math.e)


def _rnd(x):
    return x.astype(BF16).astype(F32)


def _layernorm(x):
    mean = jnp.sum(x, axis=-1, keepdims=True) * (1.0 / D)
    c = x - mean
    var = jnp.sum(c * c, axis=-1, keepdims=True) * (1.0 / D)
    z = _rnd(_rnd(var) + _rnd(jnp.float32(LN_EPS)))
    den = _rnd(z * lax.rsqrt(z))
    inv = pl.reciprocal(den, approx=True)
    inv = inv * (2.0 - den * inv)
    return _rnd(_rnd(x - _rnd(mean)) * inv)


def _dot(a, b):
    return jnp.dot(a, b, preferred_element_type=F32)


def _dot_nt(a, b):
    return lax.dot_general(a, b, (((1,), (1,)), ((), ())), preferred_element_type=F32)


def _softmax_bf16(s, mask):
    s = jnp.where(mask, s, NEG)
    m = jnp.max(s, axis=-1, keepdims=True)
    e = jnp.exp2((s - m) * EXP2_SCALE)
    l = jnp.sum(e, axis=-1, keepdims=True)
    r = pl.reciprocal(l, approx=True)
    r = r * (2.0 - l * r)
    return (e * r).astype(BF16)


def _kernel(x_hbm, mem0_hbm, wq_hbm, wk_hbm, wv_hbm, wo_hbm, wr_hbm, wg_hbm, wu_hbm, wd_hbm,
            out_hbm,
            x_raw, mem0_v, wr_v, stage, wo_raw, wg_v, wu_v, wd_v,
            wk0, wk1, wv0, wv1, wq0, wq1, wo, tmp,
            xres, x1buf, lbuf, hbuf, rbest, ibest, obuf, ostage,
            lhs_pre, pre, ybuf, anchor, sems, osem, *,
            UNROLLS, LAGA, LAGB, FILL, SMID, LNP, LNA, SLACK, KS0, LNTIE):
    wch = (wk0, wk1, wv0, wv1, wq0, wq1)
    NWO = 4
    WOP = HD // NWO
    WPARTS = (2, 2, 2, 1, 4, 4)
    SEM_X = 0
    SEM_W = [3 + sum(WPARTS[:c]) for c in range(NCH)]
    SEM_O = 3 + sum(WPARTS)
    SEM_MISC = SEM_O + NWO

    def cp_x(i):
        r0, nr = ((24, 16), (0, 24), (40, 24))[i]
        return pltpu.make_async_copy(x_hbm.at[:, pl.ds(r0, nr), :],
                                     x_raw.at[pl.ds(1, NPAIR), pl.ds(r0, nr), :],
                                     sems.at[SEM_X + i])

    def cp_w(c, part):
        w = (wk_hbm, wv_hbm, wq_hbm)[c // 2]
        nd = D // WPARTS[c]
        return pltpu.make_async_copy(
            w.at[pl.ds(part * nd, nd), pl.ds((c % 2) * HC, HC), :],
            stage.at[pl.ds(c * D + part * nd, nd)], sems.at[SEM_W[c] + part])

    def cp_o(i):
        return pltpu.make_async_copy(wo_hbm.at[pl.ds(i * WOP, WOP)],
                                     wo_raw.at[pl.ds(i * WOP, WOP)], sems.at[SEM_O + i])

    cp_small = [pltpu.make_async_copy(s_, d_, sems.at[SEM_MISC + i])
                for i, (s_, d_) in enumerate(((mem0_hbm, mem0_v), (wr_hbm, wr_v)))]
    cp_mlp = [pltpu.make_async_copy(s_, d_, sems.at[SEM_MISC + 2 + i])
              for i, (s_, d_) in enumerate(((wg_hbm, wg_v), (wu_hbm, wu_v), (wd_hbm, wd_v)))]
    cp_x(0).start()
    for c in range(3):
        cp_w(c, 0).start()
        cp_w(c, 1).start()
    cp_x(1).start()
    cp_x(2).start()
    cp_w(3, 0).start()
    for i in range(NWO):
        cp_w(4, i).start()
        cp_w(5, i).start()
        cp_o(i).start()
    for c in cp_small + cp_mlp:
        c.start()

    anchor[0] = PAIR
    anchor[1] = NCH * D
    anchor[2] = HD
    anchor[3] = NPAIR + 1
    x_raw[0] = jnp.zeros((PAIR, D), BF16)
    xres[0:PAD, :] = jnp.zeros((PAD, D), F32)

    cp_x(0).wait()

    def ln_mid(i, carry):
        for pp in range(LNP):
            pr = i * LNP + pp
            ln = _layernorm(x_raw[1 + pr, 24:40, :].astype(F32))
            hbuf[pl.ds(pl.multiple_of(PAD + pr * PAIR + 24, 8), 16), :] = ln
            lhs_pre[pl.ds(pl.multiple_of(pr * 8, 8), 8), :] = pltpu.bitcast(ln.astype(BF16), U32)
        return carry

    lax.fori_loop(0, NPAIR // LNP, ln_mid, 0)

    def ln_jobs(p0, npairs):
        def job(pp, r0):
            ln = _layernorm(x_raw[1 + p0 + pp, r0:r0 + 8, :].astype(F32))
            hbuf[pl.ds(pl.multiple_of(PAD + (p0 + pp) * PAIR + r0, 8), 8), :] = ln

        return [('x_raw', functools.partial(job, pp, r0))
                for pp in range(npairs) for r0 in (0, 8, 16, 40, 48, 56)]

    def relayout_jobs(c, blk0, nblk, slot0=0):
        def job(u):
            t0 = ((slot0 + u) % NTMP) * TSZ
            d0 = pl.multiple_of(c * D + (blk0 + u) * 16, 16)
            raw = pltpu.bitcast(stage[pl.ds(d0, 16), :, :], U32)
            for i in range(8):
                ev, od = raw[2 * i], raw[2 * i + 1]
                lo = (ev & jnp.uint32(0xFFFF)) | (od << 16)
                hi = (ev >> 16) | (od & jnp.uint32(0xFFFF0000))
                tmp[pl.ds(t0 + i * TP, 8, stride=2), :] = lo
                tmp[pl.ds(t0 + i * TP + 1, 8, stride=2), :] = hi
            o0 = pl.multiple_of((blk0 + u) * 8, 8)
            for hh in range(HC):
                col = (hh % G) * DH
                wch[c][hh // G, pl.ds(o0, 8), col:col + DH] = tmp[pl.ds(t0 + hh, 8, stride=TP), :]

        return [('stage', functools.partial(job, u)) for u in range(nblk)]

    def repack_jobs(part):
        def job(c):
            r0 = pl.multiple_of(part * WOP + c * 128, 128)
            o0 = pl.multiple_of(part * (WOP // 2) + c * 64, 64)
            wo[pl.ds(o0, 64), :] = pltpu.bitcast(wo_raw[pl.ds(r0, 128), :], U32)

        return [('wo_raw', functools.partial(job, c)) for c in range(WOP // 128)]

    def interleave(*lists):
        keyed = [((i + 0.5) / len(l), n, j) for n, l in enumerate(lists) for i, j in enumerate(l)]
        return [j for _, _, j in sorted(keyed, key=lambda t: t[:2])]

    def precompute(c, g0, ng, jobs, khalf=None):
        if khalf is None:
            lhs = pltpu.bitcast(lhs_pre[...], BF16)
            ys = [_dot(lhs, pltpu.bitcast(wch[c][g0 + gg], BF16)) for gg in range(ng)]
        else:
            k0 = khalf * (D // 2)
            lhs = pltpu.bitcast(lhs_pre[:, k0:k0 + D // 2], BF16)
            ys = [_dot(lhs, pltpu.bitcast(wch[c][g0 + gg, k0 // 2:k0 // 2 + D // 4, :], BF16))
                  for gg in range(ng)]
        nrow = 16 * NPAIR
        has_ln = any(kind == 'x_raw' for kind, _ in jobs)
        nln = 0
        for u, (kind, job) in enumerate(jobs):
            nln += kind == 'x_raw'
            if u > 0 and (kind != 'x_raw' or nln % LNTIE == 0):
                par = 1 if khalf is None else 2
                span = ng * G * nrow // par - (SLACK[1] if has_ln else SLACK[0])
                pos = max((u * span // len(jobs)) // 16 * 16 - 128, 0)
                nt, r0 = pos // nrow * par, pos % nrow
                tie = ys[nt // G][r0:r0 + 16, (nt % G) * DH:(nt % G + 1) * DH].astype(BF16)
                if kind == 'stage':
                    stage[anchor[1]] = tie
                elif kind == 'x_raw':
                    x_raw[anchor[3], 0:16, 0:DH] = tie
                else:
                    wo_raw[pl.ds(pl.multiple_of(anchor[2], 16), 16), 0:DH] = tie
            job()
        for gg in range(ng):
            if khalf == 1:
                pre[c * GPC + g0 + gg] += ys[gg]
            else:
                pre[c * GPC + g0 + gg] = ys[gg]

    def run(jobs):
        for _, job in jobs:
            job()

    NBLK = D // 16

    HB, QB = NBLK // 2, NBLK // 4
    cp_w(0, 0).wait()
    lax.fori_loop(0, HB // 8, lambda it, cr: (run(relayout_jobs(0, it * 8, 8)), cr)[1], 0)
    precompute(0, 0, 2, [], khalf=0)
    cp_w(0, 1).wait()
    precompute(0, 2, 2, relayout_jobs(0, HB, HB), khalf=0)

    def phase01(c, khalf, it, carry):
        cp_w(c + 1, it).wait()
        precompute(c, it * 2, 2, relayout_jobs(c + 1, it * HB, HB), khalf)
        return carry

    lax.fori_loop(0, 2, functools.partial(phase01, 0, 1), 0)
    lax.fori_loop(0, 2, functools.partial(phase01, 1, None), 0)
    cp_x(1).wait()
    cp_x(2).wait()
    cp_w(3, 0).wait()
    lax.fori_loop(0, 2, lambda it, cr: (
        precompute(2, it * 2, 2, interleave(relayout_jobs(3, it * HB, HB),
                                            ln_jobs(it * LNA, LNA))), cr)[1], 0)
    LNB = (NPAIR - 2 * LNA) // 4

    def last_phase(it, carry):
        cp_w(4, it).wait()
        cp_w(5, it).wait()
        cp_o(it).wait()
        precompute(3, it, 1, interleave(relayout_jobs(4, it * QB, QB),
                                        relayout_jobs(5, it * QB, QB, NTMP // 2),
                                        repack_jobs(it),
                                        ln_jobs(2 * LNA + it * LNB, LNB)))
        return carry

    lax.fori_loop(0, 4, last_phase, 0)

    for c in cp_small:
        c.wait()
    wr = wr_v[...].astype(F32).reshape(1, D)

    qi = lax.broadcasted_iota(jnp.int32, (32, 48), 0)
    kj = lax.broadcasted_iota(jnp.int32, (32, 48), 1)
    mask_a = (kj < 40) & ((qi < M) | (kj <= qi))
    qi = lax.broadcasted_iota(jnp.int32, (48, 80), 0)
    kj = lax.broadcasted_iota(jnp.int32, (48, 80), 1)
    kb0 = (kj >= 40) & (kj < 48)
    m_mem = (qi < M) & ((kj < 32) | kb0)
    m_xb = (qi >= M) & (qi < 32) & ((kj <= qi) | kb0)
    m_xa = (qi >= 32) & (qi < 40) & ((kj >= 48) | ((kj >= 32) & (kj <= qi)))
    m_b0 = (qi >= 40) & ((kj < M) | (kb0 & (kj <= qi)))
    mask_b = m_mem | m_xb | m_xa | m_b0

    def w_ref(mi, g):
        return wch[(4, 0, 2)[mi] + g // GPC].at[g % GPC]

    def wo_rows(g, n=1):
        r0 = g * GW // 2
        return pltpu.bitcast(wo[r0:r0 + n * GW // 2, :], BF16)

    def seg_step(lhs, lhs_f32, extra, mask, lags, s_mid, filler):
        q, k, v, p, o = {}, {}, {}, {}, {}
        raw = ({}, {}, {})
        acc = [None]

        def proj(mi, g, dst):
            if mi == 0 and g == 0 and lhs_f32 is not None:
                y = None
                lp = jnp.concatenate([lhs_f32[16:], lhs_f32[0:16]], axis=0)
                for kt in range(D // 128):
                    w = pltpu.bitcast(w_ref(0, 0)[kt * 64:(kt + 1) * 64, :], BF16)
                    t = _dot(lp[:, kt * 128:(kt + 1) * 128].astype(BF16), w)
                    y = t if y is None else y + t
                nr = y.shape[0]
                y = jnp.concatenate([y[nr - 16:], y[0:nr - 16]], axis=0)
            else:
                y = _dot(lhs[mi], pltpu.bitcast(w_ref(mi, g)[...], BF16))
            for j in range(G):
                h = g * G + j
                yh = y[:, j * DH:(j + 1) * DH]
                ex = extra(mi, h)
                if ex:
                    yh = jnp.concatenate([yh] + ex, axis=0)
                raw[mi][h] = yh
                dst[h] = yh.astype(BF16)

        def sc(g):
            for h in range(g * G, (g + 1) * G):
                p[h] = _softmax_bf16(_dot_nt(q[h], k[h]), mask)

        def pv(g):
            o[g] = jnp.concatenate(
                [_dot(p[h], v[h]) for h in range(g * G, (g + 1) * G)], axis=1)

        def op(g):
            if merge and g == NG - 2:
                return
            if merge and g == NG - 1:
                y = _dot(jnp.concatenate([o[g - 1], o[g]], axis=1).astype(BF16),
                         wo_rows(g - 1, 2))
            else:
                y = _dot(o[g].astype(BF16), wo_rows(g))
            acc[0] = y if acc[0] is None else acc[0] + y

        ls, lp, lo, merge, pv0 = lags
        for t in range(2 * NG + lp + lo):
            if t < NG:
                proj(0, t, q)
                if s_mid and 0 <= t - ls < NG:
                    sc(t - ls)
                proj(1, t, k)
            elif t < 2 * NG:
                proj(2, t - NG, v)
            if 0 <= t - ls < NG and not s_mid:
                sc(t - ls)
            if t == NG + lp + pv0:
                pv(0)
                if s_mid:
                    for g in range(NG - ls, NG):
                        sc(g)
            if 0 < t - NG - lp < NG:
                pv(t - NG - lp)
            if pv0 > lo - 1 and t == NG + lp + lo + 1:
                op(0)
            if (1 if pv0 > lo - 1 else 0) <= t - NG - lp - lo < NG:
                op(t - NG - lp - lo)
            if t in filler:
                src = raw[1][t * G] if t < NG else raw[2][min(t - NG, NG - 1) * G]
                filler[t](src[0:8])
        return acc[0], raw

    subr = lax.broadcasted_iota(jnp.int32, (RC, 128), 0).astype(F32)

    def post_chunk(li, pi, valid, c, tie=None):
        if tie is not None:
            obuf[pl.ds(pl.multiple_of(anchor[0], 8), 8), 0:DH] = tie
        base = pi * PAIR if isinstance(pi, int) else pl.multiple_of(pi * PAIR, PAIR)
        rows = pl.ds(base + c * RC, RC)
        x0 = x_raw[pi, c * RC:(c + 1) * RC, :].astype(F32) if li == 0 else xres[rows, :]
        x1 = _rnd(x0 + _rnd(obuf[c * RC:(c + 1) * RC, :]))
        ln = _layernorm(x1)
        r = _rnd(jnp.sum(ln * wr, axis=-1, keepdims=True))
        r = jnp.broadcast_to(jnp.where(valid, r, -jnp.inf), (RC, 128))
        rb = rbest[...]
        better = r > rb
        rbest[...] = jnp.where(better, r, rb)
        row0 = jnp.asarray(base + (c * RC - PAD), jnp.int32).astype(F32)
        ibest[...] = jnp.where(better, subr + row0, ibest[...])
        x1buf[rows, :] = x1
        lbuf[rows, :] = ln
        if li == 0:
            x2 = _rnd(x1 + ln)
            xres[rows, :] = x2
            hbuf[rows, :] = _layernorm(x2)
        else:
            ostage[rows, :] = (x1 + ln).astype(BF16)

    def out_copy(row0, nrows):
        return pltpu.make_async_copy(ostage.at[pl.ds(PAD + row0, nrows)],
                                     out_hbm.at[pl.ds(row0, nrows)], osem)

    def pair_body(li, pi, mem, first):
        base = pl.multiple_of(pi * PAIR, PAIR)
        ha = hbuf[pl.ds(base + PAD, 40), :]
        hb = hbuf[pl.ds(base + PAD + 40, 24), :]
        fill = ({}, {})
        for c, (st, t) in enumerate(FILL[li]):
            fill[st][t] = functools.partial(post_chunk, li, pi, pi > 0, c)
        aq = jnp.concatenate([mem, ha[0:24]], axis=0)
        lhs_aq = aq.astype(BF16)
        if li == 0:
            p0 = pl.multiple_of(pi * 16, 16)
            lhs_akv = lhs_aq
            extra_a = lambda mi, h: [pre[(mi - 1) * NG + h // G, pl.ds(p0, 16),
                                         (h % G) * DH:(h % G + 1) * DH]] if mi else []
        else:
            lhs_akv = jnp.concatenate([mem, ha], axis=0).astype(BF16)
            extra_a = lambda mi, h: []
        acc_a, prj = seg_step((lhs_aq, lhs_akv, lhs_akv), None if first else aq, extra_a, mask_a,
                              LAGA, SMID[0], fill[0])
        lhs_b = jnp.concatenate([acc_a[0:8], hb], axis=0).astype(BF16)
        bq = jnp.concatenate([acc_a[0:8], hb, ha[24:40]], axis=0)
        acc_b, _ = seg_step(
            (bq.astype(BF16), lhs_b, lhs_b), bq,
            lambda mi, h: [prj[mi][h][32:48], prj[mi][h][0:32]] if mi else [],
            mask_b, LAGB, SMID[1], fill[1])
        obuf[0:24, :] = acc_a[8:32]
        obuf[24:40, :] = acc_b[32:48]
        obuf[40:64, :] = acc_b[8:32]
        return acc_b[0:8]

    def loop_body(li, it, mem):
        UNROLL = UNROLLS[li]
        for u in range(UNROLL):
            mem = pair_body(li, it * UNROLL + u, mem, u == 0 and not KS0)

        if li == 1:
            @pl.when(it > 0)
            def _():
                out_copy(pl.multiple_of(it * (UNROLL * PAIR) - PAIR, PAIR),
                         UNROLL * PAIR).start()

            if UNROLL > 1:
                @pl.when(it == 0)
                def _():
                    out_copy(0, (UNROLL - 1) * PAIR).start()

        return mem

    for li in range(2):
        obuf[0:PAIR, :] = jnp.zeros((PAIR, D), F32)
        rbest[...] = jnp.full((RC, 128), -jnp.inf, F32)
        ibest[...] = jnp.zeros((RC, 128), F32)
        lax.fori_loop(0, NPAIR // UNROLLS[li], functools.partial(loop_body, li),
                      mem0_v[...].astype(F32))

        if li == 0:
            for c in cp_mlp:
                c.wait()
        else:
            out_copy(0, S - PAIR).wait()

        def top1():
            rb = rbest[...]
            rmax = jnp.max(rb, axis=0, keepdims=True)
            imin = jnp.min(jnp.where(rb == rmax, ibest[...], S - 1.0), axis=0, keepdims=True)
            return rmax, imin.astype(jnp.int32)[0, 0]

        def mod_trip(carry, li=li):
            rmax, idx = top1()
            lsel = lbuf[pl.ds(PAD + idx, 1), :]
            for c in range(PAIR // RC):
                post_chunk(li, NPAIR, True, c)
            xs = jnp.broadcast_to(lsel, (16, D)).astype(BF16)
            acts = []
            for f0, f1 in FSPLIT:
                gpre = _rnd(_dot(xs, wg_v[:, f0:f1]))
                gate = _rnd(gpre * _rnd(jax.nn.sigmoid(gpre)))
                up = _rnd(_dot(xs, wu_v[:, f0:f1]))
                acts.append((gate * up).astype(BF16))
            y = None
            for (f0, f1), act in zip(FSPLIT, acts):
                t = _dot(act, wd_v[f0:f1, :])
                y = t if y is None else y + t
            y = _rnd(y)[0:8]
            rsel = _rnd(jax.nn.sigmoid(rmax[:, 0:1]))
            ybuf[...] = _rnd(y * rsel)
            return idx, top1()[1]

        idx, _ = lax.while_loop(lambda cr: cr[0] != cr[1], mod_trip,
                                (jnp.int32(-1), jnp.int32(0)))
        row = pl.ds(PAD + idx, 1)
        lsel = lbuf[row, :]
        y = ybuf[0:1, :]
        if li == 0:
            x2 = _rnd(x1buf[row, :] + _rnd(lsel + y))
            xres[row, :] = x2
            hbuf[row, :] = _layernorm(x2)
        else:
            t0 = pl.multiple_of((idx // 16) * 16, 16)
            tile = pl.ds(PAD + t0, 16)
            sel = lax.broadcasted_iota(jnp.int32, (16, D), 0) == idx - t0
            upd = jnp.where(sel, jnp.broadcast_to(y, (16, D)), 0.0)
            ostage[tile, :] = (x1buf[tile, :] + _rnd(lbuf[tile, :] + upd)).astype(BF16)
            t1 = pl.multiple_of(jnp.minimum(t0, S - PAIR - 16), 16)
            out_copy(S - PAIR, PAIR).start()
            out_copy(t1, 16).start()
            out_copy(0, PAIR + 16).wait()


_FILL = ((0, 9), (0, 11), (0, 13), (0, 15), (1, 9), (1, 11), (1, 13), (1, 14))
CFG = dict(UNROLLS=(2, 2), LAGA=(1, 1, 2, True, 0), LAGB=(1, 1, 2, False, 1), FILL=(_FILL, _FILL),
           SMID=(False, True), LNP=16, LNA=16, SLACK=(128, 256), KS0=False, LNTIE=1)


def _build():
    any_spec = pl.BlockSpec(memory_space=pl.ANY)
    return pl.pallas_call(
        functools.partial(_kernel, **CFG),
        out_shape=jax.ShapeDtypeStruct((S, D), BF16),
        in_specs=[any_spec] * 10,
        out_specs=any_spec,
        scratch_shapes=[
            pltpu.VMEM((NPAIR + 2, PAIR, D), BF16),
            pltpu.VMEM((M, D), BF16),
            pltpu.VMEM((D,), BF16),
            pltpu.VMEM((NCH * D + 1, HC, DH), BF16),
            pltpu.VMEM((HD + 16, D), BF16),
            pltpu.VMEM((D, FF), BF16),
            pltpu.VMEM((D, FF), BF16),
            pltpu.VMEM((FF, D), BF16),
        ] + [pltpu.VMEM((GPC, D // 2, GW), U32)] * NCH + [
            pltpu.VMEM((HD // 2, D), U32),
            pltpu.VMEM((NTMP * TSZ, DH), U32),
            pltpu.VMEM((PAD + S, D), F32),
            pltpu.VMEM((PAD + S, D), F32),
            pltpu.VMEM((PAD + S, D), F32),
            pltpu.VMEM((PAD + S, D), F32),
            pltpu.VMEM((RC, 128), F32),
            pltpu.VMEM((RC, 128), F32),
            pltpu.VMEM((PAIR + 8, D), F32),
            pltpu.VMEM((PAD + S, D), BF16),
            pltpu.VMEM((8 * NPAIR, D), U32),
            pltpu.VMEM((2 * NG, 16 * NPAIR, GW), F32),
            pltpu.VMEM((8, D), F32),
            pltpu.SMEM((4,), jnp.int32),
            pltpu.SemaphoreType.DMA((27,)),
            pltpu.SemaphoreType.DMA(()),
        ],
        compiler_params=pltpu.CompilerParams(vmem_limit_bytes=120 * 1024 * 1024),
    )


@jax.jit
def pallas_interleave_layers__memory_aug_recurrent_mem_tr__moe_arch_mod__prompt_kernel(
    A_x: jax.Array,
    A_mem0: jax.Array,
    A_Wq: jax.Array,
    A_Wk: jax.Array,
    A_Wv: jax.Array,
    A_Wo: jax.Array,
    A_seg_len,
    B_x: jax.Array,
    B_w_r: jax.Array,
    B_w_gate: jax.Array,
    B_w_up: jax.Array,
    B_w_down: jax.Array,
):
    assert A_x.shape == (1, S, D) and A_mem0.shape == (1, M, D) and A_Wq.shape == (D, H, DH)
    del A_seg_len
    del B_x
    out = _build()(
        A_x.reshape(NPAIR, PAIR, D),
        A_mem0.reshape(M, D),
        A_Wq,
        A_Wk,
        A_Wv,
        A_Wo.reshape(HD, D),
        B_w_r,
        B_w_gate,
        B_w_up,
        B_w_down,
    )
    return out.reshape(1, S, D)
```

```python
import functools
import math

import jax
import jax.numpy as jnp
from jax import lax
import jax.experimental.pallas as pl
import jax.experimental.pallas.tpu as pltpu

F32 = jnp.float32
BF16 = jnp.bfloat16
U32 = jnp.uint32

S, D, H, DH, M, SEG = 2048, 512, 32, 128, 8, 32
FF = 1792
HD = H * DH
PAIR = 2 * SEG
NPAIR = S // PAIR
PAD = PAIR
G = 4
NG = H // G
GW = G * DH
HC = 16
GPC = HC // G
NCH = 3 * H // HC
TP = 20
TSZ = 8 * TP
NTMP = 8
FSPLIT = ((0, 1024), (1024, FF))
RC = 8
LN_EPS = 1e-05
NEG = -1000000000.0 * DH ** 0.5
EXP2_SCALE = (DH ** -0.5) * math.log2(math.e)


def _rnd(x):
    return x.astype(BF16).astype(F32)


def _layernorm(x):
    mean = jnp.sum(x, axis=-1, keepdims=True) * (1.0 / D)
    c = x - mean
    var = jnp.sum(c * c, axis=-1, keepdims=True) * (1.0 / D)
    z = _rnd(_rnd(var) + _rnd(jnp.float32(LN_EPS)))
    den = _rnd(z * lax.rsqrt(z))
    inv = pl.reciprocal(den, approx=True)
    inv = inv * (2.0 - den * inv)
    return _rnd(_rnd(x - _rnd(mean)) * inv)


def _dot(a, b):
    return jnp.dot(a, b, preferred_element_type=F32)


def _dot_nt(a, b):
    return lax.dot_general(a, b, (((1,), (1,)), ((), ())), preferred_element_type=F32)


def _softmax_bf16(s, mask):
    s = jnp.where(mask, s, NEG)
    m = jnp.max(s, axis=-1, keepdims=True)
    e = jnp.exp2((s - m) * EXP2_SCALE)
    l = jnp.sum(e, axis=-1, keepdims=True)
    r = pl.reciprocal(l, approx=True)
    r = r * (2.0 - l * r)
    return (e * r).astype(BF16)


def _kernel(x_hbm, mem0_hbm, wq_hbm, wk_hbm, wv_hbm, wo_hbm, wr_hbm, wg_hbm, wu_hbm, wd_hbm,
            out_hbm,
            x_raw, mem0_v, wr_v, stage, wo_raw, wg_v, wu_v, wd_v,
            wk0, wk1, wv0, wv1, wq0, wq1, wo, tmp,
            xres, x1buf, lbuf, hbuf, rbest, ibest, obuf, ostage,
            lhs_pre, pre, ybuf, anchor, sems, osem, *,
            UNROLLS, LAGA, LAGB, FILL, SMID, LNP, LNA, SLACK, KS0, LNTIE):
    wch = (wk0, wk1, wv0, wv1, wq0, wq1)
    NWO = 4
    WOP = HD // NWO
    WPARTS = (4, 2, 2, 1, 4, 4)
    SEM_X = 0
    SEM_W = [3 + sum(WPARTS[:c]) for c in range(NCH)]
    SEM_O = 3 + sum(WPARTS)
    SEM_MISC = SEM_O + NWO

    def cp_x(i):
        r0, nr = ((24, 16), (0, 24), (40, 24))[i]
        return pltpu.make_async_copy(x_hbm.at[:, pl.ds(r0, nr), :],
                                     x_raw.at[pl.ds(1, NPAIR), pl.ds(r0, nr), :],
                                     sems.at[SEM_X + i])

    def cp_w(c, part):
        w = (wk_hbm, wv_hbm, wq_hbm)[c // 2]
        nd = D // WPARTS[c]
        return pltpu.make_async_copy(
            w.at[pl.ds(part * nd, nd), pl.ds((c % 2) * HC, HC), :],
            stage.at[pl.ds(c * D + part * nd, nd)], sems.at[SEM_W[c] + part])

    def cp_o(i):
        return pltpu.make_async_copy(wo_hbm.at[pl.ds(i * WOP, WOP)],
                                     wo_raw.at[pl.ds(i * WOP, WOP)], sems.at[SEM_O + i])

    cp_small = [pltpu.make_async_copy(s_, d_, sems.at[SEM_MISC + i])
                for i, (s_, d_) in enumerate(((mem0_hbm, mem0_v), (wr_hbm, wr_v)))]
    cp_mlp = [pltpu.make_async_copy(s_, d_, sems.at[SEM_MISC + 2 + i])
              for i, (s_, d_) in enumerate(((wg_hbm, wg_v), (wu_hbm, wu_v), (wd_hbm, wd_v)))]
    cp_x(0).start()
    for c in range(3):
        for part in range(WPARTS[c]):
            cp_w(c, part).start()
    cp_x(1).start()
    cp_x(2).start()
    cp_w(3, 0).start()
    for i in range(NWO):
        cp_w(4, i).start()
        cp_w(5, i).start()
        cp_o(i).start()
    for c in cp_small + cp_mlp:
        c.start()

    anchor[0] = PAIR
    anchor[1] = NCH * D
    anchor[2] = HD
    anchor[3] = NPAIR + 1
    x_raw[0] = jnp.zeros((PAIR, D), BF16)
    xres[0:PAD, :] = jnp.zeros((PAD, D), F32)

    cp_x(0).wait()

    def ln_mid(i, carry):
        for pp in range(LNP):
            pr = i * LNP + pp
            ln = _layernorm(x_raw[1 + pr, 24:40, :].astype(F32))
            hbuf[pl.ds(pl.multiple_of(PAD + pr * PAIR + 24, 8), 16), :] = ln
            lhs_pre[pl.ds(pl.multiple_of(pr * 8, 8), 8), :] = pltpu.bitcast(ln.astype(BF16), U32)
        return carry

    lax.fori_loop(0, NPAIR // LNP, ln_mid, 0)

    def ln_jobs(p0, npairs):
        def job(pp, r0):
            ln = _layernorm(x_raw[1 + p0 + pp, r0:r0 + 8, :].astype(F32))
            hbuf[pl.ds(pl.multiple_of(PAD + (p0 + pp) * PAIR + r0, 8), 8), :] = ln

        return [('x_raw', functools.partial(job, pp, r0))
                for pp in range(npairs) for r0 in (0, 8, 16, 40, 48, 56)]

    def relayout_jobs(c, blk0, nblk, slot0=0):
        def job(u):
            t0 = ((slot0 + u) % NTMP) * TSZ
            d0 = pl.multiple_of(c * D + (blk0 + u) * 16, 16)
            raw = pltpu.bitcast(stage[pl.ds(d0, 16), :, :], U32)
            for i in range(8):
                ev, od = raw[2 * i], raw[2 * i + 1]
                lo = (ev & jnp.uint32(0xFFFF)) | (od << 16)
                hi = (ev >> 16) | (od & jnp.uint32(0xFFFF0000))
                tmp[pl.ds(t0 + i * TP, 8, stride=2), :] = lo
                tmp[pl.ds(t0 + i * TP + 1, 8, stride=2), :] = hi
            o0 = pl.multiple_of((blk0 + u) * 8, 8)
            for hh in range(HC):
                col = (hh % G) * DH
                wch[c][hh // G, pl.ds(o0, 8), col:col + DH] = tmp[pl.ds(t0 + hh, 8, stride=TP), :]

        return [('stage', functools.partial(job, u)) for u in range(nblk)]

    def repack_jobs(part):
        def job(c):
            r0 = pl.multiple_of(part * WOP + c * 128, 128)
            o0 = pl.multiple_of(part * (WOP // 2) + c * 64, 64)
            wo[pl.ds(o0, 64), :] = pltpu.bitcast(wo_raw[pl.ds(r0, 128), :], U32)

        return [('wo_raw', functools.partial(job, c)) for c in range(WOP // 128)]

    def interleave(*lists):
        keyed = [((i + 0.5) / len(l), n, j) for n, l in enumerate(lists) for i, j in enumerate(l)]
        return [j for _, _, j in sorted(keyed, key=lambda t: t[:2])]

    def precompute(c, g0, ng, jobs, k0=0, k1=D):
        lhs = pltpu.bitcast(lhs_pre[:, k0:k1], BF16)
        ys = [_dot(lhs, pltpu.bitcast(wch[c][g0 + gg, k0 // 2:k1 // 2, :], BF16))
              for gg in range(ng)]
        nrow = 16 * NPAIR
        has_ln = any(kind == 'x_raw' for kind, _ in jobs)
        nln = 0
        for u, (kind, job) in enumerate(jobs):
            nln += kind == 'x_raw'
            if u > 0 and (kind != 'x_raw' or nln % LNTIE == 0):
                par = D // (k1 - k0)
                span = ng * G * nrow // par - (SLACK[1] if has_ln else SLACK[0])
                pos = max((u * span // len(jobs)) // 16 * 16 - 128, 0)
                nt, r0 = pos // nrow * par, pos % nrow
                tie = ys[nt // G][r0:r0 + 16, (nt % G) * DH:(nt % G + 1) * DH].astype(BF16)
                if kind == 'stage':
                    stage[anchor[1]] = tie
                elif kind == 'x_raw':
                    x_raw[anchor[3], 0:16, 0:DH] = tie
                else:
                    wo_raw[pl.ds(pl.multiple_of(anchor[2], 16), 16), 0:DH] = tie
            job()
        for gg in range(ng):
            if k0 > 0:
                pre[c * GPC + g0 + gg] += ys[gg]
            else:
                pre[c * GPC + g0 + gg] = ys[gg]

    def run(jobs):
        for _, job in jobs:
            job()

    NBLK = D // 16

    HB, QB = NBLK // 2, NBLK // 4
    cp_w(0, 0).wait()
    run(relayout_jobs(0, 0, QB))
    precompute(0, 0, GPC, [], 0, D // 4)
    cp_w(0, 1).wait()
    run(relayout_jobs(0, QB, QB))
    cp_w(0, 2).wait()
    cp_w(0, 3).wait()
    precompute(0, 0, GPC, relayout_jobs(0, HB, HB), D // 4, D // 2)

    def phase01(c, k0, it, carry):
        cp_w(c + 1, it).wait()
        precompute(c, it * 2, 2, relayout_jobs(c + 1, it * HB, HB), k0, D)
        return carry

    lax.fori_loop(0, 2, functools.partial(phase01, 0, D // 2), 0)
    lax.fori_loop(0, 2, functools.partial(phase01, 1, 0), 0)
    cp_x(1).wait()
    cp_x(2).wait()
    cp_w(3, 0).wait()
    lax.fori_loop(0, 2, lambda it, cr: (
        precompute(2, it * 2, 2, interleave(relayout_jobs(3, it * HB, HB),
                                            ln_jobs(it * LNA, LNA))), cr)[1], 0)
    LNB = (NPAIR - 2 * LNA) // 4

    def last_phase(it, carry):
        cp_w(4, it).wait()
        cp_w(5, it).wait()
        cp_o(it).wait()
        precompute(3, it, 1, interleave(relayout_jobs(4, it * QB, QB),
                                        relayout_jobs(5, it * QB, QB, NTMP // 2),
                                        repack_jobs(it),
                                        ln_jobs(2 * LNA + it * LNB, LNB)))
        return carry

    lax.fori_loop(0, 4, last_phase, 0)

    for c in cp_small:
        c.wait()
    wr = wr_v[...].astype(F32).reshape(1, D)

    qi = lax.broadcasted_iota(jnp.int32, (32, 48), 0)
    kj = lax.broadcasted_iota(jnp.int32, (32, 48), 1)
    mask_a = (kj < 40) & ((qi < M) | (kj <= qi))
    qi = lax.broadcasted_iota(jnp.int32, (48, 80), 0)
    kj = lax.broadcasted_iota(jnp.int32, (48, 80), 1)
    kb0 = (kj >= 40) & (kj < 48)
    m_mem = (qi < M) & ((kj < 32) | kb0)
    m_xb = (qi >= M) & (qi < 32) & ((kj <= qi) | kb0)
    m_xa = (qi >= 32) & (qi < 40) & ((kj >= 48) | ((kj >= 32) & (kj <= qi)))
    m_b0 = (qi >= 40) & ((kj < M) | (kb0 & (kj <= qi)))
    mask_b = m_mem | m_xb | m_xa | m_b0

    def w_ref(mi, g):
        return wch[(4, 0, 2)[mi] + g // GPC].at[g % GPC]

    def wo_rows(g, n=1):
        r0 = g * GW // 2
        return pltpu.bitcast(wo[r0:r0 + n * GW // 2, :], BF16)

    def seg_step(lhs, lhs_f32, extra, mask, lags, s_mid, filler):
        q, k, v, p, o = {}, {}, {}, {}, {}
        raw = ({}, {}, {})
        acc = [None]

        def proj(mi, g, dst):
            if mi == 0 and g == 0 and lhs_f32 is not None:
                y = None
                lp = jnp.concatenate([lhs_f32[16:], lhs_f32[0:16]], axis=0)
                for kt in range(D // 128):
                    w = pltpu.bitcast(w_ref(0, 0)[kt * 64:(kt + 1) * 64, :], BF16)
                    t = _dot(lp[:, kt * 128:(kt + 1) * 128].astype(BF16), w)
                    y = t if y is None else y + t
                nr = y.shape[0]
                y = jnp.concatenate([y[nr - 16:], y[0:nr - 16]], axis=0)
            else:
                y = _dot(lhs[mi], pltpu.bitcast(w_ref(mi, g)[...], BF16))
            for j in range(G):
                h = g * G + j
                yh = y[:, j * DH:(j + 1) * DH]
                ex = extra(mi, h)
                if ex:
                    yh = jnp.concatenate([yh] + ex, axis=0)
                raw[mi][h] = yh
                dst[h] = yh.astype(BF16)

        def sc(g):
            for h in range(g * G, (g + 1) * G):
                p[h] = _softmax_bf16(_dot_nt(q[h], k[h]), mask)

        def pv(g):
            o[g] = jnp.concatenate(
                [_dot(p[h], v[h]) for h in range(g * G, (g + 1) * G)], axis=1)

        def op(g):
            if merge and g == NG - 2:
                return
            if merge and g == NG - 1:
                y = _dot(jnp.concatenate([o[g - 1], o[g]], axis=1).astype(BF16),
                         wo_rows(g - 1, 2))
            else:
                y = _dot(o[g].astype(BF16), wo_rows(g))
            acc[0] = y if acc[0] is None else acc[0] + y

        ls, lp, lo, merge, pv0 = lags
        for t in range(2 * NG + lp + lo):
            if t < NG:
                proj(0, t, q)
                if s_mid and 0 <= t - ls < NG:
                    sc(t - ls)
                proj(1, t, k)
            elif t < 2 * NG:
                proj(2, t - NG, v)
            if 0 <= t - ls < NG and not s_mid:
                sc(t - ls)
            if t == NG + lp + pv0:
                pv(0)
                if s_mid:
                    for g in range(NG - ls, NG):
                        sc(g)
            if 0 < t - NG - lp < NG:
                pv(t - NG - lp)
            if pv0 > lo - 1 and t == NG + lp + lo + 1:
                op(0)
            if (1 if pv0 > lo - 1 else 0) <= t - NG - lp - lo < NG:
                op(t - NG - lp - lo)
            if t in filler:
                src = raw[1][t * G] if t < NG else raw[2][min(t - NG, NG - 1) * G]
                filler[t](src[0:8])
        return acc[0], raw

    subr = lax.broadcasted_iota(jnp.int32, (RC, 128), 0).astype(F32)

    def post_chunk(li, pi, valid, c, tie=None):
        if tie is not None:
            obuf[pl.ds(pl.multiple_of(anchor[0], 8), 8), 0:DH] = tie
        base = pi * PAIR if isinstance(pi, int) else pl.multiple_of(pi * PAIR, PAIR)
        rows = pl.ds(base + c * RC, RC)
        x0 = x_raw[pi, c * RC:(c + 1) * RC, :].astype(F32) if li == 0 else xres[rows, :]
        x1 = _rnd(x0 + _rnd(obuf[c * RC:(c + 1) * RC, :]))
        ln = _layernorm(x1)
        r = _rnd(jnp.sum(ln * wr, axis=-1, keepdims=True))
        r = jnp.broadcast_to(jnp.where(valid, r, -jnp.inf), (RC, 128))
        rb = rbest[...]
        better = r > rb
        rbest[...] = jnp.where(better, r, rb)
        row0 = jnp.asarray(base + (c * RC - PAD), jnp.int32).astype(F32)
        ibest[...] = jnp.where(better, subr + row0, ibest[...])
        x1buf[rows, :] = x1
        lbuf[rows, :] = ln
        if li == 0:
            x2 = _rnd(x1 + ln)
            xres[rows, :] = x2
            hbuf[rows, :] = _layernorm(x2)
        else:
            ostage[rows, :] = (x1 + ln).astype(BF16)

    def out_copy(row0, nrows):
        return pltpu.make_async_copy(ostage.at[pl.ds(PAD + row0, nrows)],
                                     out_hbm.at[pl.ds(row0, nrows)], osem)

    def pair_body(li, pi, mem, first):
        base = pl.multiple_of(pi * PAIR, PAIR)
        ha = hbuf[pl.ds(base + PAD, 40), :]
        hb = hbuf[pl.ds(base + PAD + 40, 24), :]
        fill = ({}, {})
        for c, (st, t) in enumerate(FILL[li]):
            fill[st][t] = functools.partial(post_chunk, li, pi, pi > 0, c)
        aq = jnp.concatenate([mem, ha[0:24]], axis=0)
        lhs_aq = aq.astype(BF16)
        if li == 0:
            p0 = pl.multiple_of(pi * 16, 16)
            lhs_akv = lhs_aq
            extra_a = lambda mi, h: [pre[(mi - 1) * NG + h // G, pl.ds(p0, 16),
                                         (h % G) * DH:(h % G + 1) * DH]] if mi else []
        else:
            lhs_akv = jnp.concatenate([mem, ha], axis=0).astype(BF16)
            extra_a = lambda mi, h: []
        acc_a, prj = seg_step((lhs_aq, lhs_akv, lhs_akv), None if first else aq, extra_a, mask_a,
                              LAGA, SMID[0], fill[0])
        lhs_b = jnp.concatenate([acc_a[0:8], hb], axis=0).astype(BF16)
        bq = jnp.concatenate([acc_a[0:8], hb, ha[24:40]], axis=0)
        acc_b, _ = seg_step(
            (bq.astype(BF16), lhs_b, lhs_b), bq,
            lambda mi, h: [prj[mi][h][32:48], prj[mi][h][0:32]] if mi else [],
            mask_b, LAGB, SMID[1], fill[1])
        obuf[0:24, :] = acc_a[8:32]
        obuf[24:40, :] = acc_b[32:48]
        obuf[40:64, :] = acc_b[8:32]
        return acc_b[0:8]

    def loop_body(li, it, mem):
        UNROLL = UNROLLS[li]
        for u in range(UNROLL):
            mem = pair_body(li, it * UNROLL + u, mem, u == 0 and not KS0)

        if li == 1:
            @pl.when(it > 0)
            def _():
                out_copy(pl.multiple_of(it * (UNROLL * PAIR) - PAIR, PAIR),
                         UNROLL * PAIR).start()

            if UNROLL > 1:
                @pl.when(it == 0)
                def _():
                    out_copy(0, (UNROLL - 1) * PAIR).start()

        return mem

    for li in range(2):
        obuf[0:PAIR, :] = jnp.zeros((PAIR, D), F32)
        rbest[...] = jnp.full((RC, 128), -jnp.inf, F32)
        ibest[...] = jnp.zeros((RC, 128), F32)
        lax.fori_loop(0, NPAIR // UNROLLS[li], functools.partial(loop_body, li),
                      mem0_v[...].astype(F32))

        if li == 0:
            for c in cp_mlp:
                c.wait()
        else:
            out_copy(0, S - PAIR).wait()

        def top1():
            rb = rbest[...]
            rmax = jnp.max(rb, axis=0, keepdims=True)
            imin = jnp.min(jnp.where(rb == rmax, ibest[...], S - 1.0), axis=0, keepdims=True)
            return rmax, imin.astype(jnp.int32)[0, 0]

        def mod_trip(carry, li=li):
            rmax, idx = top1()
            lsel = lbuf[pl.ds(PAD + idx, 1), :]
            for c in range(PAIR // RC):
                post_chunk(li, NPAIR, True, c)
            xs = jnp.broadcast_to(lsel, (16, D)).astype(BF16)
            acts = []
            for f0, f1 in FSPLIT:
                gpre = _rnd(_dot(xs, wg_v[:, f0:f1]))
                gate = _rnd(gpre * _rnd(jax.nn.sigmoid(gpre)))
                up = _rnd(_dot(xs, wu_v[:, f0:f1]))
                acts.append((gate * up).astype(BF16))
            y = None
            for (f0, f1), act in zip(FSPLIT, acts):
                t = _dot(act, wd_v[f0:f1, :])
                y = t if y is None else y + t
            y = _rnd(y)[0:8]
            rsel = _rnd(jax.nn.sigmoid(rmax[:, 0:1]))
            ybuf[...] = _rnd(y * rsel)
            return idx, top1()[1]

        idx, _ = lax.while_loop(lambda cr: cr[0] != cr[1], mod_trip,
                                (jnp.int32(-1), jnp.int32(0)))
        row = pl.ds(PAD + idx, 1)
        lsel = lbuf[row, :]
        y = ybuf[0:1, :]
        if li == 0:
            x2 = _rnd(x1buf[row, :] + _rnd(lsel + y))
            xres[row, :] = x2
            hbuf[row, :] = _layernorm(x2)
        else:
            t0 = pl.multiple_of((idx // 16) * 16, 16)
            tile = pl.ds(PAD + t0, 16)
            sel = lax.broadcasted_iota(jnp.int32, (16, D), 0) == idx - t0
            upd = jnp.where(sel, jnp.broadcast_to(y, (16, D)), 0.0)
            ostage[tile, :] = (x1buf[tile, :] + _rnd(lbuf[tile, :] + upd)).astype(BF16)
            t1 = pl.multiple_of(jnp.minimum(t0, S - PAIR - 16), 16)
            out_copy(S - PAIR, PAIR).start()
            out_copy(t1, 16).start()
            out_copy(0, PAIR + 16).wait()


_FILL = ((0, 9), (0, 12), (0, 15), (1, 8), (1, 10), (1, 12), (1, 14), (1, 15))
CFG = dict(UNROLLS=(2, 2), LAGA=(1, 1, 2, True, 0), LAGB=(1, 1, 2, False, 1), FILL=(_FILL, _FILL),
           SMID=(False, True), LNP=16, LNA=16, SLACK=(128, 256), KS0=False, LNTIE=1)


def _build():
    any_spec = pl.BlockSpec(memory_space=pl.ANY)
    return pl.pallas_call(
        functools.partial(_kernel, **CFG),
        out_shape=jax.ShapeDtypeStruct((S, D), BF16),
        in_specs=[any_spec] * 10,
        out_specs=any_spec,
        scratch_shapes=[
            pltpu.VMEM((NPAIR + 2, PAIR, D), BF16),
            pltpu.VMEM((M, D), BF16),
            pltpu.VMEM((D,), BF16),
            pltpu.VMEM((NCH * D + 1, HC, DH), BF16),
            pltpu.VMEM((HD + 16, D), BF16),
            pltpu.VMEM((D, FF), BF16),
            pltpu.VMEM((D, FF), BF16),
            pltpu.VMEM((FF, D), BF16),
        ] + [pltpu.VMEM((GPC, D // 2, GW), U32)] * NCH + [
            pltpu.VMEM((HD // 2, D), U32),
            pltpu.VMEM((NTMP * TSZ, DH), U32),
            pltpu.VMEM((PAD + S, D), F32),
            pltpu.VMEM((PAD + S, D), F32),
            pltpu.VMEM((PAD + S, D), F32),
            pltpu.VMEM((PAD + S, D), F32),
            pltpu.VMEM((RC, 128), F32),
            pltpu.VMEM((RC, 128), F32),
            pltpu.VMEM((PAIR + 8, D), F32),
            pltpu.VMEM((PAD + S, D), BF16),
            pltpu.VMEM((8 * NPAIR, D), U32),
            pltpu.VMEM((2 * NG, 16 * NPAIR, GW), F32),
            pltpu.VMEM((8, D), F32),
            pltpu.SMEM((4,), jnp.int32),
            pltpu.SemaphoreType.DMA((29,)),
            pltpu.SemaphoreType.DMA(()),
        ],
        compiler_params=pltpu.CompilerParams(vmem_limit_bytes=120 * 1024 * 1024),
    )


@jax.jit
def pallas_interleave_layers__memory_aug_recurrent_mem_tr__moe_arch_mod__prompt_kernel(
    A_x: jax.Array,
    A_mem0: jax.Array,
    A_Wq: jax.Array,
    A_Wk: jax.Array,
    A_Wv: jax.Array,
    A_Wo: jax.Array,
    A_seg_len,
    B_x: jax.Array,
    B_w_r: jax.Array,
    B_w_gate: jax.Array,
    B_w_up: jax.Array,
    B_w_down: jax.Array,
):
    assert A_x.shape == (1, S, D) and A_mem0.shape == (1, M, D) and A_Wq.shape == (D, H, DH)
    del A_seg_len
    del B_x
    out = _build()(
        A_x.reshape(NPAIR, PAIR, D),
        A_mem0.reshape(M, D),
        A_Wq,
        A_Wk,
        A_Wv,
        A_Wo.reshape(HD, D),
        B_w_r,
        B_w_gate,
        B_w_up,
        B_w_down,
    )
    return out.reshape(1, S, D)
```

```python
import functools
import math

import jax
import jax.numpy as jnp
from jax import lax
import jax.experimental.pallas as pl
import jax.experimental.pallas.tpu as pltpu

F32 = jnp.float32
BF16 = jnp.bfloat16
U32 = jnp.uint32

S, D, H, DH, M, SEG = 2048, 512, 32, 128, 8, 32
FF = 1792
HD = H * DH
PAIR = 2 * SEG
NPAIR = S // PAIR
PAD = PAIR
G = 4
NG = H // G
GW = G * DH
HC = 16
GPC = HC // G
NCH = 3 * H // HC
TP = 20
TSZ = 8 * TP
NTMP = 8
FSPLIT = ((0, 1024), (1024, FF))
RC = 8
LN_EPS = 1e-05
NEG = -1000000000.0 * DH ** 0.5
EXP2_SCALE = (DH ** -0.5) * math.log2(math.e)


def _rnd(x):
    return x.astype(BF16).astype(F32)


def _layernorm(x):
    mean = jnp.sum(x, axis=-1, keepdims=True) * (1.0 / D)
    c = x - mean
    var = jnp.sum(c * c, axis=-1, keepdims=True) * (1.0 / D)
    z = _rnd(_rnd(var) + _rnd(jnp.float32(LN_EPS)))
    finite = z < jnp.inf
    den = _rnd(z * lax.rsqrt(z))
    inv = pl.reciprocal(den, approx=True)
    inv = jnp.where(finite, inv * (2.0 - den * inv), 0.0)
    return _rnd(_rnd(x - _rnd(mean)) * inv)


def _dot(a, b):
    return jnp.dot(a, b, preferred_element_type=F32)


def _dot_nt(a, b):
    return lax.dot_general(a, b, (((1,), (1,)), ((), ())), preferred_element_type=F32)


def _softmax_bf16(s, mask):
    s = jnp.where(mask, s, NEG)
    m = jnp.max(s, axis=-1, keepdims=True)
    e = jnp.exp2((s - m) * EXP2_SCALE)
    l = jnp.sum(e, axis=-1, keepdims=True)
    r = pl.reciprocal(l, approx=True)
    r = r * (2.0 - l * r)
    return (e * r).astype(BF16)


def _kernel(x_hbm, mem0_hbm, wq_hbm, wk_hbm, wv_hbm, wo_hbm, wr_hbm, wg_hbm, wu_hbm, wd_hbm,
            out_hbm,
            x_raw, mem0_v, wr_v, stage, wo_raw, wg_v, wu_v, wd_v,
            wk0, wk1, wv0, wv1, wq0, wq1, wo, tmp,
            xres, x1buf, lbuf, hbuf, rbest, ibest, obuf, ostage,
            lhs_pre, pre, ybuf, anchor, sems, osem, *,
            UNROLLS, LAGA, LAGB, FILL, SMID, LNP, SLACK):
    wch = (wk0, wk1, wv0, wv1, wq0, wq1)
    NWO = 4
    WOP = HD // NWO
    WPARTS = (4, 2, 2, 1, 4, 4)
    SEM_X = 0
    SEM_W = [3 + sum(WPARTS[:c]) for c in range(NCH)]
    SEM_O = 3 + sum(WPARTS)
    SEM_MISC = SEM_O + NWO

    def cp_x(i):
        r0, nr = ((24, 16), (0, 24), (40, 24))[i]
        return pltpu.make_async_copy(x_hbm.at[:, pl.ds(r0, nr), :],
                                     x_raw.at[pl.ds(1, NPAIR), pl.ds(r0, nr), :],
                                     sems.at[SEM_X + i])

    def cp_w(c, part):
        w = (wk_hbm, wv_hbm, wq_hbm)[c // 2]
        nd = D // WPARTS[c]
        return pltpu.make_async_copy(
            w.at[pl.ds(part * nd, nd), pl.ds((c % 2) * HC, HC), :],
            stage.at[pl.ds(c * D + part * nd, nd)], sems.at[SEM_W[c] + part])

    def cp_o(i):
        return pltpu.make_async_copy(wo_hbm.at[pl.ds(i * WOP, WOP)],
                                     wo_raw.at[pl.ds(i * WOP, WOP)], sems.at[SEM_O + i])

    cp_small = [pltpu.make_async_copy(s_, d_, sems.at[SEM_MISC + i])
                for i, (s_, d_) in enumerate(((mem0_hbm, mem0_v), (wr_hbm, wr_v)))]
    cp_mlp = [pltpu.make_async_copy(s_, d_, sems.at[SEM_MISC + 2 + i])
              for i, (s_, d_) in enumerate(((wg_hbm, wg_v), (wu_hbm, wu_v), (wd_hbm, wd_v)))]
    cp_x(0).start()
    for c in range(3):
        for part in range(WPARTS[c]):
            cp_w(c, part).start()
    cp_x(1).start()
    cp_x(2).start()
    cp_w(3, 0).start()
    for i in range(NWO):
        cp_w(4, i).start()
        cp_w(5, i).start()
        cp_o(i).start()
    for c in cp_small + cp_mlp:
        c.start()

    anchor[0] = PAIR
    anchor[1] = NCH * D
    anchor[2] = HD
    anchor[3] = NPAIR + 1
    x_raw[0] = jnp.zeros((PAIR, D), BF16)
    xres[0:PAD, :] = jnp.zeros((PAD, D), F32)

    cp_x(0).wait()

    def ln_mid(i, carry):
        for pp in range(LNP):
            pr = i * LNP + pp
            ln = _layernorm(x_raw[1 + pr, 24:40, :].astype(F32))
            hbuf[pl.ds(pl.multiple_of(PAD + pr * PAIR + 24, 8), 16), :] = ln
            lhs_pre[pl.ds(pl.multiple_of(pr * 8, 8), 8), :] = pltpu.bitcast(ln.astype(BF16), U32)
        return carry

    lax.fori_loop(0, NPAIR // LNP, ln_mid, 0)

    def ln_jobs(p0, npairs):
        def job(pp, r0):
            ln = _layernorm(x_raw[1 + p0 + pp, r0:r0 + 8, :].astype(F32))
            hbuf[pl.ds(pl.multiple_of(PAD + (p0 + pp) * PAIR + r0, 8), 8), :] = ln

        return [('x_raw', functools.partial(job, pp, r0))
                for pp in range(npairs) for r0 in (0, 8, 16, 40, 48, 56)]

    def relayout_jobs(c, blk0, nblk, slot0=0):
        def job(u):
            t0 = ((slot0 + u) % NTMP) * TSZ
            d0 = pl.multiple_of(c * D + (blk0 + u) * 16, 16)
            raw = pltpu.bitcast(stage[pl.ds(d0, 16), :, :], U32)
            for i in range(8):
                ev, od = raw[2 * i], raw[2 * i + 1]
                lo = (ev & jnp.uint32(0xFFFF)) | (od << 16)
                hi = (ev >> 16) | (od & jnp.uint32(0xFFFF0000))
                tmp[pl.ds(t0 + i * TP, 8, stride=2), :] = lo
                tmp[pl.ds(t0 + i * TP + 1, 8, stride=2), :] = hi
            o0 = pl.multiple_of((blk0 + u) * 8, 8)
            for hh in range(HC):
                col = (hh % G) * DH
                wch[c][hh // G, pl.ds(o0, 8), col:col + DH] = tmp[pl.ds(t0 + hh, 8, stride=TP), :]

        return [('stage', functools.partial(job, u)) for u in range(nblk)]

    def repack_jobs(part):
        def job(c):
            r0 = pl.multiple_of(part * WOP + c * 128, 128)
            o0 = pl.multiple_of(part * (WOP // 2) + c * 64, 64)
            wo[pl.ds(o0, 64), :] = pltpu.bitcast(wo_raw[pl.ds(r0, 128), :], U32)

        return [('wo_raw', functools.partial(job, c)) for c in range(WOP // 128)]

    def interleave(*lists):
        keyed = [((i + 0.5) / len(l), n, j) for n, l in enumerate(lists) for i, j in enumerate(l)]
        return [j for _, _, j in sorted(keyed, key=lambda t: t[:2])]

    def precompute(c, g0, ng, jobs, k0=0, k1=D):
        lhs = pltpu.bitcast(lhs_pre[:, k0:k1], BF16)
        ys = [_dot(lhs, pltpu.bitcast(wch[c][g0 + gg, k0 // 2:k1 // 2, :], BF16))
              for gg in range(ng)]
        nrow = 16 * NPAIR
        has_ln = any(kind == 'x_raw' for kind, _ in jobs)
        for u, (kind, job) in enumerate(jobs):
            if u > 0:
                par = D // (k1 - k0)
                span = ng * G * nrow // par - (SLACK[1] if has_ln else SLACK[0])
                pos = max((u * span // len(jobs)) // 16 * 16 - 128, 0)
                nt, r0 = pos // nrow * par, pos % nrow
                tie = ys[nt // G][r0:r0 + 16, (nt % G) * DH:(nt % G + 1) * DH].astype(BF16)
                if kind == 'stage':
                    stage[anchor[1]] = tie
                elif kind == 'x_raw':
                    x_raw[anchor[3], 0:16, 0:DH] = tie
                else:
                    wo_raw[pl.ds(pl.multiple_of(anchor[2], 16), 16), 0:DH] = tie
            job()
        for gg in range(ng):
            if k0 > 0:
                pre[c * GPC + g0 + gg] += ys[gg]
            else:
                pre[c * GPC + g0 + gg] = ys[gg]

    def run(jobs):
        for _, job in jobs:
            job()

    NBLK = D // 16
    HB, QB = NBLK // 2, NBLK // 4
    cp_w(0, 0).wait()
    run(relayout_jobs(0, 0, QB))
    precompute(0, 0, GPC, [], 0, D // 4)
    cp_w(0, 1).wait()
    run(relayout_jobs(0, QB, QB))
    cp_w(0, 2).wait()
    cp_w(0, 3).wait()
    precompute(0, 0, GPC, relayout_jobs(0, HB, HB), D // 4, D // 2)

    def phase01(c, k0, it, carry):
        cp_w(c + 1, it).wait()
        precompute(c, it * 2, 2, relayout_jobs(c + 1, it * HB, HB), k0, D)
        return carry

    lax.fori_loop(0, 2, functools.partial(phase01, 0, D // 2), 0)
    lax.fori_loop(0, 2, functools.partial(phase01, 1, 0), 0)
    cp_x(1).wait()
    cp_x(2).wait()
    cp_w(3, 0).wait()
    lax.fori_loop(0, 2, lambda it, cr: (
        precompute(2, it * 2, 2, interleave(relayout_jobs(3, it * HB, HB),
                                            ln_jobs(it * (NPAIR // 2), NPAIR // 2))), cr)[1], 0)

    def last_phase(it, carry):
        cp_w(4, it).wait()
        cp_w(5, it).wait()
        cp_o(it).wait()
        precompute(3, it, 1, interleave(relayout_jobs(4, it * QB, QB),
                                        relayout_jobs(5, it * QB, QB, NTMP // 2),
                                        repack_jobs(it)))
        return carry

    lax.fori_loop(0, 4, last_phase, 0)

    for c in cp_small:
        c.wait()
    wr = wr_v[...].astype(F32).reshape(1, D)

    qi = lax.broadcasted_iota(jnp.int32, (32, 48), 0)
    kj = lax.broadcasted_iota(jnp.int32, (32, 48), 1)
    mask_a = (kj < 40) & ((qi < M) | (kj <= qi))
    qi = lax.broadcasted_iota(jnp.int32, (48, 80), 0)
    kj = lax.broadcasted_iota(jnp.int32, (48, 80), 1)
    kb0 = (kj >= 40) & (kj < 48)
    m_mem = (qi < M) & ((kj < 32) | kb0)
    m_xb = (qi >= M) & (qi < 32) & ((kj <= qi) | kb0)
    m_xa = (qi >= 32) & (qi < 40) & ((kj >= 48) | ((kj >= 32) & (kj <= qi)))
    m_b0 = (qi >= 40) & ((kj < M) | (kb0 & (kj <= qi)))
    mask_b = m_mem | m_xb | m_xa | m_b0

    def w_ref(mi, g):
        return wch[(4, 0, 2)[mi] + g // GPC].at[g % GPC]

    def wo_rows(g, n=1):
        r0 = g * GW // 2
        return pltpu.bitcast(wo[r0:r0 + n * GW // 2, :], BF16)

    def seg_step(lhs, lhs_f32, extra, mask, lags, s_mid, filler):
        q, k, v, p, o = {}, {}, {}, {}, {}
        raw = ({}, {}, {})
        acc = [None]

        def proj(mi, g, dst):
            if mi == 0 and g == 0 and lhs_f32 is not None:
                y = None
                lp = jnp.concatenate([lhs_f32[16:], lhs_f32[0:16]], axis=0)
                for kt in range(D // 128):
                    w = pltpu.bitcast(w_ref(0, 0)[kt * 64:(kt + 1) * 64, :], BF16)
                    t = _dot(lp[:, kt * 128:(kt + 1) * 128].astype(BF16), w)
                    y = t if y is None else y + t
                nr = y.shape[0]
                y = jnp.concatenate([y[nr - 16:], y[0:nr - 16]], axis=0)
            else:
                y = _dot(lhs[mi], pltpu.bitcast(w_ref(mi, g)[...], BF16))
            for j in range(G):
                h = g * G + j
                yh = y[:, j * DH:(j + 1) * DH]
                ex = extra(mi, h)
                if ex:
                    yh = jnp.concatenate([yh] + ex, axis=0)
                raw[mi][h] = yh
                dst[h] = yh.astype(BF16)

        def sc(g):
            for h in range(g * G, (g + 1) * G):
                p[h] = _softmax_bf16(_dot_nt(q[h], k[h]), mask)

        def pv(g):
            o[g] = jnp.concatenate(
                [_dot(p[h], v[h]) for h in range(g * G, (g + 1) * G)], axis=1)

        def op(g):
            if merge and g == NG - 2:
                return
            if merge and g == NG - 1:
                y = _dot(jnp.concatenate([o[g - 1], o[g]], axis=1).astype(BF16),
                         wo_rows(g - 1, 2))
            else:
                y = _dot(o[g].astype(BF16), wo_rows(g))
            acc[0] = y if acc[0] is None else acc[0] + y

        ls, lp, lo, merge, pv0 = lags
        for t in range(2 * NG + lp + lo):
            if t < NG:
                proj(0, t, q)
                if s_mid and 0 <= t - ls < NG:
                    sc(t - ls)
                proj(1, t, k)
            elif t < 2 * NG:
                proj(2, t - NG, v)
            if 0 <= t - ls < NG and not s_mid:
                sc(t - ls)
            if t == NG + lp + pv0:
                pv(0)
                if s_mid:
                    for g in range(NG - ls, NG):
                        sc(g)
            if 0 < t - NG - lp < NG:
                pv(t - NG - lp)
            if pv0 > lo - 1 and t == NG + lp + lo + 1:
                op(0)
            if (1 if pv0 > lo - 1 else 0) <= t - NG - lp - lo < NG:
                op(t - NG - lp - lo)
            if t in filler:
                src = raw[1][t * G] if t < NG else raw[2][min(t - NG, NG - 1) * G]
                filler[t](src[0:8])
        return acc[0], raw

    subr = lax.broadcasted_iota(jnp.int32, (RC, 128), 0).astype(F32)

    def post_chunk(li, pi, valid, c, tie=None):
        if tie is not None:
            obuf[pl.ds(pl.multiple_of(anchor[0], 8), 8), 0:DH] = tie
        base = pi * PAIR if isinstance(pi, int) else pl.multiple_of(pi * PAIR, PAIR)
        rows = pl.ds(base + c * RC, RC)
        x0 = x_raw[pi, c * RC:(c + 1) * RC, :].astype(F32) if li == 0 else xres[rows, :]
        x1 = _rnd(x0 + _rnd(obuf[c * RC:(c + 1) * RC, :]))
        ln = _layernorm(x1)
        r = _rnd(jnp.sum(ln * wr, axis=-1, keepdims=True))
        r = jnp.broadcast_to(jnp.where(valid, r, -jnp.inf), (RC, 128))
        rb = rbest[...]
        better = r > rb
        rbest[...] = jnp.where(better, r, rb)
        row0 = jnp.asarray(base + (c * RC - PAD), jnp.int32).astype(F32)
        ibest[...] = jnp.where(better, subr + row0, ibest[...])
        x1buf[rows, :] = x1
        lbuf[rows, :] = ln
        if li == 0:
            x2 = _rnd(x1 + ln)
            xres[rows, :] = x2
            hbuf[rows, :] = _layernorm(x2)
        else:
            ostage[rows, :] = (x1 + ln).astype(BF16)

    def out_copy(row0, nrows):
        return pltpu.make_async_copy(ostage.at[pl.ds(PAD + row0, nrows)],
                                     out_hbm.at[pl.ds(row0, nrows)], osem)

    def pair_body(li, pi, mem, first):
        base = pl.multiple_of(pi * PAIR, PAIR)
        ha = hbuf[pl.ds(base + PAD, 40), :]
        hb = hbuf[pl.ds(base + PAD + 40, 24), :]
        fill = ({}, {})
        for c, (st, t) in enumerate(FILL[li]):
            fill[st][t] = functools.partial(post_chunk, li, pi, pi > 0, c)
        aq = jnp.concatenate([mem, ha[0:24]], axis=0)
        lhs_aq = aq.astype(BF16)
        if li == 0:
            p0 = pl.multiple_of(pi * 16, 16)
            lhs_akv = lhs_aq
            extra_a = lambda mi, h: [pre[(mi - 1) * NG + h // G, pl.ds(p0, 16),
                                         (h % G) * DH:(h % G + 1) * DH]] if mi else []
        else:
            lhs_akv = jnp.concatenate([mem, ha], axis=0).astype(BF16)
            extra_a = lambda mi, h: []
        acc_a, prj = seg_step((lhs_aq, lhs_akv, lhs_akv), None if first else aq, extra_a, mask_a,
                              LAGA, SMID[0], fill[0])
        lhs_b = jnp.concatenate([acc_a[0:8], hb], axis=0).astype(BF16)
        bq = jnp.concatenate([acc_a[0:8], hb, ha[24:40]], axis=0)
        acc_b, _ = seg_step(
            (bq.astype(BF16), lhs_b, lhs_b), bq,
            lambda mi, h: [prj[mi][h][32:48], prj[mi][h][0:32]] if mi else [],
            mask_b, LAGB, SMID[1], fill[1])
        obuf[0:24, :] = acc_a[8:32]
        obuf[24:40, :] = acc_b[32:48]
        obuf[40:64, :] = acc_b[8:32]
        return acc_b[0:8]

    def loop_body(li, it, mem):
        UNROLL = UNROLLS[li]
        for u in range(UNROLL):
            mem = pair_body(li, it * UNROLL + u, mem, u == 0)

        if li == 1:
            @pl.when(it > 0)
            def _():
                out_copy(pl.multiple_of(it * (UNROLL * PAIR) - PAIR, PAIR),
                         UNROLL * PAIR).start()

            if UNROLL > 1:
                @pl.when(it == 0)
                def _():
                    out_copy(0, (UNROLL - 1) * PAIR).start()

        return mem

    for li in range(2):
        obuf[0:PAIR, :] = jnp.zeros((PAIR, D), F32)
        rbest[...] = jnp.full((RC, 128), -jnp.inf, F32)
        ibest[...] = jnp.zeros((RC, 128), F32)
        lax.fori_loop(0, NPAIR // UNROLLS[li], functools.partial(loop_body, li),
                      mem0_v[...].astype(F32))

        if li == 0:
            for c in cp_mlp:
                c.wait()
        else:
            out_copy(0, S - PAIR).wait()

        def top1():
            rb = rbest[...]
            rmax = jnp.max(rb, axis=0, keepdims=True)
            imin = jnp.min(jnp.where(rb == rmax, ibest[...], S - 1.0), axis=0, keepdims=True)
            return rmax, imin.astype(jnp.int32)[0, 0]

        def mod_trip(carry, li=li):
            rmax, idx = top1()
            lsel = lbuf[pl.ds(PAD + idx, 1), :]
            for c in range(PAIR // RC):
                post_chunk(li, NPAIR, True, c)
            xs = jnp.broadcast_to(lsel, (16, D)).astype(BF16)
            acts = []
            for f0, f1 in FSPLIT:
                gpre = _rnd(_dot(xs, wg_v[:, f0:f1]))
                gate = _rnd(gpre * _rnd(jax.nn.sigmoid(gpre)))
                up = _rnd(_dot(xs, wu_v[:, f0:f1]))
                acts.append((gate * up).astype(BF16))
            y = None
            for (f0, f1), act in zip(FSPLIT, acts):
                t = _dot(act, wd_v[f0:f1, :])
                y = t if y is None else y + t
            y = _rnd(y)[0:8]
            rsel = _rnd(jax.nn.sigmoid(rmax[:, 0:1]))
            ybuf[...] = _rnd(y * rsel)
            return idx, top1()[1]

        idx, _ = lax.while_loop(lambda cr: cr[0] != cr[1], mod_trip,
                                (jnp.int32(-1), jnp.int32(0)))
        row = pl.ds(PAD + idx, 1)
        lsel = lbuf[row, :]
        y = ybuf[0:1, :]
        if li == 0:
            x2 = _rnd(x1buf[row, :] + _rnd(lsel + y))
            xres[row, :] = x2
            hbuf[row, :] = _layernorm(x2)
        else:
            t0 = pl.multiple_of((idx // 16) * 16, 16)
            tile = pl.ds(PAD + t0, 16)
            sel = lax.broadcasted_iota(jnp.int32, (16, D), 0) == idx - t0
            upd = jnp.where(sel, jnp.broadcast_to(y, (16, D)), 0.0)
            ostage[tile, :] = (x1buf[tile, :] + _rnd(lbuf[tile, :] + upd)).astype(BF16)
            t1 = pl.multiple_of(jnp.minimum(t0, S - PAIR - 16), 16)
            out_copy(S - PAIR, PAIR).start()
            out_copy(t1, 16).start()
            out_copy(0, PAIR + 16).wait()


_FILL = ((0, 9), (0, 12), (0, 15), (1, 8), (1, 10), (1, 12), (1, 14), (1, 15))
CFG = dict(UNROLLS=(2, 2), LAGA=(1, 1, 2, True, 0), LAGB=(1, 1, 2, False, 1), FILL=(_FILL, _FILL),
           SMID=(False, True), LNP=16, SLACK=(128, 256))


def _build():
    any_spec = pl.BlockSpec(memory_space=pl.ANY)
    return pl.pallas_call(
        functools.partial(_kernel, **CFG),
        out_shape=jax.ShapeDtypeStruct((S, D), BF16),
        in_specs=[any_spec] * 10,
        out_specs=any_spec,
        scratch_shapes=[
            pltpu.VMEM((NPAIR + 2, PAIR, D), BF16),
            pltpu.VMEM((M, D), BF16),
            pltpu.VMEM((D,), BF16),
            pltpu.VMEM((NCH * D + 1, HC, DH), BF16),
            pltpu.VMEM((HD + 16, D), BF16),
            pltpu.VMEM((D, FF), BF16),
            pltpu.VMEM((D, FF), BF16),
            pltpu.VMEM((FF, D), BF16),
        ] + [pltpu.VMEM((GPC, D // 2, GW), U32)] * NCH + [
            pltpu.VMEM((HD // 2, D), U32),
            pltpu.VMEM((NTMP * TSZ, DH), U32),
            pltpu.VMEM((PAD + S, D), F32),
            pltpu.VMEM((PAD + S, D), F32),
            pltpu.VMEM((PAD + S, D), F32),
            pltpu.VMEM((PAD + S, D), F32),
            pltpu.VMEM((RC, 128), F32),
            pltpu.VMEM((RC, 128), F32),
            pltpu.VMEM((PAIR + 8, D), F32),
            pltpu.VMEM((PAD + S, D), BF16),
            pltpu.VMEM((8 * NPAIR, D), U32),
            pltpu.VMEM((2 * NG, 16 * NPAIR, GW), F32),
            pltpu.VMEM((8, D), F32),
            pltpu.SMEM((4,), jnp.int32),
            pltpu.SemaphoreType.DMA((29,)),
            pltpu.SemaphoreType.DMA(()),
        ],
        compiler_params=pltpu.CompilerParams(vmem_limit_bytes=120 * 1024 * 1024),
    )


@jax.jit
def pallas_interleave_layers__memory_aug_recurrent_mem_tr__moe_arch_mod__prompt_kernel(
    A_x: jax.Array,
    A_mem0: jax.Array,
    A_Wq: jax.Array,
    A_Wk: jax.Array,
    A_Wv: jax.Array,
    A_Wo: jax.Array,
    A_seg_len,
    B_x: jax.Array,
    B_w_r: jax.Array,
    B_w_gate: jax.Array,
    B_w_up: jax.Array,
    B_w_down: jax.Array,
):
    assert A_x.shape == (1, S, D) and A_mem0.shape == (1, M, D) and A_Wq.shape == (D, H, DH)
    del A_seg_len
    del B_x
    out = _build()(
        A_x.reshape(NPAIR, PAIR, D),
        A_mem0.reshape(M, D),
        A_Wq,
        A_Wk,
        A_Wv,
        A_Wo.reshape(HD, D),
        B_w_r,
        B_w_gate,
        B_w_up,
        B_w_down,
    )
    return out.reshape(1, S, D)
```

```python
import functools
import math

import jax
import jax.numpy as jnp
from jax import lax
import jax.experimental.pallas as pl
import jax.experimental.pallas.tpu as pltpu

F32 = jnp.float32
BF16 = jnp.bfloat16
U32 = jnp.uint32

S, D, H, DH, M, SEG = 2048, 512, 32, 128, 8, 32
FF = 1792
HD = H * DH
PAIR = 2 * SEG
NPAIR = S // PAIR
PAD = PAIR
G = 4
NG = H // G
GW = G * DH
HC = 16
GPC = HC // G
NCH = 3 * H // HC
TP = 20
TSZ = 8 * TP
NTMP = 8
FSPLIT = ((0, 1024), (1024, FF))
RC = 8
LN_EPS = 1e-05
NEG = -1000000000.0 * DH ** 0.5
EXP2_SCALE = (DH ** -0.5) * math.log2(math.e)


def _rnd(x):
    return x.astype(BF16).astype(F32)


def _layernorm(x):
    mean = jnp.sum(x, axis=-1, keepdims=True) * (1.0 / D)
    c = x - mean
    var = jnp.sum(c * c, axis=-1, keepdims=True) * (1.0 / D)
    z = _rnd(_rnd(var) + _rnd(jnp.float32(LN_EPS)))
    finite = z < jnp.inf
    den = _rnd(z * lax.rsqrt(z))
    inv = pl.reciprocal(den, approx=True)
    inv = jnp.where(finite, inv * (2.0 - den * inv), 0.0)
    return _rnd(_rnd(x - _rnd(mean)) * inv)


def _dot(a, b):
    return jnp.dot(a, b, preferred_element_type=F32)


def _dot_nt(a, b):
    return lax.dot_general(a, b, (((1,), (1,)), ((), ())), preferred_element_type=F32)


def _softmax_bf16(s, mask):
    s = jnp.where(mask, s, NEG)
    m = jnp.max(s, axis=-1, keepdims=True)
    e = jnp.exp2((s - m) * EXP2_SCALE)
    l = jnp.sum(e, axis=-1, keepdims=True)
    r = pl.reciprocal(l, approx=True)
    r = r * (2.0 - l * r)
    return (e * r).astype(BF16)


def _kernel(x_hbm, mem0_hbm, wq_hbm, wk_hbm, wv_hbm, wo_hbm, wr_hbm, wg_hbm, wu_hbm, wd_hbm,
            out_hbm,
            x_raw, mem0_v, wr_v, stage, wo_raw, wg_v, wu_v, wd_v,
            wk0, wk1, wv0, wv1, wq0, wq1, wo, tmp,
            xres, x1buf, lbuf, hbuf, rbest, ibest, obuf, ostage,
            lhs_pre, pre, ybuf, anchor, sems, osem, *,
            UNROLLS, LAGA, LAGB, FILL, SMID, LNP, SLACK):
    wch = (wk0, wk1, wv0, wv1, wq0, wq1)
    NWO = 4
    WOP = HD // NWO
    WPARTS = (4, 2, 2, 1, 4, 4)
    SEM_X = 0
    SEM_W = [3 + sum(WPARTS[:c]) for c in range(NCH)]
    SEM_O = 3 + sum(WPARTS)
    SEM_MISC = SEM_O + NWO

    def cp_x(i):
        r0, nr = ((24, 16), (0, 24), (40, 24))[i]
        return pltpu.make_async_copy(x_hbm.at[:, pl.ds(r0, nr), :],
                                     x_raw.at[pl.ds(1, NPAIR), pl.ds(r0, nr), :],
                                     sems.at[SEM_X + i])

    def cp_w(c, part):
        w = (wk_hbm, wv_hbm, wq_hbm)[c // 2]
        nd = D // WPARTS[c]
        return pltpu.make_async_copy(
            w.at[pl.ds(part * nd, nd), pl.ds((c % 2) * HC, HC), :],
            stage.at[pl.ds(c * D + part * nd, nd)], sems.at[SEM_W[c] + part])

    def cp_o(i):
        return pltpu.make_async_copy(wo_hbm.at[pl.ds(i * WOP, WOP)],
                                     wo_raw.at[pl.ds(i * WOP, WOP)], sems.at[SEM_O + i])

    cp_small = [pltpu.make_async_copy(s_, d_, sems.at[SEM_MISC + i])
                for i, (s_, d_) in enumerate(((mem0_hbm, mem0_v), (wr_hbm, wr_v)))]
    cp_mlp = [pltpu.make_async_copy(s_, d_, sems.at[SEM_MISC + 2 + i])
              for i, (s_, d_) in enumerate(((wg_hbm, wg_v), (wu_hbm, wu_v), (wd_hbm, wd_v)))]
    cp_x(0).start()
    for c in range(3):
        for part in range(WPARTS[c]):
            cp_w(c, part).start()
    cp_x(1).start()
    cp_x(2).start()
    cp_w(3, 0).start()
    for i in range(NWO):
        cp_w(4, i).start()
        cp_w(5, i).start()
        cp_o(i).start()
    for c in cp_small + cp_mlp:
        c.start()

    anchor[0] = PAIR
    anchor[1] = NCH * D
    anchor[2] = HD
    anchor[3] = NPAIR + 1
    x_raw[0] = jnp.zeros((PAIR, D), BF16)
    xres[0:PAD, :] = jnp.zeros((PAD, D), F32)

    cp_x(0).wait()

    def ln_mid(i, carry):
        for pp in range(LNP):
            pr = i * LNP + pp
            ln = _layernorm(x_raw[1 + pr, 24:40, :].astype(F32))
            hbuf[pl.ds(pl.multiple_of(PAD + pr * PAIR + 24, 8), 16), :] = ln
            lhs_pre[pl.ds(pl.multiple_of(pr * 8, 8), 8), :] = pltpu.bitcast(ln.astype(BF16), U32)
        return carry

    lax.fori_loop(0, NPAIR // LNP, ln_mid, 0)

    def ln_jobs(p0, npairs):
        def job(pp, ra, rb):
            xv = jnp.concatenate([x_raw[1 + p0 + pp, r:r + 8, :].astype(F32) for r in (ra, rb)],
                                 axis=0)
            ln = _layernorm(xv)
            for n, r in enumerate((ra, rb)):
                hbuf[pl.ds(pl.multiple_of(PAD + (p0 + pp) * PAIR + r, 8), 8), :] = (
                    ln[n * 8:(n + 1) * 8])

        return [('x_raw', functools.partial(job, pp, ra, rb))
                for pp in range(npairs) for ra, rb in ((0, 8), (16, 40), (48, 56))]

    def relayout_jobs(c, blk0, nblk, slot0=0):
        def job(u):
            t0 = ((slot0 + u) % NTMP) * TSZ
            d0 = pl.multiple_of(c * D + (blk0 + u) * 16, 16)
            raw = pltpu.bitcast(stage[pl.ds(d0, 16), :, :], U32)
            for i in range(8):
                ev, od = raw[2 * i], raw[2 * i + 1]
                lo = (ev & jnp.uint32(0xFFFF)) | (od << 16)
                hi = (ev >> 16) | (od & jnp.uint32(0xFFFF0000))
                tmp[pl.ds(t0 + i * TP, 8, stride=2), :] = lo
                tmp[pl.ds(t0 + i * TP + 1, 8, stride=2), :] = hi
            o0 = pl.multiple_of((blk0 + u) * 8, 8)
            for hh in range(HC):
                col = (hh % G) * DH
                wch[c][hh // G, pl.ds(o0, 8), col:col + DH] = tmp[pl.ds(t0 + hh, 8, stride=TP), :]

        return [('stage', functools.partial(job, u)) for u in range(nblk)]

    def repack_jobs(part):
        def job(c):
            r0 = pl.multiple_of(part * WOP + c * 128, 128)
            o0 = pl.multiple_of(part * (WOP // 2) + c * 64, 64)
            wo[pl.ds(o0, 64), :] = pltpu.bitcast(wo_raw[pl.ds(r0, 128), :], U32)

        return [('wo_raw', functools.partial(job, c)) for c in range(WOP // 128)]

    def interleave(*lists):
        keyed = [((i + 0.5) / len(l), n, j) for n, l in enumerate(lists) for i, j in enumerate(l)]
        return [j for _, _, j in sorted(keyed, key=lambda t: t[:2])]

    def precompute(c, g0, ng, jobs, k0=0, k1=D):
        lhs = pltpu.bitcast(lhs_pre[:, k0:k1], BF16)
        ys = [_dot(lhs, pltpu.bitcast(wch[c][g0 + gg, k0 // 2:k1 // 2, :], BF16))
              for gg in range(ng)]
        nrow = 16 * NPAIR
        has_ln = any(kind == 'x_raw' for kind, _ in jobs)
        for u, (kind, job) in enumerate(jobs):
            if u > 0:
                par = D // (k1 - k0)
                span = ng * G * nrow // par - (SLACK[1] if has_ln else SLACK[0])
                pos = max((u * span // len(jobs)) // 16 * 16 - 128, 0)
                nt, r0 = pos // nrow * par, pos % nrow
                tie = ys[nt // G][r0:r0 + 16, (nt % G) * DH:(nt % G + 1) * DH].astype(BF16)
                if kind == 'stage':
                    stage[anchor[1]] = tie
                elif kind == 'x_raw':
                    x_raw[anchor[3], 0:16, 0:DH] = tie
                else:
                    wo_raw[pl.ds(pl.multiple_of(anchor[2], 16), 16), 0:DH] = tie
            job()
        for gg in range(ng):
            if k0 > 0:
                pre[c * GPC + g0 + gg] += ys[gg]
            else:
                pre[c * GPC + g0 + gg] = ys[gg]

    def run(jobs):
        for _, job in jobs:
            job()

    NBLK = D // 16
    HB, QB = NBLK // 2, NBLK // 4
    cp_w(0, 0).wait()
    run(relayout_jobs(0, 0, QB))
    precompute(0, 0, GPC, [], 0, D // 4)
    cp_w(0, 1).wait()
    run(relayout_jobs(0, QB, QB))
    cp_w(0, 2).wait()
    cp_w(0, 3).wait()
    precompute(0, 0, GPC, relayout_jobs(0, HB, HB), D // 4, D // 2)

    def phase01(c, k0, it, carry):
        cp_w(c + 1, it).wait()
        precompute(c, it * 2, 2, relayout_jobs(c + 1, it * HB, HB), k0, D)
        return carry

    lax.fori_loop(0, 2, functools.partial(phase01, 0, D // 2), 0)
    lax.fori_loop(0, 2, functools.partial(phase01, 1, 0), 0)
    cp_x(1).wait()
    cp_x(2).wait()
    cp_w(3, 0).wait()
    lax.fori_loop(0, 2, lambda it, cr: (
        precompute(2, it * 2, 2, interleave(relayout_jobs(3, it * HB, HB),
                                            ln_jobs(it * (NPAIR // 2), NPAIR // 2))), cr)[1], 0)

    def last_phase(it, carry):
        cp_w(4, it).wait()
        cp_w(5, it).wait()
        cp_o(it).wait()
        precompute(3, it, 1, interleave(relayout_jobs(4, it * QB, QB),
                                        relayout_jobs(5, it * QB, QB, NTMP // 2),
                                        repack_jobs(it)))
        return carry

    lax.fori_loop(0, 4, last_phase, 0)

    for c in cp_small:
        c.wait()
    wr = wr_v[...].astype(F32).reshape(1, D)

    qi = lax.broadcasted_iota(jnp.int32, (32, 48), 0)
    kj = lax.broadcasted_iota(jnp.int32, (32, 48), 1)
    mask_a = (kj < 40) & ((qi < M) | (kj <= qi))
    qi = lax.broadcasted_iota(jnp.int32, (48, 80), 0)
    kj = lax.broadcasted_iota(jnp.int32, (48, 80), 1)
    kb0 = (kj >= 40) & (kj < 48)
    m_mem = (qi < M) & ((kj < 32) | kb0)
    m_xb = (qi >= M) & (qi < 32) & ((kj <= qi) | kb0)
    m_xa = (qi >= 32) & (qi < 40) & ((kj >= 48) | ((kj >= 32) & (kj <= qi)))
    m_b0 = (qi >= 40) & ((kj < M) | (kb0 & (kj <= qi)))
    mask_b = m_mem | m_xb | m_xa | m_b0

    def w_ref(mi, g):
        return wch[(4, 0, 2)[mi] + g // GPC].at[g % GPC]

    def wo_rows(g, n=1):
        r0 = g * GW // 2
        return pltpu.bitcast(wo[r0:r0 + n * GW // 2, :], BF16)

    def seg_step(lhs, lhs_f32, extra, mask, lags, s_mid, filler):
        q, k, v, p, o = {}, {}, {}, {}, {}
        raw = ({}, {}, {})
        acc = [None]

        def proj(mi, g, dst):
            if mi == 0 and g == 0 and lhs_f32 is not None:
                y = None
                lp = jnp.concatenate([lhs_f32[16:], lhs_f32[0:16]], axis=0)
                for kt in range(D // 128):
                    w = pltpu.bitcast(w_ref(0, 0)[kt * 64:(kt + 1) * 64, :], BF16)
                    t = _dot(lp[:, kt * 128:(kt + 1) * 128].astype(BF16), w)
                    y = t if y is None else y + t
                nr = y.shape[0]
                y = jnp.concatenate([y[nr - 16:], y[0:nr - 16]], axis=0)
            else:
                y = _dot(lhs[mi], pltpu.bitcast(w_ref(mi, g)[...], BF16))
            for j in range(G):
                h = g * G + j
                yh = y[:, j * DH:(j + 1) * DH]
                ex = extra(mi, h)
                if ex:
                    yh = jnp.concatenate([yh] + ex, axis=0)
                raw[mi][h] = yh
                dst[h] = yh.astype(BF16)

        def sc(g):
            for h in range(g * G, (g + 1) * G):
                p[h] = _softmax_bf16(_dot_nt(q[h], k[h]), mask)

        def pv(g):
            o[g] = jnp.concatenate(
                [_dot(p[h], v[h]) for h in range(g * G, (g + 1) * G)], axis=1)

        def op(g):
            if merge and g == NG - 2:
                return
            if merge and g == NG - 1:
                y = _dot(jnp.concatenate([o[g - 1], o[g]], axis=1).astype(BF16),
                         wo_rows(g - 1, 2))
            else:
                y = _dot(o[g].astype(BF16), wo_rows(g))
            acc[0] = y if acc[0] is None else acc[0] + y

        ls, lp, lo, merge, pv0 = lags
        for t in range(2 * NG + lp + lo):
            if t < NG:
                proj(0, t, q)
                if s_mid and 0 <= t - ls < NG:
                    sc(t - ls)
                proj(1, t, k)
            elif t < 2 * NG:
                proj(2, t - NG, v)
            if 0 <= t - ls < NG and not s_mid:
                sc(t - ls)
            if t == NG + lp + pv0:
                pv(0)
                if s_mid:
                    for g in range(NG - ls, NG):
                        sc(g)
            if 0 < t - NG - lp < NG:
                pv(t - NG - lp)
            if pv0 > lo - 1 and t == NG + lp + lo + 1:
                op(0)
            if (1 if pv0 > lo - 1 else 0) <= t - NG - lp - lo < NG:
                op(t - NG - lp - lo)
            if t in filler:
                src = raw[1][t * G] if t < NG else raw[2][min(t - NG, NG - 1) * G]
                filler[t](src[0:8])
        return acc[0], raw

    subr = lax.broadcasted_iota(jnp.int32, (RC, 128), 0).astype(F32)

    def post_chunk(li, pi, valid, c, tie=None):
        if tie is not None:
            obuf[pl.ds(pl.multiple_of(anchor[0], 8), 8), 0:DH] = tie
        base = pi * PAIR if isinstance(pi, int) else pl.multiple_of(pi * PAIR, PAIR)
        rows = pl.ds(base + c * RC, RC)
        x0 = x_raw[pi, c * RC:(c + 1) * RC, :].astype(F32) if li == 0 else xres[rows, :]
        x1 = _rnd(x0 + _rnd(obuf[c * RC:(c + 1) * RC, :]))
        ln = _layernorm(x1)
        r = _rnd(jnp.sum(ln * wr, axis=-1, keepdims=True))
        r = jnp.broadcast_to(jnp.where(valid, r, -jnp.inf), (RC, 128))
        rb = rbest[...]
        better = r > rb
        rbest[...] = jnp.where(better, r, rb)
        row0 = jnp.asarray(base + (c * RC - PAD), jnp.int32).astype(F32)
        ibest[...] = jnp.where(better, subr + row0, ibest[...])
        x1buf[rows, :] = x1
        lbuf[rows, :] = ln
        if li == 0:
            x2 = _rnd(x1 + ln)
            xres[rows, :] = x2
            hbuf[rows, :] = _layernorm(x2)
        else:
            ostage[rows, :] = (x1 + ln).astype(BF16)

    def out_copy(row0, nrows):
        return pltpu.make_async_copy(ostage.at[pl.ds(PAD + row0, nrows)],
                                     out_hbm.at[pl.ds(row0, nrows)], osem)

    def pair_body(li, pi, mem, first):
        base = pl.multiple_of(pi * PAIR, PAIR)
        ha = hbuf[pl.ds(base + PAD, 40), :]
        hb = hbuf[pl.ds(base + PAD + 40, 24), :]
        fill = ({}, {})
        for c, (st, t) in enumerate(FILL[li]):
            fill[st][t] = functools.partial(post_chunk, li, pi, pi > 0, c)
        aq = jnp.concatenate([mem, ha[0:24]], axis=0)
        lhs_aq = aq.astype(BF16)
        if li == 0:
            p0 = pl.multiple_of(pi * 16, 16)
            lhs_akv = lhs_aq
            extra_a = lambda mi, h: [pre[(mi - 1) * NG + h // G, pl.ds(p0, 16),
                                         (h % G) * DH:(h % G + 1) * DH]] if mi else []
        else:
            lhs_akv = jnp.concatenate([mem, ha], axis=0).astype(BF16)
            extra_a = lambda mi, h: []
        acc_a, prj = seg_step((lhs_aq, lhs_akv, lhs_akv), None if first else aq, extra_a, mask_a,
                              LAGA, SMID[0], fill[0])
        lhs_b = jnp.concatenate([acc_a[0:8], hb], axis=0).astype(BF16)
        bq = jnp.concatenate([acc_a[0:8], hb, ha[24:40]], axis=0)
        acc_b, _ = seg_step(
            (bq.astype(BF16), lhs_b, lhs_b), bq,
            lambda mi, h: [prj[mi][h][32:48], prj[mi][h][0:32]] if mi else [],
            mask_b, LAGB, SMID[1], fill[1])
        obuf[0:24, :] = acc_a[8:32]
        obuf[24:40, :] = acc_b[32:48]
        obuf[40:64, :] = acc_b[8:32]
        return acc_b[0:8]

    def loop_body(li, it, mem):
        UNROLL = UNROLLS[li]
        for u in range(UNROLL):
            mem = pair_body(li, it * UNROLL + u, mem, u == 0)

        if li == 1:
            @pl.when(it > 0)
            def _():
                out_copy(pl.multiple_of(it * (UNROLL * PAIR) - PAIR, PAIR),
                         UNROLL * PAIR).start()

            if UNROLL > 1:
                @pl.when(it == 0)
                def _():
                    out_copy(0, (UNROLL - 1) * PAIR).start()

        return mem

    for li in range(2):
        obuf[0:PAIR, :] = jnp.zeros((PAIR, D), F32)
        rbest[...] = jnp.full((RC, 128), -jnp.inf, F32)
        ibest[...] = jnp.zeros((RC, 128), F32)
        lax.fori_loop(0, NPAIR // UNROLLS[li], functools.partial(loop_body, li),
                      mem0_v[...].astype(F32))

        if li == 0:
            for c in cp_mlp:
                c.wait()
        else:
            out_copy(0, S - PAIR).wait()

        def top1():
            rb = rbest[...]
            rmax = jnp.max(rb, axis=0, keepdims=True)
            imin = jnp.min(jnp.where(rb == rmax, ibest[...], S - 1.0), axis=0, keepdims=True)
            return rmax, imin.astype(jnp.int32)[0, 0]

        def mod_trip(carry, li=li):
            rmax, idx = top1()
            lsel = lbuf[pl.ds(PAD + idx, 1), :]
            for c in range(PAIR // RC):
                post_chunk(li, NPAIR, True, c)
            xs = jnp.broadcast_to(lsel, (16, D)).astype(BF16)
            acts = []
            for f0, f1 in FSPLIT:
                gpre = _rnd(_dot(xs, wg_v[:, f0:f1]))
                gate = _rnd(gpre * _rnd(jax.nn.sigmoid(gpre)))
                up = _rnd(_dot(xs, wu_v[:, f0:f1]))
                acts.append((gate * up).astype(BF16))
            y = None
            for (f0, f1), act in zip(FSPLIT, acts):
                t = _dot(act, wd_v[f0:f1, :])
                y = t if y is None else y + t
            y = _rnd(y)[0:8]
            rsel = _rnd(jax.nn.sigmoid(rmax[:, 0:1]))
            ybuf[...] = _rnd(y * rsel)
            return idx, top1()[1]

        idx, _ = lax.while_loop(lambda cr: cr[0] != cr[1], mod_trip,
                                (jnp.int32(-1), jnp.int32(0)))
        row = pl.ds(PAD + idx, 1)
        lsel = lbuf[row, :]
        y = ybuf[0:1, :]
        if li == 0:
            x2 = _rnd(x1buf[row, :] + _rnd(lsel + y))
            xres[row, :] = x2
            hbuf[row, :] = _layernorm(x2)
        else:
            t0 = pl.multiple_of((idx // 16) * 16, 16)
            tile = pl.ds(PAD + t0, 16)
            sel = lax.broadcasted_iota(jnp.int32, (16, D), 0) == idx - t0
            upd = jnp.where(sel, jnp.broadcast_to(y, (16, D)), 0.0)
            ostage[tile, :] = (x1buf[tile, :] + _rnd(lbuf[tile, :] + upd)).astype(BF16)
            t1 = pl.multiple_of(jnp.minimum(t0, S - PAIR - 16), 16)
            out_copy(S - PAIR, PAIR).start()
            out_copy(t1, 16).start()
            out_copy(0, PAIR + 16).wait()


_FILL = ((0, 9), (0, 12), (0, 15), (1, 8), (1, 10), (1, 12), (1, 14), (1, 15))
CFG = dict(UNROLLS=(2, 2), LAGA=(1, 1, 2, True, 0), LAGB=(1, 1, 2, False, 1), FILL=(_FILL, _FILL),
           SMID=(False, True), LNP=16, SLACK=(128, 256))


def _build():
    any_spec = pl.BlockSpec(memory_space=pl.ANY)
    return pl.pallas_call(
        functools.partial(_kernel, **CFG),
        out_shape=jax.ShapeDtypeStruct((S, D), BF16),
        in_specs=[any_spec] * 10,
        out_specs=any_spec,
        scratch_shapes=[
            pltpu.VMEM((NPAIR + 2, PAIR, D), BF16),
            pltpu.VMEM((M, D), BF16),
            pltpu.VMEM((D,), BF16),
            pltpu.VMEM((NCH * D + 1, HC, DH), BF16),
            pltpu.VMEM((HD + 16, D), BF16),
            pltpu.VMEM((D, FF), BF16),
            pltpu.VMEM((D, FF), BF16),
            pltpu.VMEM((FF, D), BF16),
        ] + [pltpu.VMEM((GPC, D // 2, GW), U32)] * NCH + [
            pltpu.VMEM((HD // 2, D), U32),
            pltpu.VMEM((NTMP * TSZ, DH), U32),
            pltpu.VMEM((PAD + S, D), F32),
            pltpu.VMEM((PAD + S, D), F32),
            pltpu.VMEM((PAD + S, D), F32),
            pltpu.VMEM((PAD + S, D), F32),
            pltpu.VMEM((RC, 128), F32),
            pltpu.VMEM((RC, 128), F32),
            pltpu.VMEM((PAIR + 8, D), F32),
            pltpu.VMEM((PAD + S, D), BF16),
            pltpu.VMEM((8 * NPAIR, D), U32),
            pltpu.VMEM((2 * NG, 16 * NPAIR, GW), F32),
            pltpu.VMEM((8, D), F32),
            pltpu.SMEM((4,), jnp.int32),
            pltpu.SemaphoreType.DMA((29,)),
            pltpu.SemaphoreType.DMA(()),
        ],
        compiler_params=pltpu.CompilerParams(vmem_limit_bytes=120 * 1024 * 1024),
    )


@jax.jit
def pallas_interleave_layers__memory_aug_recurrent_mem_tr__moe_arch_mod__prompt_kernel(
    A_x: jax.Array,
    A_mem0: jax.Array,
    A_Wq: jax.Array,
    A_Wk: jax.Array,
    A_Wv: jax.Array,
    A_Wo: jax.Array,
    A_seg_len,
    B_x: jax.Array,
    B_w_r: jax.Array,
    B_w_gate: jax.Array,
    B_w_up: jax.Array,
    B_w_down: jax.Array,
):
    assert A_x.shape == (1, S, D) and A_mem0.shape == (1, M, D) and A_Wq.shape == (D, H, DH)
    del A_seg_len
    del B_x
    out = _build()(
        A_x.reshape(NPAIR, PAIR, D),
        A_mem0.reshape(M, D),
        A_Wq,
        A_Wk,
        A_Wv,
        A_Wo.reshape(HD, D),
        B_w_r,
        B_w_gate,
        B_w_up,
        B_w_down,
    )
    return out.reshape(1, S, D)
```

```python
import functools
import math

import jax
import jax.numpy as jnp
from jax import lax
import jax.experimental.pallas as pl
import jax.experimental.pallas.tpu as pltpu

F32 = jnp.float32
BF16 = jnp.bfloat16
U32 = jnp.uint32

S, D, H, DH, M, SEG = 2048, 512, 32, 128, 8, 32
FF = 1792
HD = H * DH
PAIR = 2 * SEG
NPAIR = S // PAIR
PAD = PAIR
G = 4
NG = H // G
GW = G * DH
HC = 16
GPC = HC // G
NCH = 3 * H // HC
TP = 20
TSZ = 8 * TP
NTMP = 8
FSPLIT = ((0, 1024), (1024, FF))
RC = 8
LN_EPS = 1e-05
NEG = -1000000000.0 * DH ** 0.5
EXP2_SCALE = (DH ** -0.5) * math.log2(math.e)


def _rnd(x):
    return x.astype(BF16).astype(F32)


def _layernorm(x):
    mean = jnp.sum(x, axis=-1, keepdims=True) * (1.0 / D)
    c = x - mean
    var = jnp.sum(c * c, axis=-1, keepdims=True) * (1.0 / D)
    z = _rnd(_rnd(var) + _rnd(jnp.float32(LN_EPS)))
    finite = z < jnp.inf
    den = _rnd(z * lax.rsqrt(z))
    inv = pl.reciprocal(den, approx=True)
    inv = jnp.where(finite, inv * (2.0 - den * inv), 0.0)
    return _rnd(_rnd(x - _rnd(mean)) * inv)


def _dot(a, b):
    return jnp.dot(a, b, preferred_element_type=F32)


def _dot_nt(a, b):
    return lax.dot_general(a, b, (((1,), (1,)), ((), ())), preferred_element_type=F32)


def _softmax_bf16(s, mask):
    s = jnp.where(mask, s, NEG)
    m = jnp.max(s, axis=-1, keepdims=True)
    e = jnp.exp2((s - m) * EXP2_SCALE)
    l = jnp.sum(e, axis=-1, keepdims=True)
    r = pl.reciprocal(l, approx=True)
    r = r * (2.0 - l * r)
    return (e * r).astype(BF16)


def _kernel(x_hbm, mem0_hbm, wq_hbm, wk_hbm, wv_hbm, wo_hbm, wr_hbm, wg_hbm, wu_hbm, wd_hbm,
            out_hbm,
            x_raw, mem0_v, wr_v, stage, wo_raw, wg_v, wu_v, wd_v,
            wk0, wk1, wv0, wv1, wq0, wq1, wo, tmp,
            xres, x1buf, lbuf, hbuf, rbest, ibest, obuf, ostage,
            lhs_pre, pre, ybuf, anchor, sems, osem, *,
            UNROLLS, LAGA, LAGB, FILL, SMID, LNP, SLACK):
    wch = (wk0, wk1, wv0, wv1, wq0, wq1)
    NWO = 4
    WOP = HD // NWO
    WPARTS = (4, 2, 2, 1, 4, 4)
    SEM_X = 0
    SEM_W = [3 + sum(WPARTS[:c]) for c in range(NCH)]
    SEM_O = 3 + sum(WPARTS)
    SEM_MISC = SEM_O + NWO

    def cp_x(i):
        r0, nr = ((24, 16), (0, 24), (40, 24))[i]
        return pltpu.make_async_copy(x_hbm.at[:, pl.ds(r0, nr), :],
                                     x_raw.at[pl.ds(1, NPAIR), pl.ds(r0, nr), :],
                                     sems.at[SEM_X + i])

    def cp_w(c, part):
        w = (wk_hbm, wv_hbm, wq_hbm)[c // 2]
        nd = D // WPARTS[c]
        return pltpu.make_async_copy(
            w.at[pl.ds(part * nd, nd), pl.ds((c % 2) * HC, HC), :],
            stage.at[pl.ds(c * D + part * nd, nd)], sems.at[SEM_W[c] + part])

    def cp_o(i):
        return pltpu.make_async_copy(wo_hbm.at[pl.ds(i * WOP, WOP)],
                                     wo_raw.at[pl.ds(i * WOP, WOP)], sems.at[SEM_O + i])

    cp_small = [pltpu.make_async_copy(s_, d_, sems.at[SEM_MISC + i])
                for i, (s_, d_) in enumerate(((mem0_hbm, mem0_v), (wr_hbm, wr_v)))]
    cp_mlp = [pltpu.make_async_copy(s_, d_, sems.at[SEM_MISC + 2 + i])
              for i, (s_, d_) in enumerate(((wg_hbm, wg_v), (wu_hbm, wu_v), (wd_hbm, wd_v)))]
    cp_x(0).start()
    for c in range(3):
        for part in range(WPARTS[c]):
            cp_w(c, part).start()
    cp_x(1).start()
    cp_x(2).start()
    cp_w(3, 0).start()
    for i in range(NWO):
        cp_w(4, i).start()
        cp_w(5, i).start()
        cp_o(i).start()
    for c in cp_small + cp_mlp:
        c.start()

    anchor[0] = PAIR
    anchor[1] = NCH * D
    anchor[2] = HD
    anchor[3] = NPAIR + 1
    x_raw[0] = jnp.zeros((PAIR, D), BF16)
    xres[0:PAD, :] = jnp.zeros((PAD, D), F32)

    cp_x(0).wait()

    def ln_mid(i, carry):
        for pp in range(LNP):
            pr = i * LNP + pp
            ln = _layernorm(x_raw[1 + pr, 24:40, :].astype(F32))
            hbuf[pl.ds(pl.multiple_of(PAD + pr * PAIR + 24, 8), 16), :] = ln
            lhs_pre[pl.ds(pl.multiple_of(pr * 8, 8), 8), :] = pltpu.bitcast(ln.astype(BF16), U32)
        return carry

    lax.fori_loop(0, NPAIR // LNP, ln_mid, 0)

    def ln_jobs(p0, npairs):
        def job(pp, ra, rb):
            xv = jnp.concatenate([x_raw[1 + p0 + pp, r:r + 8, :].astype(F32) for r in (ra, rb)],
                                 axis=0)
            ln = _layernorm(xv)
            for n, r in enumerate((ra, rb)):
                hbuf[pl.ds(pl.multiple_of(PAD + (p0 + pp) * PAIR + r, 8), 8), :] = (
                    ln[n * 8:(n + 1) * 8])

        return [('x_raw', functools.partial(job, pp, ra, rb))
                for pp in range(npairs) for ra, rb in ((0, 8), (16, 40), (48, 56))]

    def relayout_jobs(c, blk0, nblk, slot0=0):
        def job(u):
            t0 = ((slot0 + u) % NTMP) * TSZ
            d0 = pl.multiple_of(c * D + (blk0 + u) * 16, 16)
            raw = pltpu.bitcast(stage[pl.ds(d0, 16), :, :], U32)
            for i in range(8):
                ev, od = raw[2 * i], raw[2 * i + 1]
                lo = (ev & jnp.uint32(0xFFFF)) | (od << 16)
                hi = (ev >> 16) | (od & jnp.uint32(0xFFFF0000))
                tmp[pl.ds(t0 + i * TP, 8, stride=2), :] = lo
                tmp[pl.ds(t0 + i * TP + 1, 8, stride=2), :] = hi
            o0 = pl.multiple_of((blk0 + u) * 8, 8)
            for hh in range(HC):
                col = (hh % G) * DH
                wch[c][hh // G, pl.ds(o0, 8), col:col + DH] = tmp[pl.ds(t0 + hh, 8, stride=TP), :]

        return [('stage', functools.partial(job, u)) for u in range(nblk)]

    def repack_jobs(part):
        def job(c):
            r0 = pl.multiple_of(part * WOP + c * 128, 128)
            o0 = pl.multiple_of(part * (WOP // 2) + c * 64, 64)
            wo[pl.ds(o0, 64), :] = pltpu.bitcast(wo_raw[pl.ds(r0, 128), :], U32)

        return [('wo_raw', functools.partial(job, c)) for c in range(WOP // 128)]

    def interleave(*lists):
        keyed = [((i + 0.5) / len(l), n, j) for n, l in enumerate(lists) for i, j in enumerate(l)]
        return [j for _, _, j in sorted(keyed, key=lambda t: t[:2])]

    def precompute(c, g0, ng, jobs, k0=0, k1=D):
        lhs = pltpu.bitcast(lhs_pre[:, k0:k1], BF16)
        ys = [_dot(lhs, pltpu.bitcast(wch[c][g0 + gg, k0 // 2:k1 // 2, :], BF16))
              for gg in range(ng)]
        nrow = 16 * NPAIR
        has_ln = any(kind == 'x_raw' for kind, _ in jobs)
        for u, (kind, job) in enumerate(jobs):
            if u > 0:
                par = D // (k1 - k0)
                span = ng * G * nrow // par - (SLACK[1] if has_ln else SLACK[0])
                pos = max((u * span // len(jobs)) // 16 * 16 - 128, 0)
                nt, r0 = pos // nrow * par, pos % nrow
                tie = ys[nt // G][r0:r0 + 16, (nt % G) * DH:(nt % G + 1) * DH].astype(BF16)
                if kind == 'stage':
                    stage[anchor[1]] = tie
                elif kind == 'x_raw':
                    x_raw[anchor[3], 0:16, 0:DH] = tie
                else:
                    wo_raw[pl.ds(pl.multiple_of(anchor[2], 16), 16), 0:DH] = tie
            job()
        for gg in range(ng):
            if k0 > 0:
                pre[c * GPC + g0 + gg] += ys[gg]
            else:
                pre[c * GPC + g0 + gg] = ys[gg]

    def run(jobs):
        for _, job in jobs:
            job()

    NBLK = D // 16
    HB, QB = NBLK // 2, NBLK // 4
    cp_w(0, 0).wait()
    run(relayout_jobs(0, 0, QB))
    precompute(0, 0, GPC, [], 0, D // 4)
    cp_w(0, 1).wait()
    run(relayout_jobs(0, QB, QB))
    cp_w(0, 2).wait()
    cp_w(0, 3).wait()
    precompute(0, 0, GPC, relayout_jobs(0, HB, HB), D // 4, D // 2)

    def phase01(c, k0, it, carry):
        cp_w(c + 1, it).wait()
        precompute(c, it * 2, 2, relayout_jobs(c + 1, it * HB, HB), k0, D)
        return carry

    lax.fori_loop(0, 2, functools.partial(phase01, 0, D // 2), 0)
    lax.fori_loop(0, 2, functools.partial(phase01, 1, 0), 0)
    cp_x(1).wait()
    cp_x(2).wait()
    cp_w(3, 0).wait()
    lax.fori_loop(0, 2, lambda it, cr: (
        precompute(2, it * 2, 2, interleave(relayout_jobs(3, it * HB, HB),
                                            ln_jobs(it * (NPAIR // 2), NPAIR // 2))), cr)[1], 0)

    def last_phase(it, carry):
        cp_w(4, it).wait()
        cp_w(5, it).wait()
        cp_o(it).wait()
        precompute(3, it, 1, interleave(relayout_jobs(4, it * QB, QB),
                                        relayout_jobs(5, it * QB, QB, NTMP // 2),
                                        repack_jobs(it)))
        return carry

    lax.fori_loop(0, 4, last_phase, 0)

    for c in cp_small:
        c.wait()
    wr = wr_v[...].astype(F32).reshape(1, D)

    qi = lax.broadcasted_iota(jnp.int32, (32, 48), 0)
    kj = lax.broadcasted_iota(jnp.int32, (32, 48), 1)
    mask_a = (kj < 40) & ((qi < M) | (kj <= qi))
    qi = lax.broadcasted_iota(jnp.int32, (48, 80), 0)
    kj = lax.broadcasted_iota(jnp.int32, (48, 80), 1)
    kb0 = (kj >= 40) & (kj < 48)
    m_mem = (qi < M) & ((kj < 32) | kb0)
    m_xb = (qi >= M) & (qi < 32) & ((kj <= qi) | kb0)
    m_xa = (qi >= 32) & (qi < 40) & ((kj >= 48) | ((kj >= 32) & (kj <= qi)))
    m_b0 = (qi >= 40) & ((kj < M) | (kb0 & (kj <= qi)))
    mask_b = m_mem | m_xb | m_xa | m_b0

    def w_ref(mi, g):
        return wch[(4, 0, 2)[mi] + g // GPC].at[g % GPC]

    def wo_rows(g, n=1):
        r0 = g * GW // 2
        return pltpu.bitcast(wo[r0:r0 + n * GW // 2, :], BF16)

    def seg_step(lhs, lhs_f32, extra, mask, lags, s_mid, filler):
        q, k, v, p, o = {}, {}, {}, {}, {}
        raw = ({}, {}, {})
        acc = [None]

        def proj(mi, g, dst):
            if mi == 0 and g == 0 and lhs_f32 is not None:
                y = None
                lp = jnp.concatenate([lhs_f32[16:], lhs_f32[0:16]], axis=0)
                for kt in range(D // 128):
                    w = pltpu.bitcast(w_ref(0, 0)[kt * 64:(kt + 1) * 64, :], BF16)
                    t = _dot(lp[:, kt * 128:(kt + 1) * 128].astype(BF16), w)
                    y = t if y is None else y + t
                nr = y.shape[0]
                y = jnp.concatenate([y[nr - 16:], y[0:nr - 16]], axis=0)
            else:
                y = _dot(lhs[mi], pltpu.bitcast(w_ref(mi, g)[...], BF16))
            for j in range(G):
                h = g * G + j
                yh = y[:, j * DH:(j + 1) * DH]
                ex = extra(mi, h)
                if ex:
                    yh = jnp.concatenate([yh] + ex, axis=0)
                raw[mi][h] = yh
                dst[h] = yh.astype(BF16)

        def sc(g):
            for h in range(g * G, (g + 1) * G):
                p[h] = _softmax_bf16(_dot_nt(q[h], k[h]), mask)

        def pv(g):
            o[g] = jnp.concatenate(
                [_dot(p[h], v[h]) for h in range(g * G, (g + 1) * G)], axis=1)

        def op(g):
            if merge and g == NG - 2:
                return
            if merge and g == NG - 1:
                y = _dot(jnp.concatenate([o[g - 1], o[g]], axis=1).astype(BF16),
                         wo_rows(g - 1, 2))
            else:
                y = _dot(o[g].astype(BF16), wo_rows(g))
            acc[0] = y if acc[0] is None else acc[0] + y

        ls, lp, lo, merge, pv0 = lags
        for t in range(2 * NG + lp + lo):
            if t < NG:
                proj(0, t, q)
                if s_mid and 0 <= t - ls < NG:
                    sc(t - ls)
                proj(1, t, k)
            elif t < 2 * NG:
                proj(2, t - NG, v)
            if 0 <= t - ls < NG and not s_mid:
                sc(t - ls)
            if t == NG + lp + pv0:
                pv(0)
                if s_mid:
                    for g in range(NG - ls, NG):
                        sc(g)
            if 0 < t - NG - lp < NG:
                pv(t - NG - lp)
            if pv0 > lo - 1 and t == NG + lp + lo + 1:
                op(0)
            if (1 if pv0 > lo - 1 else 0) <= t - NG - lp - lo < NG:
                op(t - NG - lp - lo)
            if t in filler:
                src = raw[1][t * G] if t < NG else raw[2][min(t - NG, NG - 1) * G]
                filler[t](src[0:8])
        return acc[0], raw

    subr = lax.broadcasted_iota(jnp.int32, (RC, 128), 0).astype(F32)

    def post_chunk(li, pi, valid, c, tie=None):
        if tie is not None:
            obuf[pl.ds(pl.multiple_of(anchor[0], 8), 8), 0:DH] = tie
        base = pi * PAIR if isinstance(pi, int) else pl.multiple_of(pi * PAIR, PAIR)
        rows = pl.ds(base + c * RC, RC)
        x0 = x_raw[pi, c * RC:(c + 1) * RC, :].astype(F32) if li == 0 else xres[rows, :]
        x1 = _rnd(x0 + _rnd(obuf[c * RC:(c + 1) * RC, :]))
        ln = _layernorm(x1)
        r = _rnd(jnp.sum(ln * wr, axis=-1, keepdims=True))
        r = jnp.broadcast_to(jnp.where(valid, r, -jnp.inf), (RC, 128))
        rb = rbest[...]
        better = r > rb
        rbest[...] = jnp.where(better, r, rb)
        row0 = jnp.asarray(base + (c * RC - PAD), jnp.int32).astype(F32)
        ibest[...] = jnp.where(better, subr + row0, ibest[...])
        x1buf[rows, :] = x1
        lbuf[rows, :] = ln
        if li == 0:
            x2 = _rnd(x1 + ln)
            xres[rows, :] = x2
            hbuf[rows, :] = _layernorm(x2)
        else:
            ostage[rows, :] = (x1 + ln).astype(BF16)

    def out_copy(row0, nrows):
        return pltpu.make_async_copy(ostage.at[pl.ds(PAD + row0, nrows)],
                                     out_hbm.at[pl.ds(row0, nrows)], osem)

    def pair_body(li, pi, mem, first):
        base = pl.multiple_of(pi * PAIR, PAIR)
        ha = hbuf[pl.ds(base + PAD, 40), :]
        hb = hbuf[pl.ds(base + PAD + 40, 24), :]
        fill = ({}, {})
        for c, (st, t) in enumerate(FILL[li]):
            fill[st][t] = functools.partial(post_chunk, li, pi, pi > 0, c)
        aq = jnp.concatenate([mem, ha[0:24]], axis=0)
        lhs_aq = aq.astype(BF16)
        if li == 0:
            p0 = pl.multiple_of(pi * 16, 16)
            lhs_akv = lhs_aq
            extra_a = lambda mi, h: [pre[(mi - 1) * NG + h // G, pl.ds(p0, 16),
                                         (h % G) * DH:(h % G + 1) * DH]] if mi else []
        else:
            lhs_akv = jnp.concatenate([mem, ha], axis=0).astype(BF16)
            extra_a = lambda mi, h: []
        acc_a, prj = seg_step((lhs_aq, lhs_akv, lhs_akv), None if first else aq, extra_a, mask_a,
                              LAGA, SMID[0], fill[0])
        lhs_b = jnp.concatenate([acc_a[0:8], hb], axis=0).astype(BF16)
        bq = jnp.concatenate([acc_a[0:8], hb, ha[24:40]], axis=0)
        acc_b, _ = seg_step(
            (bq.astype(BF16), lhs_b, lhs_b), bq,
            lambda mi, h: [prj[mi][h][32:48], prj[mi][h][0:32]] if mi else [],
            mask_b, LAGB, SMID[1], fill[1])
        obuf[0:24, :] = acc_a[8:32]
        obuf[24:40, :] = acc_b[32:48]
        obuf[40:64, :] = acc_b[8:32]
        return acc_b[0:8]

    def loop_body(li, it, mem):
        UNROLL = UNROLLS[li]
        for u in range(UNROLL):
            mem = pair_body(li, it * UNROLL + u, mem, u == 0)

        if li == 1:
            @pl.when(it > 0)
            def _():
                out_copy(pl.multiple_of(it * (UNROLL * PAIR) - PAIR, PAIR),
                         UNROLL * PAIR).start()

            if UNROLL > 1:
                @pl.when(it == 0)
                def _():
                    out_copy(0, (UNROLL - 1) * PAIR).start()

        return mem

    for li in range(2):
        obuf[0:PAIR, :] = jnp.zeros((PAIR, D), F32)
        rbest[...] = jnp.full((RC, 128), -jnp.inf, F32)
        ibest[...] = jnp.zeros((RC, 128), F32)
        lax.fori_loop(0, NPAIR // UNROLLS[li], functools.partial(loop_body, li),
                      mem0_v[...].astype(F32))

        if li == 0:
            for c in cp_mlp:
                c.wait()
        else:
            out_copy(0, S - PAIR).wait()

        def top1():
            rb = rbest[...]
            rmax = jnp.max(rb, axis=0, keepdims=True)
            imin = jnp.min(jnp.where(rb == rmax, ibest[...], S - 1.0), axis=0, keepdims=True)
            return rmax, imin.astype(jnp.int32)[0, 0]

        def mod_trip(carry, li=li):
            rmax, idx = top1()
            lsel = lbuf[pl.ds(PAD + idx, 1), :]
            for c in range(PAIR // RC):
                post_chunk(li, NPAIR, True, c)
            xs = jnp.broadcast_to(lsel, (16, D)).astype(BF16)
            acts = []
            for f0, f1 in FSPLIT:
                gpre = _rnd(_dot(xs, wg_v[:, f0:f1]))
                gate = _rnd(gpre * _rnd(jax.nn.sigmoid(gpre)))
                up = _rnd(_dot(xs, wu_v[:, f0:f1]))
                acts.append((gate * up).astype(BF16))
            y = None
            for (f0, f1), act in zip(FSPLIT, acts):
                t = _dot(act, wd_v[f0:f1, :])
                y = t if y is None else y + t
            y = _rnd(y)[0:8]
            rsel = _rnd(jax.nn.sigmoid(rmax[:, 0:1]))
            ybuf[...] = _rnd(y * rsel)
            return idx, top1()[1]

        idx, _ = lax.while_loop(lambda cr: cr[0] != cr[1], mod_trip,
                                (jnp.int32(-1), jnp.int32(0)))
        row = pl.ds(PAD + idx, 1)
        lsel = lbuf[row, :]
        y = ybuf[0:1, :]
        if li == 0:
            x2 = _rnd(x1buf[row, :] + _rnd(lsel + y))
            xres[row, :] = x2
            hbuf[row, :] = _layernorm(x2)
        else:
            t0 = pl.multiple_of((idx // 16) * 16, 16)
            tile = pl.ds(PAD + t0, 16)
            sel = lax.broadcasted_iota(jnp.int32, (16, D), 0) == idx - t0
            upd = jnp.where(sel, jnp.broadcast_to(y, (16, D)), 0.0)
            ostage[tile, :] = (x1buf[tile, :] + _rnd(lbuf[tile, :] + upd)).astype(BF16)
            t1 = pl.multiple_of(jnp.minimum(t0, S - PAIR - 16), 16)
            last = [out_copy(S - PAIR, PAIR), out_copy(t1, 16)]
            for cp in last:
                cp.start()
            for cp in last:
                cp.wait()


_FILL = ((0, 9), (0, 12), (0, 15), (1, 8), (1, 10), (1, 12), (1, 14), (1, 15))
CFG = dict(UNROLLS=(2, 2), LAGA=(1, 1, 2, True, 0), LAGB=(1, 1, 2, False, 1), FILL=(_FILL, _FILL),
           SMID=(False, True), LNP=16, SLACK=(128, 256))


def _build():
    any_spec = pl.BlockSpec(memory_space=pl.ANY)
    return pl.pallas_call(
        functools.partial(_kernel, **CFG),
        out_shape=jax.ShapeDtypeStruct((S, D), BF16),
        in_specs=[any_spec] * 10,
        out_specs=any_spec,
        scratch_shapes=[
            pltpu.VMEM((NPAIR + 2, PAIR, D), BF16),
            pltpu.VMEM((M, D), BF16),
            pltpu.VMEM((D,), BF16),
            pltpu.VMEM((NCH * D + 1, HC, DH), BF16),
            pltpu.VMEM((HD + 16, D), BF16),
            pltpu.VMEM((D, FF), BF16),
            pltpu.VMEM((D, FF), BF16),
            pltpu.VMEM((FF, D), BF16),
        ] + [pltpu.VMEM((GPC, D // 2, GW), U32)] * NCH + [
            pltpu.VMEM((HD // 2, D), U32),
            pltpu.VMEM((NTMP * TSZ, DH), U32),
            pltpu.VMEM((PAD + S, D), F32),
            pltpu.VMEM((PAD + S, D), F32),
            pltpu.VMEM((PAD + S, D), F32),
            pltpu.VMEM((PAD + S, D), F32),
            pltpu.VMEM((RC, 128), F32),
            pltpu.VMEM((RC, 128), F32),
            pltpu.VMEM((PAIR + 8, D), F32),
            pltpu.VMEM((PAD + S, D), BF16),
            pltpu.VMEM((8 * NPAIR, D), U32),
            pltpu.VMEM((2 * NG, 16 * NPAIR, GW), F32),
            pltpu.VMEM((8, D), F32),
            pltpu.SMEM((4,), jnp.int32),
            pltpu.SemaphoreType.DMA((29,)),
            pltpu.SemaphoreType.DMA(()),
        ],
        compiler_params=pltpu.CompilerParams(vmem_limit_bytes=120 * 1024 * 1024),
    )


@jax.jit
def pallas_interleave_layers__memory_aug_recurrent_mem_tr__moe_arch_mod__prompt_kernel(
    A_x: jax.Array,
    A_mem0: jax.Array,
    A_Wq: jax.Array,
    A_Wk: jax.Array,
    A_Wv: jax.Array,
    A_Wo: jax.Array,
    A_seg_len,
    B_x: jax.Array,
    B_w_r: jax.Array,
    B_w_gate: jax.Array,
    B_w_up: jax.Array,
    B_w_down: jax.Array,
):
    assert A_x.shape == (1, S, D) and A_mem0.shape == (1, M, D) and A_Wq.shape == (D, H, DH)
    del A_seg_len
    del B_x
    out = _build()(
        A_x.reshape(NPAIR, PAIR, D),
        A_mem0.reshape(M, D),
        A_Wq,
        A_Wk,
        A_Wv,
        A_Wo.reshape(HD, D),
        B_w_r,
        B_w_gate,
        B_w_up,
        B_w_down,
    )
    return out.reshape(1, S, D)
```
